```python
import jax
import jax.numpy as jnp

def _softmax(x, axis=-1):
    return jax.nn.softmax(x, axis=axis)

def _gelu(x):
    return jax.nn.gelu(x, approximate=True)

def _silu(x):
    return jax.nn.silu(x)

def _sigmoid(x):
    return jax.nn.sigmoid(x)

def _layernorm(x, axis=-1, eps=1e-05):
    m = jnp.mean(x, axis=axis, keepdims=True)
    v = jnp.var(x, axis=axis, keepdims=True)
    return (x - m) / jnp.sqrt(v + eps)

def _scatter_add(tgt, idx, src, axis=0):
    return tgt.at[idx].add(src)

def _segment_sum(src, seg, n):
    return jax.ops.segment_sum(src, seg, n)

class _Rng:

    def __init__(self, key):
        self._k = key

    def _next(self):
        self._k, sub = jax.random.split(self._k)
        return sub

    def normal(self, shape):
        return jax.random.normal(self._next(), shape, dtype=jnp.bfloat16)

    def randint(self, lo, hi, shape):
        return jax.random.randint(self._next(), shape, lo, hi, dtype=jnp.int32)

    def uniform(self, shape, lo=0.0, hi=1.0):
        return jax.random.uniform(self._next(), shape, jnp.bfloat16, lo, hi)

    def permutation(self, n):
        return jax.random.permutation(self._next(), n)
kernel_name = 'concat_heads__spectral_gfnet__memory_aug_recurrent_mem_tr__prompt'

def setup_inputs():
    _rng = _Rng(jax.random.key(int.from_bytes(__import__("os").urandom(4), "little")))
    _w = lambda a: (lambda t: t.astype(jnp.bfloat16) if jnp.issubdtype(t.dtype, jnp.floating) else t)(jnp.asarray(a))

    def _A_setup():
        B, S, D = (1, 2048, 1024)
        Df = D // 2 + 1
        return {'x': _w((lambda *s: _rng.normal(s) * 0.05)(B, S, D)), 'w_r': _w((lambda *s: _rng.normal(s) * 0.05)(S, Df) * 0.02), 'w_i': _w((lambda *s: _rng.normal(s) * 0.05)(S, Df) * 0.02)}
    _A_in = _A_setup()

    def _B_setup():
        B, S, Dm = (1, 2048, 1024)
        H, Dh = (32, 128)
        M, seg = (8, 32)
        seg = min(seg, S)
        S = S // seg * seg
        return {'x': _w((lambda *s: _rng.normal(s) * 0.05)(B, S, Dm)), 'mem0': _w((lambda *s: _rng.normal(s) * 0.05)(B, M, Dm)), 'Wq': _w((lambda *s: _rng.normal(s) * 0.05)(Dm, H, Dh) * Dm ** (-0.5)), 'Wk': _w((lambda *s: _rng.normal(s) * 0.05)(Dm, H, Dh) * Dm ** (-0.5)), 'Wv': _w((lambda *s: _rng.normal(s) * 0.05)(Dm, H, Dh) * Dm ** (-0.5)), 'Wo': _w((lambda *s: _rng.normal(s) * 0.05)(H, Dh, Dm) * (H * Dh) ** (-0.5)), 'seg_len': seg}
    _B_in = _B_setup()
    return {'A_x': _A_in['x'], 'A_w_r': _A_in['w_r'], 'A_w_i': _A_in['w_i'], 'B_x': _B_in['x'], 'B_mem0': _B_in['mem0'], 'B_Wq': _B_in['Wq'], 'B_Wk': _B_in['Wk'], 'B_Wv': _B_in['Wv'], 'B_Wo': _B_in['Wo'], 'B_seg_len': _B_in['seg_len']}

def reference(A_x, A_w_r, A_w_i, B_x, B_mem0, B_Wq, B_Wk, B_Wv, B_Wo, B_seg_len):

    def _A_ref(x, w_r, w_i):
        B, S, D = x.shape
        X = (lambda x, axes=(-2, -1): jnp.fft.rfft2(x.astype(jnp.float32), axes=axes))(x, axes=(-2, -1))
        W = w_r + 1j * w_i
        X = X * W
        y = (lambda x, s, axes=(-2, -1): jnp.fft.irfft2(x, s=s, axes=axes).astype(jnp.bfloat16))(X, (S, D), axes=(-2, -1))
        return y

    def _B_ref(x, mem0, Wq, Wk, Wv, Wo, seg_len):
        B, S, Dm = x.shape
        H, Dh = (Wq.shape[1], Wq.shape[2])
        M = mem0.shape[1]
        scale = Dh ** (-0.5)
        n_seg = S // seg_len
        L = M + seg_len
        idx = jnp.arange(L)
        mask = (idx[:, None] < M) | (idx[:, None] >= idx[None, :])
        mem = mem0
        outs = []
        for s in range(n_seg):
            xs = x[:, s * seg_len:(s + 1) * seg_len, :].copy()
            h = jnp.concatenate([mem, xs], axis=1)
            q = jnp.einsum('btd,dhe->bhte', h, Wq)
            k = jnp.einsum('btd,dhe->bhte', h, Wk)
            v = jnp.einsum('btd,dhe->bhte', h, Wv)
            scores = jnp.einsum('bhqe,bhke->bhqk', q, k) * scale
            scores = jnp.where(mask[None, None], scores, -1000000000.0)
            p = _softmax(scores, axis=-1)
            o = jnp.einsum('bhqk,bhke->bhqe', p, v)
            o = jnp.einsum('bhte,hed->btd', o, Wo)
            mem = o[:, :M, :].copy()
            outs.append(o[:, M:, :])
        return jnp.concatenate(outs, axis=1)
    a = _A_ref(A_x, A_w_r, A_w_i)
    b = _B_ref(B_x, B_mem0, B_Wq, B_Wk, B_Wv, B_Wo, B_seg_len)
    return jnp.concatenate([a, b], axis=-1)
```

```python
import functools

import jax
import jax.numpy as jnp
import numpy as np
from jax.experimental import pallas as pl
from jax.experimental.pallas import tpu as pltpu

S, D = 2048, 1024
H, DH, M, SEG = 32, 128, 8, 32
L = M + SEG
NSEG = S // SEG
P, Q = 16, 128
CB = 16
NCH = Q // CB
NB = 5
PITCH = 40
RS = float(np.sqrt(0.5))
CLASSES = ((0, 4), (1, 7), (2, 6), (3, 5))

NN = (((1,), (0,)), ((), ()))
NT = (((1,), (1,)), ((), ()))


def _dot(a, b, dims=NN):
    return jax.lax.dot_general(a, b, dims, preferred_element_type=jnp.float32)


def _bf16(w):
    return pltpu.bitcast(w, jnp.bfloat16)


def _words(x):
    return pltpu.bitcast(x.astype(jnp.bfloat16), jnp.uint32)


def _radix8(x):
    t0 = x[0] + x[4]; t1 = x[0] - x[4]; t2 = x[2] + x[6]; t3 = x[2] - x[6]
    t4 = x[1] + x[5]; t5 = x[1] - x[5]; t6 = x[3] + x[7]; t7 = x[3] - x[7]
    e = t0 + t2; o = t4 + t6
    u = (t5 - t7) * RS; w = (t5 + t7) * RS
    return [e + o, e - o, t1 + u, t3 + w, t0 - t2, t4 - t6, t1 - u, t3 - w]


def _radix8_t(p):
    e = p[0] + p[1]; o = p[0] - p[1]
    t1 = p[2] + p[6]; u = (p[2] - p[6]) * RS
    t3 = p[3] + p[7]; w = (p[3] - p[7]) * RS
    t0 = e + p[4]; t2 = e - p[4]
    t4 = o + p[5]; t6 = o - p[5]
    t5 = w + u; t7 = w - u
    return [t0 + t1, t4 + t5, t2 + t3, t6 + t7, t0 - t1, t4 - t5, t2 - t3, t6 - t7]


def _radix4(ar, ai):
    s0r = ar[0] + ar[2]; s0i = ai[0] + ai[2]; d0r = ar[0] - ar[2]; d0i = ai[0] - ai[2]
    s1r = ar[1] + ar[3]; s1i = ai[1] + ai[3]; d1r = ar[1] - ar[3]; d1i = ai[1] - ai[3]
    return ([s0r + s1r, d0r + d1i, s0r - s1r, d0r - d1i],
            [s0i + s1i, d0i - d1r, s0i - s1i, d0i + d1r])


def _radix16(xr, xi):
    ur = [[None] * 4 for _ in range(4)]
    ui = [[None] * 4 for _ in range(4)]
    for n in range(4):
        pr, pi = _radix4([xr[4 * m + n] for m in range(4)], [xi[4 * m + n] for m in range(4)])
        for p in range(4):
            e = n * p
            r, i = pr[p], pi[p]
            if e == 4:
                r, i = i, -r
            elif e == 2:
                r, i = (r + i) * RS, (i - r) * RS
            elif e == 6:
                r, i = (i - r) * RS, (r + i) * (-RS)
            elif e != 0:
                c, s = float(np.cos(np.pi * e / 8)), float(-np.sin(np.pi * e / 8))
                r, i = r * c - i * s, r * s + i * c
            ur[n][p], ui[n][p] = r, i
    yr = [None] * 16
    yi = [None] * 16
    for p in range(4):
        qr, qi = _radix4([ur[n][p] for n in range(4)], [ui[n][p] for n in range(4)])
        for q in range(4):
            yr[p + 4 * q], yi[p + 4 * q] = qr[q], qi[q]
    return yr, yi


def _pack_rows(a):
    u = np.ascontiguousarray(a, np.float32).view(np.uint32)
    u = (u + 0x7FFF + ((u >> 16) & 1)) >> 16
    return np.ascontiguousarray(u[..., 0::2, :] | (u[..., 1::2, :] << 16))


def _tables():
    r = np.array(_radix8(list(np.eye(8))))
    e = np.exp(-2j * np.pi * np.outer(np.arange(8), np.arange(8)) / 8)
    c = e @ np.linalg.inv(r)
    lane = np.arange(128)
    f = np.zeros((4, 256, 256))
    for j in range(4):
        cls = np.where(lane >= 64, CLASSES[j][1], CLASSES[j][0])
        v = 8 * (lane & 63) + cls
        ph = np.exp(-2j * np.pi * ((lane[:, None] * v[None, :]) % D) / D)
        for pp in range(2):
            z = c[cls, 2 * j + pp][None, :] * ph
            f[j, 128 * pp:128 * pp + 128, :128] = z.real
            f[j, 128 * pp:128 * pp + 128, 128:] = z.imag
    f[0, :128, 128] = c[0, 0].real * (1 - 2 * (lane % 2))
    f[0, 128:, 128] = 0
    fi = np.transpose(f, (0, 2, 1)).copy()
    fi[0, 0, :] *= 0.5
    fi[0, 128, :] *= 0.5
    g = np.zeros((P, 2 * Q, 2 * Q))
    for k1 in range(P):
        u = k1 + P * np.arange(Q)
        z = np.exp(-2j * np.pi * ((u[:, None] * np.arange(Q)[None, :]) % S) / S)
        g[k1] = np.block([[z.real, -z.imag], [z.imag, z.real]])
    gi = np.transpose(g, (0, 2, 1)) * (2.0 / (S * D))
    return _pack_rows(np.concatenate([f, fi])), _pack_rows(np.concatenate([g, gi]))


_F_TAB, _G_TAB = _tables()


def _make_kernel(cfg):
    scope = jax.named_scope if cfg.get("scopes") else (lambda name: _Null())
    split = cfg.get("split", 16)
    nbulk = cfg.get("nbulk", 0)
    do_a = cfg.get("do_a", True)
    nseg = cfg.get("nseg", NSEG)

    def kernel(xa_hbm, wr_hbm, wi_hbm, xb_hbm, mem0_hbm, wq_hbm, wk_hbm, wv_hbm, wo_hbm, f_hbm, g_hbm,
               out_hbm,
               wqkv, wo, stage, xb, mem0, outb, h_scr, o_scr, acc_scr,
               sem_w, sem_o, sem_x, sem_out):
        w_hbm = (wq_hbm, wk_hbm, wv_hbm)

        def w_copy(i):
            return pltpu.make_async_copy(w_hbm[i].bitcast(jnp.uint32), stage[i].at[:, 0:32, :], sem_w.at[i])

        def wo_copy(n):
            return pltpu.make_async_copy(wo_hbm.bitcast(jnp.uint32).at[:, pl.ds(128 * n, 128)], wo.at[n], sem_o.at[n])

        xb_copy = pltpu.make_async_copy(xb_hbm, xb, sem_x.at[0])
        mem_copy = pltpu.make_async_copy(mem0_hbm, mem0, sem_x.at[1])

        def start_wo():
            def body(n, c):
                pltpu.make_async_copy(
                    wo_hbm.bitcast(jnp.uint32).at[:, pl.ds(pl.multiple_of(128 * n, 128), 128)], wo.at[n],
                    sem_o.at[n]).start()
                return c

            jax.lax.fori_loop(0, 8, body, 0)

        b_stages = [mem_copy.start]
        if nbulk:
            b_stages.append(xb_copy.start)
        b_stages += [lambda: w_copy(0).start(), lambda: w_copy(1).start(), lambda: w_copy(2).start(), start_wo]
        if not nbulk:
            b_stages.append(xb_copy.start)

        def start_b_copies():
            def body(t, c):
                for n, st in enumerate(b_stages):
                    pl.when(t == n)(st)
                return c

            jax.lax.fori_loop(0, len(b_stages), body, 0)

        def relayout(i):
            su = stage[i].reshape(D // 2 * PITCH, 128)
            npair = 32

            def body(t, c):
                sv = su.at[pl.ds(pl.multiple_of(t * (npair * PITCH), npair * PITCH), npair * PITCH), :]
                ob = pl.multiple_of(t * npair, npair)
                for j in range(H // 2):
                    a = sv[pl.ds(j, npair, stride=PITCH), :]
                    b = sv[pl.ds(H // 2 + j, npair, stride=PITCH), :]
                    wqkv[i * H + 2 * j, pl.ds(ob, npair), :] = (a & jnp.uint32(0xFFFF)) | (b << 16)
                    wqkv[i * H + 2 * j + 1, pl.ds(ob, npair), :] = (a >> 16) | (b & jnp.uint32(0xFFFF0000))
                return c

            jax.lax.fori_loop(0, D // 2 // npair, body, 0)

        def branch_a(xa, f_tab, g_tab, w_st, w_last, w_perm, spec, planes, freq, ya, sem_a, sem_c, sem_y):
            def xa_copy(i):
                return pltpu.make_async_copy(
                    xa_hbm.bitcast(jnp.uint32).at[:, pl.ds(CB // 2 * i, CB // 2), :], xa.at[i], sem_a.at[i])

            f_copy = pltpu.make_async_copy(f_hbm, f_tab, sem_c.at[0])
            g_copy = pltpu.make_async_copy(g_hbm, g_tab, sem_c.at[1])
            w_copies = []
            for t, src in enumerate((wr_hbm, wi_hbm)):
                src_words = src.at[pl.ds(0, D // 2), :].bitcast(jnp.uint32)
                for ub in range(P):
                    w_copies.append(pltpu.make_async_copy(
                        src_words.at[:, pl.ds(128 * ub, 128)], w_st.at[t, ub], sem_c.at[2 + t]))
                w_copies.append(pltpu.make_async_copy(src.at[pl.ds(D // 2, 1), :], w_last.at[t], sem_c.at[4 + t]))

            def y_copy(i):
                return pltpu.make_async_copy(ya.at[i], out_hbm.at[:, pl.ds(CB * i, CB), pl.ds(0, D)], sem_y.at[i])

            f_copy.start()

            def start_xa(i, c):
                pltpu.make_async_copy(
                    xa_hbm.bitcast(jnp.uint32).at[:, pl.ds(pl.multiple_of(CB // 2 * i, CB // 2), CB // 2), :],
                    xa.at[i], sem_a.at[i]).start()
                return c

            jax.lax.fori_loop(0, NCH, start_xa, 0)
            for c in w_copies:
                c.start()

            def start_rest(t, c):
                pl.when(t == 0)(g_copy.start)
                pl.when(t == 1)(start_b_copies)
                return c

            jax.lax.fori_loop(0, 2, start_rest, 0)

            lane = jax.lax.broadcasted_iota(jnp.int32, (8, 128), 1)
            lane0 = lane == 0

            f_copy.wait()

            def fwd(i, carry):
                xa_copy_wait(i)
                for a in range(P):
                    x = _bf16(xa[i, a]).astype(jnp.float32)
                    pl_ = _radix8([x[:, 128 * c:128 * c + 128] for c in range(8)])
                    for c in range(8):
                        planes[CB * a:CB * a + CB, 128 * c:128 * c + 128] = pl_[c]
                for j in range(4):
                    freq[:, 256 * j:256 * j + 256] = _dot(planes[:, 256 * j:256 * j + 256], _bf16(f_tab[j]))
                row = pl.multiple_of(i * (CB // 2), CB // 2)
                for j in range(NB):
                    outr = [[] for _ in range(P)]
                    outi = [[] for _ in range(P)]
                    for hh in range(CB // 8):
                        def at(a, col):
                            return freq[CB * a + 8 * hh:CB * a + 8 * hh + 8, col:col + 128]
                        if j == 0:
                            xr = [at(a, 0) for a in range(P)]
                            xi = [jnp.where(lane0, 0.0, at(a, 128)) for a in range(P)]
                        elif j < 4:
                            xr = [at(a, 256 * j) for a in range(P)]
                            xi = [at(a, 256 * j + 128) for a in range(P)]
                        else:
                            xr = [jnp.where(lane0, at(a, 128), 0.0) for a in range(P)]
                            xi = [jnp.zeros((8, 128), jnp.float32)] * P
                        yr, yi = _radix16(xr, xi)
                        for k in range(P):
                            outr[k].append(yr[k])
                            outi[k].append(yi[k])
                    for k in range(P):
                        spec[k, pl.ds(row, CB // 2), 128 * j:128 * j + 128] = _words(jnp.concatenate(outr[k], 0))
                        spec[k, pl.ds(Q // 2 + row, CB // 2), 128 * j:128 * j + 128] = _words(
                            jnp.concatenate(outi[k], 0))
                return carry

            def xa_copy_wait(i):
                pltpu.make_async_copy(xa.at[i], xa.at[i], sem_a.at[i]).wait()

            with scope("a_fwd"):
                jax.lax.fori_loop(0, NCH, fwd, 0)

            for c in w_copies:
                c.wait()
            with scope("a_wperm"):
                def wperm(ub, carry):
                    ln = jax.lax.broadcasted_iota(jnp.int32, (128, 128), 1)
                    idx = 16 * (ln & 7) + (ln >> 3)
                    cls = {}
                    for p in range(4):
                        a = w_st[0, ub, pl.ds(p, 64, stride=4), :]
                        b = w_st[1, ub, pl.ds(p, 64, stride=4), :]
                        cls[2 * p] = (a & jnp.uint32(0xFFFF)) | (b << 16)
                        cls[2 * p + 1] = (a >> 16) | (b & jnp.uint32(0xFFFF0000))
                    tiles = [jnp.concatenate([cls[ca], cls[cb]], 0) for ca, cb in CLASSES]
                    cols = pl.ds(pl.multiple_of(ub * 128, 128), 128)
                    a = jax.lax.bitcast_convert_type(w_last[0, :, cols].astype(jnp.float32), jnp.uint32)
                    b = jax.lax.bitcast_convert_type(w_last[1, :, cols].astype(jnp.float32), jnp.uint32)
                    rw = jax.lax.broadcasted_iota(jnp.int32, (128, 128), 0)
                    tiles.append(jnp.where(rw == 0, jnp.broadcast_to((a >> 16) | b, (128, 128)), jnp.uint32(0)))
                    rows = pl.ds(pl.multiple_of(ub * 8, 8), 8)
                    for j in range(NB):
                        t = jnp.take_along_axis(tiles[j], idx, axis=1, mode="promise_in_bounds").T
                        for k in range(P):
                            w_perm[j, k, rows, :] = t[8 * k:8 * k + 8]
                    return carry

                jax.lax.fori_loop(0, P, wperm, 0)
            g_copy.wait()

            def mid(k):
                g = _bf16(g_tab[k])
                gi = _bf16(g_tab[P + k])
                for j in range(NB):
                    x = _dot(g, _bf16(spec[k, :, 128 * j:128 * j + 128]))
                    w = w_perm[j, k]
                    wr = jax.lax.bitcast_convert_type(w << 16, jnp.float32)
                    wi = jax.lax.bitcast_convert_type(w & jnp.uint32(0xFFFF0000), jnp.float32)
                    xr, xi = x[:Q], x[Q:]
                    y = jnp.concatenate([xr * wr - xi * wi, xr * wi + xi * wr], 0).astype(jnp.bfloat16)
                    spec[k, :, 128 * j:128 * j + 128] = _words(_dot(gi, y))

            with scope("a_mid"):
                for k in range(P):
                    mid(k)

            def inv(i, carry):
                row = pl.multiple_of(i * (CB // 2), CB // 2)
                nyq = {}
                for j in (4, 0, 1, 2, 3):
                    br = [_bf16(spec[k, pl.ds(row, CB // 2), 128 * j:128 * j + 128]).astype(jnp.float32)
                          for k in range(P)]
                    bi = [_bf16(spec[k, pl.ds(Q // 2 + row, CB // 2), 128 * j:128 * j + 128]).astype(jnp.float32)
                          for k in range(P)]
                    for hh in range(CB // 8):
                        zi, zr = _radix16([b[8 * hh:8 * hh + 8] for b in bi], [b[8 * hh:8 * hh + 8] for b in br])
                        for a in range(P):
                            r0 = CB * a + 8 * hh
                            if j == 4:
                                nyq[a, hh] = zr[a]
                            else:
                                freq[r0:r0 + 8, 256 * j:256 * j + 128] = zr[a]
                                freq[r0:r0 + 8, 256 * j + 128:256 * j + 256] = (
                                    jnp.where(lane0, nyq[a, hh], zi[a]) if j == 0 else zi[a])
                for j in range(4):
                    planes[:, 256 * j:256 * j + 256] = _dot(freq[:, 256 * j:256 * j + 256], _bf16(f_tab[4 + j]))
                for a in range(P):
                    y = _radix8_t([planes[CB * a:CB * a + CB, 128 * c:128 * c + 128] for c in range(8)])
                    for c in range(8):
                        ya[i, a, :, 128 * c:128 * c + 128] = y[c].astype(jnp.bfloat16)
                pltpu.make_async_copy(
                    ya.at[i], out_hbm.at[:, pl.ds(pl.multiple_of(CB * i, CB), CB), pl.ds(0, D)], sem_y.at[i]).start()
                return carry

            with scope("a_inv"):
                jax.lax.fori_loop(0, NCH, inv, 0)

            for i in range(NCH):
                y_copy(i).wait()

        if do_a:
            pl.run_scoped(
                branch_a,
                pltpu.VMEM((NCH, P, CB // 2, D), jnp.uint32),
                pltpu.VMEM((8, 128, 256), jnp.uint32),
                pltpu.VMEM((2 * P, Q, 2 * Q), jnp.uint32),
                pltpu.VMEM((2, P, D // 4, 128), jnp.uint32),
                pltpu.VMEM((2, 1, S), jnp.bfloat16),
                pltpu.VMEM((NB, P, Q, 128), jnp.uint32),
                pltpu.VMEM((P, Q, NB * 128), jnp.uint32),
                pltpu.VMEM((P * CB, D), jnp.float32),
                pltpu.VMEM((P * CB, D), jnp.float32),
                pltpu.VMEM((NCH, P, CB, D), jnp.bfloat16),
                pltpu.SemaphoreType.DMA((NCH,)),
                pltpu.SemaphoreType.DMA((6,)),
                pltpu.SemaphoreType.DMA((NCH,)),
            )
        else:
            start_b_copies()

        def branch_b(xbulk, bulk):
            if nbulk:
                xb_copy.wait()

                def gather(t, c):
                    x = xb[pl.ds(pl.multiple_of(t * 8, 8), 8), SEG - 8:SEG, :].astype(jnp.float32)
                    xbulk[pl.ds(pl.multiple_of(t * 64, 64), 64), :] = x.reshape(64, D)
                    return c

                jax.lax.fori_loop(0, NSEG // 8, gather, 0)
            for i in range(3):
                with scope("relayout%d" % i):
                    w_copy(i).wait()
                    relayout(i)
                if i < nbulk:
                    def bulk_head(t, c, i=i):
                        for u in range(cfg.get("bulk_unroll", 4)):
                            hd = i * H + t * cfg.get("bulk_unroll", 4) + u
                            bulk[hd] = _dot(xbulk[...], _bf16(wqkv[hd]))
                        return c

                    with scope("bulk%d" % i):
                        jax.lax.fori_loop(0, H // cfg.get("bulk_unroll", 4), bulk_head, 0)
            for n in range(8):
                wo_copy(n).wait()
            if not nbulk:
                xb_copy.wait()
            mem_copy.wait()

            scale = DH ** -0.5
            h_scr[0:M, :] = mem0[...].astype(jnp.float32)
            qi = jax.lax.broadcasted_iota(jnp.int32, (L, L), 0)
            ki = jax.lax.broadcasted_iota(jnp.int32, (L, L), 1)
            mask = (qi < M) | (qi >= ki)

            def out_copy(s):
                return pltpu.make_async_copy(
                    outb.at[s],
                    out_hbm.at[s // 4, pl.ds(pl.multiple_of((s % 4) * SEG, SEG), SEG), pl.ds(D, D)], sem_out)

            def step(s, carry):
                h_scr[M:L, :] = xb[s].astype(jnp.float32)
                qkv, sc, pp = {}, {}, {}

                def proj(i, hd):
                    w = _bf16(wqkv[i * H + hd])
                    if i < nbulk:
                        return jnp.concatenate(
                            [_dot(h_scr[0:L - 8, :], w), bulk[i * H + hd, pl.ds(pl.multiple_of(s * 8, 8), 8), :]], 0)
                    return _dot(h_scr[...], w)

                def wo1(n):
                    acc_scr[:, 128 * n:128 * n + 128] = _dot(
                        o_scr[:, 0:split * DH], _bf16(wo[n, 0:split * DH // 2, :]))

                tail = list(range(8))
                for i in range(H + 3):
                    if i < H:
                        qkv[i] = (proj(0, i), proj(1, i).astype(jnp.bfloat16), proj(2, i).astype(jnp.bfloat16))
                    else:
                        for _ in range(3):
                            if tail:
                                wo1(tail.pop(0))
                    if 0 <= i - 1 < H:
                        sc[i - 1] = _dot(qkv[i - 1][0], qkv[i - 1][1], NT)
                    if 0 <= i - 2 < H:
                        z = jnp.where(mask, sc.pop(i - 2) * scale, -1e9)
                        e = jnp.exp(z - jnp.max(z, axis=-1, keepdims=True))
                        pp[i - 2] = e / jnp.sum(e, axis=-1, keepdims=True)
                    if 0 <= i - 3 < H:
                        o_scr[:, (i - 3) * DH:(i - 2) * DH] = _dot(pp.pop(i - 3), qkv.pop(i - 3)[2])
                for n in range(8):
                    r = (_dot(o_scr[:, split * DH:], _bf16(wo[n, split * DH // 2:, :]))
                         + acc_scr[:, 128 * n:128 * n + 128])
                    h_scr[0:M, 128 * n:128 * n + 128] = r[0:M]
                    outb[s, :, 128 * n:128 * n + 128] = r[M:L].astype(jnp.bfloat16)
                out_copy(s).start()
                return carry

            with scope("chain"):
                jax.lax.fori_loop(0, nseg, step, 0)

            def drain(s, carry):
                out_copy(s).wait()
                return carry

            jax.lax.fori_loop(0, nseg, drain, 0)

        pl.run_scoped(
            branch_b,
            pltpu.VMEM((NSEG * 8, D), jnp.float32),
            pltpu.VMEM((max(nbulk * H, 1), NSEG * 8, DH), jnp.float32),
        )

    return kernel


class _Null:
    def __enter__(self):
        return self

    def __exit__(self, *a):
        return False


def make(cfg):
    kernel = _make_kernel(cfg)

    @functools.partial(jax.jit, static_argnames=("B_seg_len",))
    def f(A_x, A_w_r, A_w_i, B_x, B_mem0, B_Wq, B_Wk, B_Wv, B_Wo, B_seg_len):
        assert B_seg_len == SEG
        any_spec = pl.BlockSpec(memory_space=pltpu.HBM)
        out = pl.pallas_call(
            kernel,
            out_shape=jax.ShapeDtypeStruct((P, Q, 2 * D), jnp.bfloat16),
            in_specs=[any_spec] * 11,
            out_specs=any_spec,
            scratch_shapes=[
                pltpu.VMEM((3 * H, D // 2, DH), jnp.uint32),
                pltpu.VMEM((8, H * DH // 2, 128), jnp.uint32),
                [pltpu.VMEM((D // 2, PITCH, DH), jnp.uint32)] * 3,
                pltpu.VMEM((NSEG, SEG, D), jnp.bfloat16),
                pltpu.VMEM((M, D), jnp.bfloat16),
                pltpu.VMEM((NSEG, SEG, D), jnp.bfloat16),
                pltpu.VMEM((L, D), jnp.float32),
                pltpu.VMEM((L, H * DH), jnp.float32),
                pltpu.VMEM((L, D), jnp.float32),
                pltpu.SemaphoreType.DMA((3,)),
                pltpu.SemaphoreType.DMA((8,)),
                pltpu.SemaphoreType.DMA((2,)),
                pltpu.SemaphoreType.DMA(()),
            ],
            compiler_params=pltpu.CompilerParams(
                vmem_limit_bytes=cfg.get("vmem", 120) * 1024 * 1024, flags=cfg.get("flags")),
        )(
            A_x.reshape(P, Q, D), A_w_r.T, A_w_i.T,
            B_x.reshape(NSEG, SEG, D), B_mem0.reshape(M, D),
            B_Wq.reshape(D // 2, 2 * H, DH), B_Wk.reshape(D // 2, 2 * H, DH), B_Wv.reshape(D // 2, 2 * H, DH),
            B_Wo.reshape(H * DH, D), _F_TAB, _G_TAB,
        )
        return out.reshape(1, S, 2 * D)

    return f


pallas_concat_heads__spectral_gfnet__memory_aug_recurrent_mem_tr__prompt_kernel = make(dict(nbulk=1))
```

```python
import functools

import jax
import jax.numpy as jnp
import numpy as np
from jax.experimental import pallas as pl
from jax.experimental.pallas import tpu as pltpu

S, D = 2048, 1024
H, DH, M, SEG = 32, 128, 8, 32
L = M + SEG
NSEG = S // SEG
P, Q = 16, 128
CB = 16
NCH = Q // CB
NB = 5
PITCH = 40
RS = float(np.sqrt(0.5))
CLASSES = ((0, 4), (1, 7), (2, 6), (3, 5))

NN = (((1,), (0,)), ((), ()))
NT = (((1,), (1,)), ((), ()))


def _dot(a, b, dims=NN):
    return jax.lax.dot_general(a, b, dims, preferred_element_type=jnp.float32)


def _bf16(w):
    return pltpu.bitcast(w, jnp.bfloat16)


def _words(x):
    return pltpu.bitcast(x.astype(jnp.bfloat16), jnp.uint32)


def _radix8(x):
    t0 = x[0] + x[4]; t1 = x[0] - x[4]; t2 = x[2] + x[6]; t3 = x[2] - x[6]
    t4 = x[1] + x[5]; t5 = x[1] - x[5]; t6 = x[3] + x[7]; t7 = x[3] - x[7]
    e = t0 + t2; o = t4 + t6
    u = (t5 - t7) * RS; w = (t5 + t7) * RS
    return [e + o, e - o, t1 + u, t3 + w, t0 - t2, t4 - t6, t1 - u, t3 - w]


def _radix8_t(p):
    e = p[0] + p[1]; o = p[0] - p[1]
    t1 = p[2] + p[6]; u = (p[2] - p[6]) * RS
    t3 = p[3] + p[7]; w = (p[3] - p[7]) * RS
    t0 = e + p[4]; t2 = e - p[4]
    t4 = o + p[5]; t6 = o - p[5]
    t5 = w + u; t7 = w - u
    return [t0 + t1, t4 + t5, t2 + t3, t6 + t7, t0 - t1, t4 - t5, t2 - t3, t6 - t7]


def _radix4(ar, ai):
    s0r = ar[0] + ar[2]; s0i = ai[0] + ai[2]; d0r = ar[0] - ar[2]; d0i = ai[0] - ai[2]
    s1r = ar[1] + ar[3]; s1i = ai[1] + ai[3]; d1r = ar[1] - ar[3]; d1i = ai[1] - ai[3]
    return ([s0r + s1r, d0r + d1i, s0r - s1r, d0r - d1i],
            [s0i + s1i, d0i - d1r, s0i - s1i, d0i + d1r])


def _twiddle(r, i, e, n):
    e %= n
    if e == 0:
        return r, i
    if 8 * e % n == 0:
        o = 8 * e // n
        if o == 2:
            return i, -r
        if o == 4:
            return -r, -i
        if o == 6:
            return -i, r
        if o == 1:
            return (r + i) * RS, (i - r) * RS
        if o == 3:
            return (i - r) * RS, (r + i) * (-RS)
        if o == 5:
            return (r + i) * (-RS), (r - i) * RS
        return (r - i) * RS, (r + i) * RS
    c, s = float(np.cos(2 * np.pi * e / n)), float(-np.sin(2 * np.pi * e / n))
    return r * c - i * s, r * s + i * c


def _radix16(xr, xi):
    ur = [[None] * 4 for _ in range(4)]
    ui = [[None] * 4 for _ in range(4)]
    for n in range(4):
        pr, pi = _radix4([xr[4 * m + n] for m in range(4)], [xi[4 * m + n] for m in range(4)])
        for p in range(4):
            r, i = _twiddle(pr[p], pi[p], n * p, 16)
            ur[n][p], ui[n][p] = r, i
    yr = [None] * 16
    yi = [None] * 16
    for p in range(4):
        qr, qi = _radix4([ur[n][p] for n in range(4)], [ui[n][p] for n in range(4)])
        for q in range(4):
            yr[p + 4 * q], yi[p + 4 * q] = qr[q], qi[q]
    return yr, yi


def _pack_rows(a):
    u = np.ascontiguousarray(a, np.float32).view(np.uint32)
    u = (u + 0x7FFF + ((u >> 16) & 1)) >> 16
    return np.ascontiguousarray(u[..., 0::2, :] | (u[..., 1::2, :] << 16))


def _tables():
    r = np.array(_radix8(list(np.eye(8))))
    e = np.exp(-2j * np.pi * np.outer(np.arange(8), np.arange(8)) / 8)
    c = e @ np.linalg.inv(r)
    lane = np.arange(128)
    f = np.zeros((4, 256, 256))
    for j in range(4):
        cls = np.where(lane >= 64, CLASSES[j][1], CLASSES[j][0])
        v = 8 * (lane & 63) + cls
        ph = np.exp(-2j * np.pi * ((lane[:, None] * v[None, :]) % D) / D)
        for pp in range(2):
            z = c[cls, 2 * j + pp][None, :] * ph
            f[j, 128 * pp:128 * pp + 128, :128] = z.real
            f[j, 128 * pp:128 * pp + 128, 128:] = z.imag
    f[0, :128, 128] = c[0, 0].real * (1 - 2 * (lane % 2))
    f[0, 128:, 128] = 0
    fi = np.transpose(f, (0, 2, 1)).copy()
    fi[0, 0, :] *= 0.5
    fi[0, 128, :] *= 0.5
    g = np.zeros((2 * P, Q, Q))
    for k in range(P):
        for e in range(2):
            u = k + P * e + 2 * P * np.arange(Q // 2)
            z = np.exp(-2j * np.pi * ((u[:, None] * np.arange(Q // 2)[None, :]) % S) / S)
            g[2 * k + e] = np.block([[z.real, -z.imag], [z.imag, z.real]])
    r16 = np.arange(Q)
    order = (r16 >> 4) * 8 + (r16 & 7) + (Q // 2) * ((r16 >> 3) & 1)
    g = g[:, order][:, :, order]
    gi = np.transpose(g, (0, 2, 1)) * (2.0 / (S * D))
    return _pack_rows(np.concatenate([f, fi])), _pack_rows(np.concatenate([g, gi]))


_F_TAB, _G_TAB = _tables()


def _make_kernel(cfg):
    scope = jax.named_scope if cfg.get("scopes") else (lambda name: _Null())
    split = cfg.get("split", 16)
    HB = cfg.get("HB", 24)
    nseg = cfg.get("nseg", NSEG)
    wlag = cfg.get("wlag", 5)
    NW = 8
    WP = D // 2 // NW

    def kernel(xa_hbm, wr_hbm, wi_hbm, xb_hbm, mem0_hbm, wq_hbm, wk_hbm, wv_hbm, wo_hbm, f_hbm, g_hbm,
               out_hbm,
               wqkv, wo, stage, xb, xtail, xbulk, bk, mem0, ya, outb, h_scr, o_scr, acc_scr,
               sem_w, sem_o, sem_x, sem_out):
        w_hbm = (wq_hbm, wk_hbm, wv_hbm)

        def w_copy(i, c):
            rows = pl.ds(pl.multiple_of(c * WP, WP), WP)
            return pltpu.make_async_copy(
                w_hbm[i].bitcast(jnp.uint32).at[rows], stage[i].at[rows, pl.ds(0, H), :], sem_w.at[i * NW + c])

        def wo_copy(n):
            return pltpu.make_async_copy(
                wo_hbm.bitcast(jnp.uint32).at[:, pl.ds(pl.multiple_of(128 * n, 128), 128)], wo.at[n], sem_o.at[n])

        xb_copy = pltpu.make_async_copy(xb_hbm, xb, sem_x.at[0])
        mem_copy = pltpu.make_async_copy(mem0_hbm, mem0, sem_x.at[1])
        xtail_copy = pltpu.make_async_copy(xb_hbm.at[:, pl.ds(SEG - 8, 8), :], xtail, sem_x.at[2])
        ya_copy = pltpu.make_async_copy(ya, out_hbm.at[:, :, pl.ds(0, D)], sem_x.at[3])

        def in_order(n, start):
            def body(t, c):
                start(t)
                return c

            jax.lax.fori_loop(0, n, body, 0)

        def relayout(i, c, part=0, nparts=1):
            su = stage[i].reshape(D // 2 * PITCH, DH)
            sv = su.at[pl.ds(pl.multiple_of(c * (WP * PITCH), WP * PITCH), WP * PITCH), :]
            rows = pl.ds(pl.multiple_of(c * WP, WP), WP)
            for j in range(part * (H // 2 // nparts), (part + 1) * (H // 2 // nparts)):
                a = sv[pl.ds(j, WP, stride=PITCH), :]
                b = sv[pl.ds(H // 2 + j, WP, stride=PITCH), :]
                wqkv[i * H + 2 * j, rows, :] = (a & jnp.uint32(0xFFFF)) | (b << 16)
                wqkv[i * H + 2 * j + 1, rows, :] = (a >> 16) | (b & jnp.uint32(0xFFFF0000))

        def branch_a(xa, f_tab, g_tab, w_st, w_last, w_perm, spec, sem_a, sem_g, sem_f, sem_c):
            def xa_copy(i):
                return pltpu.make_async_copy(
                    xa_hbm.at[:, pl.ds(pl.multiple_of(CB * i, CB), CB), :], xa.at[i], sem_a.at[i])

            def f_copy(t):
                return pltpu.make_async_copy(f_hbm.at[pl.ds(4 * t, 4)], f_tab.at[pl.ds(4 * t, 4)], sem_c.at[t])

            def g_copy(t):
                return pltpu.make_async_copy(
                    g_hbm.at[pl.ds(2 * P * t, 2 * P)], g_tab.at[pl.ds(2 * P * t, 2 * P)], sem_g.at[t])

            def filt_copy(t, ub):
                src = (wr_hbm, wi_hbm)[t].at[pl.ds(0, D // 2), :].bitcast(jnp.uint32)
                return pltpu.make_async_copy(
                    src.at[:, pl.ds(pl.multiple_of(128 * ub, 128), 128)], w_st.at[t, ub], sem_f.at[t * P + ub])

            def last_copy(t):
                return pltpu.make_async_copy(
                    (wr_hbm, wi_hbm)[t].at[pl.ds(D // 2, 1), :], w_last.at[t], sem_c.at[2 + t])

            def start_filt(ub):
                filt_copy(0, ub).start()
                filt_copy(1, ub).start()

            def start_small():
                last_copy(0).start()
                last_copy(1).start()
                mem_copy.start()

            def start_all(stages):
                def start_stage(t):
                    for n, st in enumerate(stages):
                        pl.when(t == n)(st)

                in_order(len(stages), start_stage)

            start_all([
                lambda: xa_copy(0).start(),
                lambda: f_copy(0).start(),
                lambda: in_order(NCH - 1, lambda i: xa_copy(i + 1).start()),
                start_small,
                lambda: g_copy(0).start(),
                lambda: in_order(P, start_filt),
            ])

            lane0 = jax.lax.broadcasted_iota(jnp.int32, (8, 128), 1) == 0

            planes, freq = {}, {}

            def fwd_radix8(i, a):
                x = xa[i, a].astype(jnp.float32)
                planes[i, a] = _radix8([x[:, 128 * c:128 * c + 128] for c in range(8)])

            def fwd_dot(i, j):
                lhs = jnp.concatenate(
                    [jnp.concatenate(planes[i, a][2 * j:2 * j + 2], 1) for a in range(P)], 0)
                freq[i, j] = _dot(lhs, _bf16(f_tab[j]))

            def fwd_radix16(i, j):
                for hh in range(CB // 8):
                    def at(a, part):
                        return freq[i, j % 4][CB * a + 8 * hh:CB * a + 8 * hh + 8, 128 * part:128 * part + 128]
                    if j == 0:
                        xr = [at(a, 0) for a in range(P)]
                        xi = [jnp.where(lane0, 0.0, at(a, 1)) for a in range(P)]
                    elif j < 4:
                        xr = [at(a, 0) for a in range(P)]
                        xi = [at(a, 1) for a in range(P)]
                    else:
                        xr = [jnp.where(lane0, at(a, 1), 0.0) for a in range(P)]
                        xi = [jnp.zeros((8, 128), jnp.float32)] * P
                    yr, yi = _radix16(xr, xi)
                    r0 = i * CB + 8 * hh
                    for k in range(P):
                        spec[k, r0:r0 + 8, 128 * j:128 * j + 128] = _words(jnp.concatenate([yr[k], yi[k]], 0))

            with scope("a_fwd"):
                waits = cfg.get("xa_waits", (0, 1, 2, 4, 6, 8))
                for t in range(NCH + 2):
                    if t == 1:
                        f_copy(0).wait()
                    if t in waits and t < NCH:
                        for u in range(t, waits[waits.index(t) + 1]):
                            xa_copy(u).wait()
                        if t == waits[-3]:
                            g_copy(1).start()
                            f_copy(1).start()
                            xtail_copy.start()
                        if t == waits[-2]:
                            for c in range(NW):
                                w_copy(0, c).start()
                    for q in range(4):
                        if 0 <= t - 1 < NCH:
                            fwd_dot(t - 1, q)
                        if t < NCH:
                            for a in range(4 * q, 4 * q + 4):
                                fwd_radix8(t, a)
                        if 0 <= t - 2 < NCH:
                            fwd_radix16(t - 2, q)
                            if q == 0:
                                fwd_radix16(t - 2, 4)

            def filt_tile(ub, j):
                if j < 4:
                    halves = []
                    for cls in CLASSES[j]:
                        a = w_st[0, ub, pl.ds(cls // 2, 64, stride=4), :]
                        b = w_st[1, ub, pl.ds(cls // 2, 64, stride=4), :]
                        if cls % 2 == 0:
                            halves.append((a & jnp.uint32(0xFFFF)) | (b << 16))
                        else:
                            halves.append((a >> 16) | (b & jnp.uint32(0xFFFF0000)))
                    tile = jnp.concatenate(halves, 0)
                else:
                    cols = slice(128 * ub, 128 * ub + 128)
                    a = jax.lax.bitcast_convert_type(w_last[0, :, cols].astype(jnp.float32), jnp.uint32)
                    b = jax.lax.bitcast_convert_type(w_last[1, :, cols].astype(jnp.float32), jnp.uint32)
                    row = jax.lax.broadcasted_iota(jnp.int32, (128, 128), 0)
                    tile = jnp.where(row == 0, jnp.broadcast_to((a >> 16) | b, (128, 128)), jnp.uint32(0))
                t = tile.T
                for m in range(4):
                    r0 = (4 * ub + m) * PITCH
                    w_perm[j, r0:r0 + 32, :] = t[32 * m:32 * m + 32]

            def halves(k, j):
                x = _bf16(spec[k, :, 128 * j:128 * j + 128]).astype(jnp.float32)
                even, odd = [], []
                for t in range(Q // 16):
                    lr, li = x[16 * t:16 * t + 8], x[16 * t + 8:16 * t + 16]
                    hr, hi = _twiddle(x[Q + 16 * t:Q + 16 * t + 8], x[Q + 16 * t + 8:Q + 16 * t + 16], k, 2 * P)
                    even += [lr + hr, li + hi]
                    odd += [lr - hr, li - hi]
                return [jnp.concatenate(v, 0).astype(jnp.bfloat16) for v in (even, odd)]

            with scope("a_mid1"):
                last_copy(0).wait()
                last_copy(1).wait()
                g_copy(0).wait()
                for c in range(NW):
                    w_copy(1, c).start()
                wsched = cfg.get("wsched", (4, 6))
                done = 0
                for grp in range(len(wsched)):
                    tiles = []
                    for ub in range(done, done + wsched[grp]):
                        filt_copy(0, ub).wait()
                        filt_copy(1, ub).wait()
                        tiles += [(ub, j) for j in range(NB)]
                    done += wsched[grp]
                    nk = P // len(wsched)
                    items = [(k, j) for k in range(nk * grp, nk * grp + nk) for j in range(NB)]
                    rhs = halves(*items[0])
                    for n, (k, j) in enumerate(items):
                        rhs_next = halves(*items[n + 1]) if n + 1 < len(items) else None
                        for e in range(2):
                            spec[k, Q // 2 * e:Q // 2 * (e + 1), 128 * j:128 * j + 128] = _words(
                                _dot(_bf16(g_tab[2 * k + e]), rhs[e]))
                        rhs = rhs_next
                        for t in tiles[n * len(tiles) // len(items):(n + 1) * len(tiles) // len(items)]:
                            filt_tile(*t)
            with scope("a_wrest"):
                for ub in range(done, P):
                    filt_copy(0, ub).wait()
                    filt_copy(1, ub).wait()
                for c in range(NW):
                    w_copy(2, c).start()
                for ub in range(done, P):
                    for j in range(NB):
                        filt_tile(ub, j)

            def filtered(k, j):
                res = []
                for e in range(2):
                    x = _bf16(spec[k, Q // 2 * e:Q // 2 * (e + 1), 128 * j:128 * j + 128]).astype(jnp.float32)
                    w = w_perm[j, pl.ds(k + P * e, Q // 2, stride=PITCH), :]
                    wr = jax.lax.bitcast_convert_type(w << 16, jnp.float32)
                    wi = jax.lax.bitcast_convert_type(w & jnp.uint32(0xFFFF0000), jnp.float32)
                    out = []
                    for t in range(Q // 16):
                        xr, xi = x[16 * t:16 * t + 8], x[16 * t + 8:16 * t + 16]
                        a, b = wr[8 * t:8 * t + 8], wi[8 * t:8 * t + 8]
                        out += [xr * a - xi * b, xr * b + xi * a]
                    res.append(jnp.concatenate(out, 0).astype(jnp.bfloat16))
                return res

            def merge(k, j, even, odd):
                lo, hi = [], []
                for t in range(Q // 16):
                    er, ei = even[16 * t:16 * t + 8], even[16 * t + 8:16 * t + 16]
                    orr, oi = odd[16 * t:16 * t + 8], odd[16 * t + 8:16 * t + 16]
                    lo += [er + orr, ei + oi]
                    hi += list(_twiddle(er - orr, ei - oi, -k, 2 * P))
                spec[k, :, 128 * j:128 * j + 128] = _words(jnp.concatenate(lo + hi, 0))

            with scope("a_mid2"):
                g_copy(1).wait()
                for n in range(8):
                    wo_copy(n).start()
                items = [(k, j) for k in range(P) for j in range(NB)]
                y = filtered(*items[0])
                prev = None
                for n, (k, j) in enumerate(items):
                    y_next = filtered(*items[n + 1]) if n + 1 < len(items) else None
                    cur = [_dot(_bf16(g_tab[2 * P + 2 * k + e]), y[e]) for e in range(2)]
                    if prev is not None:
                        merge(*items[n - 1], *prev)
                    prev, y = cur, y_next
                merge(*items[-1], *prev)

            def inv_radix16(i, j, nyq):
                rows = {}
                for hh in range(CB // 8):
                    r0 = i * CB + 8 * hh
                    b = [_bf16(spec[k, r0:r0 + 8, 128 * j:128 * j + 128]).astype(jnp.float32) for k in range(P)]
                    zi, zr = _radix16([x[8:16] for x in b], [x[0:8] for x in b])
                    for a in range(P):
                        if j == 4:
                            nyq[a, hh] = zr[a]
                        else:
                            rows[a, hh] = jnp.concatenate(
                                [zr[a], jnp.where(lane0, nyq[a, hh], zi[a]) if j == 0 else zi[a]], 1)
                if j < 4:
                    freq[i, j] = jnp.concatenate([rows[a, hh] for a in range(P) for hh in range(CB // 8)], 0)

            def inv_dot(i, j):
                planes[i, j] = _dot(freq[i, j], _bf16(f_tab[4 + j]))

            def inv_radix8(i, a):
                y = _radix8_t([planes[i, c // 2][CB * a:CB * a + CB, 128 * (c % 2):128 * (c % 2) + 128]
                               for c in range(8)])
                for c in range(8):
                    ya[a, CB * i:CB * i + CB, 128 * c:128 * c + 128] = y[c].astype(jnp.bfloat16)

            with scope("a_inv"):
                f_copy(1).wait()
                xtail_copy.wait()
                xb_copy.start()
                rl = cfg.get("rl", (4, 6))
                for t in range(NCH + 2):
                    nyq = {}
                    if t in rl:
                        for c in range(2):
                            w_copy(0, 2 * rl.index(t) + c).wait()
                    for q in range(4):
                        if 0 <= t - 1 < NCH:
                            inv_dot(t - 1, q)
                        if t < NCH:
                            if q == 0:
                                inv_radix16(t, 4, nyq)
                            inv_radix16(t, q, nyq)
                        if 0 <= t - 2 < NCH:
                            for a in range(4 * q, 4 * q + 4):
                                inv_radix8(t - 2, a)
                        if t in rl or t - 1 in rl:
                            n = rl.index(t) * 2 if t in rl else rl.index(t - 1) * 2 + 1
                            relayout(0, n, q, 4)
                        if t == 0:
                            rows = slice(q * (NSEG // 4), (q + 1) * (NSEG // 4))
                            xbulk[q * 128:q * 128 + 128, :] = xtail[rows].astype(jnp.float32).reshape(128, D)

        pl.run_scoped(
            branch_a,
            pltpu.VMEM((NCH, P, CB, D), jnp.bfloat16),
            pltpu.VMEM((8, 128, 256), jnp.uint32),
            pltpu.VMEM((4 * P, Q // 2, Q), jnp.uint32),
            pltpu.VMEM((2, P, D // 4, 128), jnp.uint32),
            pltpu.VMEM((2, 1, S), jnp.bfloat16),
            pltpu.VMEM((NB, (S // 32 + 1) * PITCH, 128), jnp.uint32),
            pltpu.VMEM((P, Q, NB * 128), jnp.uint32),
            pltpu.SemaphoreType.DMA((NCH,)),
            pltpu.SemaphoreType.DMA((2,)),
            pltpu.SemaphoreType.DMA((2 * P,)),
            pltpu.SemaphoreType.DMA((4,)),
        )

        def branch_b():
            bq = stage[0].reshape(D // 2 * PITCH, DH)
            nb = NSEG * 8

            half = D // 2

            def interleave(dots, pieces):
                for n, d in enumerate(dots):
                    d()
                    for p in pieces[n * len(pieces) // len(dots):(n + 1) * len(pieces) // len(dots)]:
                        relayout(*p)

            def pass_a(c, carry):
                def one(hd):
                    bk[hd] = _dot(xbulk[:, :half], _bf16(wqkv[hd, :half // 2, :]))

                interleave([functools.partial(one, c * 8 + u) for u in range(8)],
                           [(0, 4 + c, u, 8) for u in range(8)])
                return carry

            def pass_b(c, carry):
                ms = cfg.get("ms_b", 2)

                def one(hd, m):
                    rows = slice(m * nb // ms, (m + 1) * nb // ms)
                    r = bk[hd, rows, :] + _dot(xbulk[rows, half:], _bf16(wqkv[hd, half // 2:, :]))
                    bq[pl.ds(pl.multiple_of(hd * nb + m * (nb // ms), nb // ms), nb // ms), :] = (
                        jax.lax.bitcast_convert_type(r, jnp.uint32))

                interleave([functools.partial(one, c * 8 + u, m) for u in range(8) for m in range(ms)],
                           [(1, 2 * c + u // 8, u % 8, 8) for u in range(16)])
                return carry

            def pass_k(c, carry):
                ms = cfg.get("ms_k", 4)

                def one(hd, m):
                    rows = slice(m * nb // ms, (m + 1) * nb // ms)
                    bk[hd, rows, :] = _dot(xbulk[rows, :], _bf16(wqkv[H + hd]))

                interleave([functools.partial(one, c * (HB // 4) + u, m) for u in range(HB // 4) for m in range(ms)],
                           [(2, 2 * c + u // 8, u % 8, 8) for u in range(16)])
                return carry

            with scope("pass_a"):
                for c in range(4, NW):
                    w_copy(0, c).wait()
                jax.lax.fori_loop(0, 4, pass_a, 0)
            with scope("pass_b"):
                for c in range(NW):
                    w_copy(1, c).wait()
                jax.lax.fori_loop(0, 4, pass_b, 0)
            with scope("pass_k"):
                for c in range(NW):
                    w_copy(2, c).wait()
                jax.lax.fori_loop(0, 4, pass_k, 0)
            for n in range(8):
                wo_copy(n).wait()
            xb_copy.wait()
            mem_copy.wait()
            ya_copy.start()

            scale = DH ** -0.5
            h_scr[0:M, :] = mem0[...].astype(jnp.float32)
            h_scr[M:L, :] = xb[0].astype(jnp.float32)
            qi = jax.lax.broadcasted_iota(jnp.int32, (L, L), 0)
            ki = jax.lax.broadcasted_iota(jnp.int32, (L, L), 1)
            mask = (qi < M) | (qi >= ki)

            def out_copy(s):
                return pltpu.make_async_copy(
                    outb.at[s],
                    out_hbm.at[s // 4, pl.ds(pl.multiple_of((s % 4) * SEG, SEG), SEG), pl.ds(D, D)], sem_out)

            def step(s, carry):
                if not cfg.get("xnext", False):
                    h_scr[M:L, :] = xb[s].astype(jnp.float32)
                qkv, sc, pp = {}, {}, {}

                def proj(i, hd):
                    w = _bf16(wqkv[i * H + hd])
                    if i == 0:
                        rest = jax.lax.bitcast_convert_type(
                            bq[pl.ds(pl.multiple_of(hd * nb + s * 8, 8), 8), :], jnp.float32)
                        return jnp.concatenate([_dot(h_scr[0:L - 8, :], w), rest], 0)
                    if i == 1 and hd < HB:
                        rest = bk[hd, pl.ds(pl.multiple_of(s * 8, 8), 8), :]
                        return jnp.concatenate([_dot(h_scr[0:L - 8, :], w), rest], 0)
                    return _dot(h_scr[...], w)

                def wo1(n):
                    acc_scr[:, 128 * n:128 * n + 128] = _dot(
                        o_scr[:, 0:split * DH], _bf16(wo[n, 0:split * DH // 2, :]))

                tail = list(range(8))
                for i in range(H + 3):
                    if i < H:
                        qkv[i] = (proj(0, i), proj(1, i).astype(jnp.bfloat16), proj(2, i).astype(jnp.bfloat16))
                    else:
                        for _ in range(3):
                            if tail:
                                wo1(tail.pop(0))
                    if 0 <= i - 1 < H:
                        sc[i - 1] = _dot(qkv[i - 1][0], qkv[i - 1][1], NT)
                    if 0 <= i - 2 < H:
                        z = jnp.where(mask, sc.pop(i - 2) * scale, -1e9)
                        e = jnp.exp(z - jnp.max(z, axis=-1, keepdims=True))
                        pp[i - 2] = e / jnp.sum(e, axis=-1, keepdims=True)
                    if 0 <= i - 3 < H:
                        o_scr[:, (i - 3) * DH:(i - 2) * DH] = _dot(pp.pop(i - 3), qkv.pop(i - 3)[2])
                if cfg.get("xnext", False):
                    h_scr[M:L, :] = xb[jnp.minimum(s + 1, NSEG - 1)].astype(jnp.float32)
                for n in range(8):
                    r = (_dot(o_scr[:, split * DH:], _bf16(wo[n, split * DH // 2:, :]))
                         + acc_scr[:, 128 * n:128 * n + 128])
                    h_scr[0:M, 128 * n:128 * n + 128] = r[0:M]
                    outb[s, :, 128 * n:128 * n + 128] = r[M:L].astype(jnp.bfloat16)
                out_copy(s).start()
                return carry

            with scope("chain"):
                jax.lax.fori_loop(0, nseg, step, 0, unroll=cfg.get("unroll", 1))

            def drain(s, carry):
                out_copy(s).wait()
                return carry

            jax.lax.fori_loop(0, nseg, drain, 0)
            ya_copy.wait()

        branch_b()

    return kernel


class _Null:
    def __enter__(self):
        return self

    def __exit__(self, *a):
        return False


def make(cfg):
    kernel = _make_kernel(cfg)

    @functools.partial(jax.jit, static_argnames=("B_seg_len",))
    def f(A_x, A_w_r, A_w_i, B_x, B_mem0, B_Wq, B_Wk, B_Wv, B_Wo, B_seg_len):
        assert B_seg_len == SEG
        any_spec = pl.BlockSpec(memory_space=pltpu.HBM)
        out = pl.pallas_call(
            kernel,
            out_shape=jax.ShapeDtypeStruct((P, Q, 2 * D), jnp.bfloat16),
            in_specs=[any_spec] * 11,
            out_specs=any_spec,
            scratch_shapes=[
                pltpu.VMEM((3 * H, D // 2, DH), jnp.uint32),
                pltpu.VMEM((8, H * DH // 2, 128), jnp.uint32),
                [pltpu.VMEM((D // 2, PITCH, DH), jnp.uint32)] * 3,
                pltpu.VMEM((NSEG, SEG, D), jnp.bfloat16),
                pltpu.VMEM((NSEG, 8, D), jnp.bfloat16),
                pltpu.VMEM((NSEG * 8, D), jnp.float32),
                pltpu.VMEM((H, NSEG * 8, DH), jnp.float32),
                pltpu.VMEM((M, D), jnp.bfloat16),
                pltpu.VMEM((P, Q, D), jnp.bfloat16),
                pltpu.VMEM((NSEG, SEG, D), jnp.bfloat16),
                pltpu.VMEM((L, D), jnp.float32),
                pltpu.VMEM((L, H * DH), jnp.float32),
                pltpu.VMEM((L, D), jnp.float32),
                pltpu.SemaphoreType.DMA((24,)),
                pltpu.SemaphoreType.DMA((8,)),
                pltpu.SemaphoreType.DMA((4,)),
                pltpu.SemaphoreType.DMA(()),
            ],
            compiler_params=pltpu.CompilerParams(
                vmem_limit_bytes=cfg.get("vmem", 120) * 1024 * 1024, flags=cfg.get("flags")),
        )(
            A_x.reshape(P, Q, D), A_w_r.T, A_w_i.T,
            B_x.reshape(NSEG, SEG, D), B_mem0.reshape(M, D),
            B_Wq.reshape(D // 2, 2 * H, DH), B_Wk.reshape(D // 2, 2 * H, DH), B_Wv.reshape(D // 2, 2 * H, DH),
            B_Wo.reshape(H * DH, D), _F_TAB, _G_TAB,
        )
        return out.reshape(1, S, 2 * D)

    return f


pallas_concat_heads__spectral_gfnet__memory_aug_recurrent_mem_tr__prompt_kernel = make(dict())
```

```python
import functools

import jax
import jax.numpy as jnp
import numpy as np
from jax.experimental import pallas as pl
from jax.experimental.pallas import tpu as pltpu

S, D = 2048, 1024
H, DH, M, SEG = 32, 128, 8, 32
L = M + SEG
NSEG = S // SEG
P, Q = 16, 128
CB = 16
NCH = Q // CB
NB = 4
PITCH = 40
FIRST = 8
RS = float(np.sqrt(0.5))
CLASSES = ((0, 4), (1, 7), (2, 6), (3, 5))

NN = (((1,), (0,)), ((), ()))
NT = (((1,), (1,)), ((), ()))


def _dot(a, b, dims=NN):
    return jax.lax.dot_general(a, b, dims, preferred_element_type=jnp.float32)


def _bf16(w):
    return pltpu.bitcast(w, jnp.bfloat16)


def _words(x):
    return pltpu.bitcast(x.astype(jnp.bfloat16), jnp.uint32)


def _radix8(x):
    t0 = x[0] + x[4]; t1 = x[0] - x[4]; t2 = x[2] + x[6]; t3 = x[2] - x[6]
    t4 = x[1] + x[5]; t5 = x[1] - x[5]; t6 = x[3] + x[7]; t7 = x[3] - x[7]
    e = t0 + t2; o = t4 + t6
    u = (t5 - t7) * RS; w = (t5 + t7) * RS
    return [e + o, e - o, t1 + u, t3 + w, t0 - t2, t4 - t6, t1 - u, t3 - w]


def _radix8_t(p):
    e = p[0] + p[1]; o = p[0] - p[1]
    t1 = p[2] + p[6]; u = (p[2] - p[6]) * RS
    t3 = p[3] + p[7]; w = (p[3] - p[7]) * RS
    t0 = e + p[4]; t2 = e - p[4]
    t4 = o + p[5]; t6 = o - p[5]
    t5 = w + u; t7 = w - u
    return [t0 + t1, t4 + t5, t2 + t3, t6 + t7, t0 - t1, t4 - t5, t2 - t3, t6 - t7]


def _radix4(ar, ai):
    s0r = ar[0] + ar[2]; s0i = ai[0] + ai[2]; d0r = ar[0] - ar[2]; d0i = ai[0] - ai[2]
    s1r = ar[1] + ar[3]; s1i = ai[1] + ai[3]; d1r = ar[1] - ar[3]; d1i = ai[1] - ai[3]
    return ([s0r + s1r, d0r + d1i, s0r - s1r, d0r - d1i],
            [s0i + s1i, d0i - d1r, s0i - s1i, d0i + d1r])


def _twiddle(r, i, e, n):
    e %= n
    if e == 0:
        return r, i
    if 8 * e % n == 0:
        o = 8 * e // n
        if o == 2:
            return i, -r
        if o == 4:
            return -r, -i
        if o == 6:
            return -i, r
        if o == 1:
            return (r + i) * RS, (i - r) * RS
        if o == 3:
            return (i - r) * RS, (r + i) * (-RS)
        if o == 5:
            return (r + i) * (-RS), (r - i) * RS
        return (r - i) * RS, (r + i) * RS
    c, s = float(np.cos(2 * np.pi * e / n)), float(-np.sin(2 * np.pi * e / n))
    return r * c - i * s, r * s + i * c


def _radix16(xr, xi):
    ur = [[None] * 4 for _ in range(4)]
    ui = [[None] * 4 for _ in range(4)]
    for n in range(4):
        pr, pi = _radix4([xr[4 * m + n] for m in range(4)], [xi[4 * m + n] for m in range(4)])
        for p in range(4):
            r, i = _twiddle(pr[p], pi[p], n * p, 16)
            ur[n][p], ui[n][p] = r, i
    yr = [None] * 16
    yi = [None] * 16
    for p in range(4):
        qr, qi = _radix4([ur[n][p] for n in range(4)], [ui[n][p] for n in range(4)])
        for q in range(4):
            yr[p + 4 * q], yi[p + 4 * q] = qr[q], qi[q]
    return yr, yi


def _pack_rows(a):
    u = np.ascontiguousarray(a, np.float32).view(np.uint32)
    u = (u + 0x7FFF + ((u >> 16) & 1)) >> 16
    return np.ascontiguousarray(u[..., 0::2, :] | (u[..., 1::2, :] << 16))


def _tables():
    r = np.array(_radix8(list(np.eye(8))))
    e = np.exp(-2j * np.pi * np.outer(np.arange(8), np.arange(8)) / 8)
    c = e @ np.linalg.inv(r)
    lane = np.arange(128)
    f = np.zeros((4, 256, 256))
    for j in range(4):
        cls = np.where(lane >= 64, CLASSES[j][1], CLASSES[j][0])
        v = 8 * (lane & 63) + cls
        ph = np.exp(-2j * np.pi * ((lane[:, None] * v[None, :]) % D) / D)
        for pp in range(2):
            z = c[cls, 2 * j + pp][None, :] * ph
            f[j, 128 * pp:128 * pp + 128, :128] = z.real
            f[j, 128 * pp:128 * pp + 128, 128:] = z.imag
    f[0, :128, 128] = c[0, 0].real * (1 - 2 * (lane % 2))
    f[0, 128:, 128] = 0
    fi = np.transpose(f, (0, 2, 1)).copy()
    fi[0, 0, :] *= 0.5
    fi[0, 128, :] *= 0.5
    r16 = np.arange(Q)
    order = (r16 >> 4) * 8 + (r16 & 7) + (Q // 2) * ((r16 >> 3) & 1)
    z = np.exp(-2j * np.pi * np.outer(np.arange(Q // 2), np.arange(Q // 2)) / (Q // 2))
    base = [np.block([[w.real, -w.imag], [w.imag, w.real]])[order][:, order] for w in (z, 1j * z)]
    res = np.array([k + P * e for k in range(P) for e in range(2)])
    col = np.exp(-2j * np.pi * np.outer(res, order % (Q // 2)) / S)
    g = np.concatenate(base + [col.real, col.imag]).astype(np.float32)
    z = np.exp(-2j * np.pi * np.outer(np.arange(Q), np.arange(Q)) / Q)
    r16 = np.arange(2 * Q)
    order = (r16 >> 4) * 8 + (r16 & 7) + Q * ((r16 >> 3) & 1)
    n = np.block([[z.real, -z.imag], [z.imag, z.real]])[order][:, order]
    outer = np.exp(-2j * np.pi * np.outer(np.arange(P), lane) / P) * (lane < P)
    twiddle = np.exp(-2j * np.pi * np.outer(np.arange(Q), lane) / S) * (lane < P)
    n_tab = np.concatenate([outer.real, outer.imag, twiddle.real, twiddle.imag]).astype(np.float32)
    f_tab = np.concatenate([f, fi * (2.0 / (S * D)), n[None], n.T[None]])
    return _pack_rows(f_tab), g, n_tab


_F_TAB, _G_TAB, _N_TAB = _tables()


def _make_kernel(cfg):
    scope = jax.named_scope if cfg.get("scopes") else (lambda name: _Null())
    split = cfg.get("split", 16)
    HB = cfg.get("HB", 24)
    nseg = cfg.get("nseg", NSEG)
    wlag = cfg.get("wlag", 5)
    NW = 8
    WP = D // 2 // NW

    def kernel(xa_hbm, wr_hbm, wi_hbm, xb_hbm, mem0_hbm, wq_hbm, wk_hbm, wv_hbm, wo_hbm, f_hbm, g_hbm, n_hbm,
               out_hbm,
               wqkv, wo, stage, xb, xtail, bk, mem0, ya, outb, h_scr, o_scr, acc_scr,
               sem_w, sem_o, sem_x, sem_out):
        w_hbm = (wq_hbm, wk_hbm, wv_hbm)

        def w_copy(i, c):
            rows = pl.ds(pl.multiple_of(c * WP, WP), WP)
            return pltpu.make_async_copy(
                w_hbm[i].bitcast(jnp.uint32).at[rows], stage[i].at[rows, pl.ds(0, H), :], sem_w.at[i * NW + c])

        def wo_copy(n):
            return pltpu.make_async_copy(
                wo_hbm.bitcast(jnp.uint32).at[:, pl.ds(pl.multiple_of(128 * n, 128), 128)], wo.at[n], sem_o.at[n])

        def xb_copy(t):
            part = pl.ds(0, FIRST) if t == 0 else pl.ds(FIRST, NSEG - FIRST)
            return pltpu.make_async_copy(xb_hbm.at[part], xb.at[part], sem_x.at[4 * t])

        mem_copy = pltpu.make_async_copy(mem0_hbm, mem0, sem_x.at[1])
        xtail_copy = pltpu.make_async_copy(xb_hbm.at[:, pl.ds(SEG - 8, 8), :], xtail, sem_x.at[2])
        ya_copy = pltpu.make_async_copy(ya, out_hbm.at[:, :, pl.ds(0, D)], sem_x.at[3])

        def in_order(n, start):
            def body(t, c):
                start(t)
                return c

            jax.lax.fori_loop(0, n, body, 0)

        def relayout(i, c, part=0, nparts=1):
            su = stage[i].reshape(D // 2 * PITCH, DH)
            sv = su.at[pl.ds(pl.multiple_of(c * (WP * PITCH), WP * PITCH), WP * PITCH), :]
            rows = pl.ds(pl.multiple_of(c * WP, WP), WP)
            for j in range(part * (H // 2 // nparts), (part + 1) * (H // 2 // nparts)):
                a = sv[pl.ds(j, WP, stride=PITCH), :]
                b = sv[pl.ds(H // 2 + j, WP, stride=PITCH), :]
                wqkv[i * H + 2 * j, rows, :] = (a & jnp.uint32(0xFFFF)) | (b << 16)
                wqkv[i * H + 2 * j + 1, rows, :] = (a >> 16) | (b & jnp.uint32(0xFFFF0000))

        def branch_a(xa, f_tab, g_src, g_tab, n_tab, nyq, w_st, w_last, w_perm, spec, x32, sem_a, sem_g, sem_f, sem_c):
            def xa_copy(i):
                return pltpu.make_async_copy(
                    xa_hbm.at[:, pl.ds(pl.multiple_of(CB * i, CB), CB), :], xa.at[i], sem_a.at[i])

            def f_copy(t):
                part = pl.ds(4 * t, 4 + 2 * t)
                return pltpu.make_async_copy(f_hbm.at[part], f_tab.at[part], sem_c.at[t])

            n_copy = pltpu.make_async_copy(n_hbm, n_tab, sem_c.at[4])

            g_copy = pltpu.make_async_copy(g_hbm, g_src, sem_g)

            def filt_copy(t, ub):
                src = (wr_hbm, wi_hbm)[t].at[pl.ds(0, D // 2), :].bitcast(jnp.uint32)
                return pltpu.make_async_copy(
                    src.at[:, pl.ds(pl.multiple_of(128 * ub, 128), 128)], w_st.at[t, ub], sem_f.at[t * P + ub])

            def last_copy(t):
                return pltpu.make_async_copy(
                    (wr_hbm, wi_hbm)[t].at[pl.ds(D // 2, 1), :], w_last.at[t], sem_c.at[2 + t])

            def start_filt(ub):
                filt_copy(0, ub).start()
                filt_copy(1, ub).start()

            def start_small():
                last_copy(0).start()
                last_copy(1).start()
                mem_copy.start()

            def start_all(stages):
                def start_stage(t):
                    for n, st in enumerate(stages):
                        pl.when(t == n)(st)

                in_order(len(stages), start_stage)

            start_all([
                g_copy.start,
                lambda: xa_copy(0).start(),
                lambda: f_copy(0).start(),
                n_copy.start,
                lambda: in_order(NCH - 1, lambda i: xa_copy(i + 1).start()),
                start_small,
                lambda: in_order(P, start_filt),
            ])

            lane0 = jax.lax.broadcasted_iota(jnp.int32, (8, 128), 1) == 0

            def inner_matrices(t, carry):
                for u in range(4):
                    n = 4 * t + u
                    m = (g_src[0:Q, :] * g_src[pl.ds(2 * Q + n, 1), :]
                         + g_src[Q:2 * Q, :] * g_src[pl.ds(2 * Q + 2 * P + n, 1), :])
                    g_tab[n] = _words(m)
                    g_tab[2 * P + n] = _words(m.T)
                return carry

            g_copy.wait()
            jax.lax.fori_loop(0, 2 * P // 4, inner_matrices, 0)

            planes, freq = {}, {}

            def forward(i, carry):
                xa_copy(i).wait()

                @pl.when(i == 0)
                def _():
                    f_copy(0).wait()
                    n_copy.wait()

                @pl.when(i == 4)
                def _():
                    f_copy(1).start()
                    xtail_copy.start()

                @pl.when(i == 6)
                def _():
                    in_order(NW, lambda c: w_copy(0, c).start())

                rows = []
                for a in range(P):
                    x = xa[i, a].astype(jnp.float32)
                    rows.append(_radix8([x[:, 128 * c:128 * c + 128] for c in range(8)]))

                def transform(j, hh):
                    lhs = jnp.concatenate(
                        [jnp.concatenate([p[8 * hh:8 * hh + 8] for p in rows[a][2 * j:2 * j + 2]], 1)
                         for a in range(P)], 0)
                    return _dot(lhs, _bf16(f_tab[j]))

                def outer(j, hh, x):
                    xr = [x[8 * a:8 * a + 8, :128] for a in range(P)]
                    xi = [x[8 * a:8 * a + 8, 128:] for a in range(P)]
                    dst = pl.ds(pl.multiple_of(i * CB + 8 * hh, 8), 8)
                    if j == 0:
                        re = im = None
                        for a in range(P):
                            t = jnp.broadcast_to(xi[a][:, 0:1], (8, 128))
                            pr, pi = t * n_tab[a:a + 1, :], t * n_tab[P + a:P + a + 1, :]
                            re, im = (pr, pi) if a == 0 else (re + pr, im + pi)
                        nyq[0, dst, :] = re
                        nyq[1, dst, :] = im
                        xi = [jnp.where(lane0, 0.0, v) for v in xi]
                    yr, yi = _radix16(xr, xi)
                    for k in range(P):
                        spec[k, dst, 128 * j:128 * j + 128] = _words(jnp.concatenate([yr[k], yi[k]], 0))

                parts = [(j, hh) for j in range(NB) for hh in range(CB // 8)]
                pending = {}
                for n in range(len(parts) + 1):
                    if n < len(parts):
                        pending[n] = transform(*parts[n])
                    if n >= 1:
                        outer(*parts[n - 1], pending.pop(n - 1))
                return carry

            with scope("a_fwd"):
                jax.lax.fori_loop(0, NCH, forward, 0)

            def filt_tile(ub, j):
                parts = []
                for cls in CLASSES[j]:
                    a = w_st[0, ub, pl.ds(cls // 2, 64, stride=4), :]
                    b = w_st[1, ub, pl.ds(cls // 2, 64, stride=4), :]
                    if cls % 2 == 0:
                        parts.append((a & jnp.uint32(0xFFFF)) | (b << 16))
                    else:
                        parts.append((a >> 16) | (b & jnp.uint32(0xFFFF0000)))
                tile = jnp.concatenate(parts, 0)
                t = tile.T
                for m in range(4):
                    r0 = (4 * ub + m) * PITCH
                    w_perm[j, r0:r0 + 32, :] = t[32 * m:32 * m + 32]

            def halves(k, j):
                x = _bf16(spec[k, :, 128 * j:128 * j + 128]).astype(jnp.float32)
                even, odd = [], []
                for t in range(Q // 16):
                    lr, li = x[16 * t:16 * t + 8], x[16 * t + 8:16 * t + 16]
                    hr, hi = _twiddle(x[Q + 16 * t:Q + 16 * t + 8], x[Q + 16 * t + 8:Q + 16 * t + 16], k, 2 * P)
                    even += [lr + hr, li + hi]
                    odd += [lr - hr, li - hi]
                return [jnp.concatenate(v, 0).astype(jnp.bfloat16) for v in (even, odd)]

            with scope("a_mid1"):
                last_copy(0).wait()
                last_copy(1).wait()
                for c in range(NW):
                    w_copy(1, c).start()
                wsched = cfg.get("wsched", (4, 6))
                done = 0
                for grp in range(len(wsched)):
                    tiles = []
                    for ub in range(done, done + wsched[grp]):
                        filt_copy(0, ub).wait()
                        filt_copy(1, ub).wait()
                        tiles += [(ub, j) for j in range(NB)]
                    done += wsched[grp]
                    nk = P // len(wsched)
                    items = [(k, j) for k in range(nk * grp, nk * grp + nk) for j in range(NB)]
                    rhs = halves(*items[0])
                    for n, (k, j) in enumerate(items):
                        rhs_next = halves(*items[n + 1]) if n + 1 < len(items) else None
                        for e in range(2):
                            x32[k, e, :, 128 * j:128 * j + 128] = _dot(_bf16(g_tab[2 * k + e]), rhs[e])
                        rhs = rhs_next
                        for t in tiles[n * len(tiles) // len(items):(n + 1) * len(tiles) // len(items)]:
                            filt_tile(*t)
            def filtered(k, j):
                res = []
                for e in range(2):
                    x = x32[k, e, :, 128 * j:128 * j + 128]
                    w = w_perm[j, pl.ds(k + P * e, Q // 2, stride=PITCH), :]
                    wr = jax.lax.bitcast_convert_type(w << 16, jnp.float32)
                    wi = jax.lax.bitcast_convert_type(w & jnp.uint32(0xFFFF0000), jnp.float32)
                    out = []
                    for t in range(Q // 16):
                        xr, xi = x[16 * t:16 * t + 8], x[16 * t + 8:16 * t + 16]
                        a, b = wr[8 * t:8 * t + 8], wi[8 * t:8 * t + 8]
                        out += [xr * a - xi * b, xr * b + xi * a]
                    res.append(jnp.concatenate(out, 0).astype(jnp.bfloat16))
                return res

            def merge(k, j, even, odd):
                lo, hi = [], []
                for t in range(Q // 16):
                    er, ei = even[16 * t:16 * t + 8], even[16 * t + 8:16 * t + 16]
                    orr, oi = odd[16 * t:16 * t + 8], odd[16 * t + 8:16 * t + 16]
                    lo += [er + orr, ei + oi]
                    hi += list(_twiddle(er - orr, ei - oi, -k, 2 * P))
                spec[k, :, 128 * j:128 * j + 128] = _words(jnp.concatenate(lo + hi, 0))

            def nyquist_column():
                row = jax.lax.broadcasted_iota(jnp.int32, (8, 128), 0)
                lane = jax.lax.broadcasted_iota(jnp.int32, (8, 128), 1)
                idx = (P * row + lane) & 127

                def twiddles(t):
                    r0 = 2 * P + 8 * t
                    return n_tab[r0:r0 + 8, :], n_tab[Q + r0:Q + r0 + 8, :]

                out = []
                for t in range(Q // 8):
                    c, s = twiddles(t)
                    re, im = nyq[0, 8 * t:8 * t + 8, :], nyq[1, 8 * t:8 * t + 8, :]
                    out += [re * c - im * s, re * s + im * c]
                x = _dot(_bf16(f_tab[8]), jnp.concatenate(out, 0).astype(jnp.bfloat16))
                out = []
                for t in range(Q // 8):
                    a, b = [
                        jnp.where(lane < P, jnp.take_along_axis(
                            jnp.broadcast_to(w_last[p, :, 128 * t:128 * t + 128].astype(jnp.float32), (8, 128)),
                            idx, axis=1, mode="promise_in_bounds"), 0.0)
                        for p in range(2)]
                    xr, xi = x[16 * t:16 * t + 8], x[16 * t + 8:16 * t + 16]
                    out += [xr * a - xi * b, xr * b + xi * a]
                y = _dot(_bf16(f_tab[9]), jnp.concatenate(out, 0).astype(jnp.bfloat16))
                for t in range(Q // 8):
                    c, s = twiddles(t)
                    re, im = y[16 * t:16 * t + 8], y[16 * t + 8:16 * t + 16]
                    nyq[0, 8 * t:8 * t + 8, :] = re * c + im * s
                    nyq[1, 8 * t:8 * t + 8, :] = im * c - re * s

            with scope("a_mid2"):
                for ub in range(done, P):
                    filt_copy(0, ub).wait()
                    filt_copy(1, ub).wait()
                for c in range(NW):
                    w_copy(2, c).start()
                for ub in range(done, P):
                    filt_tile(ub, 0)
                items = [(k, j) for j in range(NB) for k in range(P)]
                y = filtered(*items[0])
                prev = None
                for n, (k, j) in enumerate(items):
                    if j + 1 < NB and k < P - done:
                        filt_tile(done + k, j + 1)
                    y_next = filtered(*items[n + 1]) if n + 1 < len(items) else None
                    cur = [_dot(_bf16(g_tab[2 * P + 2 * k + e]), y[e]) for e in range(2)]
                    if prev is not None:
                        merge(*items[n - 1], *prev)
                    prev, y = cur, y_next
                merge(*items[-1], *prev)

            def inv_radix16(i, j, hh):
                r0 = i * CB + 8 * hh
                b = [_bf16(spec[k, r0:r0 + 8, 128 * j:128 * j + 128]).astype(jnp.float32) for k in range(P)]
                zi, zr = _radix16([x[8:16] for x in b], [x[0:8] for x in b])
                if j == 0:
                    for a in range(P):
                        z = (nyq[0, r0:r0 + 8, :] * n_tab[a:a + 1, :]
                             + nyq[1, r0:r0 + 8, :] * n_tab[P + a:P + a + 1, :])
                        zi[a] = jnp.where(lane0, jnp.sum(z, axis=1, keepdims=True), zi[a])
                freq[i, j, hh] = jnp.concatenate([jnp.concatenate([zr[a], zi[a]], 1) for a in range(P)], 0)

            def inv_dot(i, j, hh):
                planes[i, j, hh] = _dot(freq[i, j, hh], _bf16(f_tab[4 + j]))

            def inv_radix8(i, a):
                y = _radix8_t([
                    jnp.concatenate([planes[i, c // 2, hh][8 * a:8 * a + 8, 128 * (c % 2):128 * (c % 2) + 128]
                                     for hh in range(2)], 0)
                    for c in range(8)])
                for c in range(8):
                    ya[a, CB * i:CB * i + CB, 128 * c:128 * c + 128] = y[c].astype(jnp.bfloat16)

            with scope("a_inv"):
                f_copy(1).wait()
                xb_copy(0).start()
                for n in range(8):
                    wo_copy(n).start()
                nyquist_column()
                ilag = cfg.get("ilag", 2)
                rl = cfg.get("rl", (4, 6))
                for t in range(NCH + 2):
                    if t in rl:
                        for c in range(2):
                            w_copy(0, 2 * rl.index(t) + c).wait()
                        if t == rl[0]:
                            xb_copy(1).start()
                    for q in range(8):
                        n = 8 * t + q - ilag
                        if 0 <= n < 8 * NCH:
                            inv_dot(n // 8, (n % 8 // 2 + 1) % 4, n % 2)
                        if t < NCH:
                            inv_radix16(t, (q // 2 + 1) % 4, q % 2)
                        n = 8 * t + q - ilag - 8 - cfg.get("ilag8", 2)
                        if 0 <= n < 8 * NCH:
                            for a in (2 * (n % 8), 2 * (n % 8) + 1):
                                inv_radix8(n // 8, a)
                        if t in rl or t - 1 in rl:
                            n = rl.index(t) * 2 if t in rl else rl.index(t - 1) * 2 + 1
                            relayout(0, n, q, 8)

        pl.run_scoped(
            branch_a,
            pltpu.VMEM((NCH, P, CB, D), jnp.bfloat16),
            pltpu.VMEM((10, 128, 256), jnp.uint32),
            pltpu.VMEM((2 * Q + 4 * P, Q), jnp.float32),
            pltpu.VMEM((4 * P, Q // 2, Q), jnp.uint32),
            pltpu.VMEM((2 * P + 2 * Q, 128), jnp.float32),
            pltpu.VMEM((2, Q, 128), jnp.float32),
            pltpu.VMEM((2, P, D // 4, 128), jnp.uint32),
            pltpu.VMEM((2, 1, S), jnp.bfloat16),
            pltpu.VMEM((NB, (S // 32 + 1) * PITCH, 128), jnp.uint32),
            pltpu.VMEM((P, Q, NB * 128), jnp.uint32),
            pltpu.VMEM((P, 2, Q, NB * 128), jnp.float32),
            pltpu.SemaphoreType.DMA((NCH,)),
            pltpu.SemaphoreType.DMA(()),
            pltpu.SemaphoreType.DMA((2 * P,)),
            pltpu.SemaphoreType.DMA((5,)),
        )

        def branch_b():
            bq = stage[0].reshape(D // 2 * PITCH, DH)
            nb = NSEG * 8

            half = D // 2

            def tail_rows(m, ms, cols):
                n = NSEG // ms
                x = xtail[m * n:(m + 1) * n, :, cols]
                return x.reshape(n * 8, x.shape[-1])

            def interleave(dots, pieces):
                for n, d in enumerate(dots):
                    d()
                    for p in pieces[n * len(pieces) // len(dots):(n + 1) * len(pieces) // len(dots)]:
                        relayout(*p)

            def pass_a(c, carry):
                w_copy(0, 4 + c).wait()

                def one(hd):
                    bk[hd] = _dot(tail_rows(0, 1, slice(0, half)), _bf16(wqkv[hd, :half // 2, :]))

                interleave([functools.partial(one, c * 8 + u) for u in range(8)],
                           [(0, 4 + c, u, 8) for u in range(8)])
                return carry

            def pass_b(c, carry):
                ms = cfg.get("ms_b", 2)

                def one(hd, m):
                    rows = slice(m * nb // ms, (m + 1) * nb // ms)
                    r = bk[hd, rows, :] + _dot(tail_rows(m, ms, slice(half, D)), _bf16(wqkv[hd, half // 2:, :]))
                    bq[pl.ds(pl.multiple_of(hd * nb + m * (nb // ms), nb // ms), nb // ms), :] = (
                        jax.lax.bitcast_convert_type(r, jnp.uint32))

                interleave([functools.partial(one, c * 8 + u, m) for u in range(8) for m in range(ms)],
                           [(1, 2 * c + u // 8, u % 8, 8) for u in range(16)])
                return carry

            def pass_k(c, carry):
                ms = cfg.get("ms_k", 4)

                def one(hd, m):
                    rows = slice(m * nb // ms, (m + 1) * nb // ms)
                    bk[hd, rows, :] = _dot(tail_rows(m, ms, slice(0, D)), _bf16(wqkv[H + hd]))

                interleave([functools.partial(one, c * (HB // 4) + u, m) for u in range(HB // 4) for m in range(ms)],
                           [(2, 2 * c + u // 8, u % 8, 8) for u in range(16)])
                return carry

            with scope("pass_a"):
                xtail_copy.wait()
                jax.lax.fori_loop(0, 4, pass_a, 0)
            with scope("pass_b"):
                for c in range(NW):
                    w_copy(1, c).wait()
                jax.lax.fori_loop(0, 4, pass_b, 0)
            with scope("pass_k"):
                for c in range(NW):
                    w_copy(2, c).wait()
                jax.lax.fori_loop(0, 4, pass_k, 0)
            for n in range(8):
                wo_copy(n).wait()
            xb_copy(0).wait()
            mem_copy.wait()
            ya_copy.start()

            scale = DH ** -0.5
            h_scr[0:M, :] = mem0[...].astype(jnp.float32)
            h_scr[M:L, :] = xb[0].astype(jnp.float32)
            qi = jax.lax.broadcasted_iota(jnp.int32, (L, L), 0)
            ki = jax.lax.broadcasted_iota(jnp.int32, (L, L), 1)
            mask = (qi < M) | (qi >= ki)

            def out_copy(s):
                return pltpu.make_async_copy(
                    outb.at[s],
                    out_hbm.at[s >> 2, pl.ds(pl.multiple_of((s & 3) * SEG, SEG), SEG), pl.ds(D, D)], sem_out)

            def step(s, carry):
                if not cfg.get("xnext", False):
                    h_scr[M:L, :] = xb[s].astype(jnp.float32)
                qkv, sc, pp = {}, {}, {}

                def proj(i, hd):
                    w = _bf16(wqkv[i * H + hd])
                    if i == 0:
                        rest = jax.lax.bitcast_convert_type(
                            bq[pl.ds(pl.multiple_of(hd * nb + s * 8, 8), 8), :], jnp.float32)
                        return jnp.concatenate([_dot(h_scr[0:L - 8, :], w), rest], 0)
                    if i == 1 and hd < HB:
                        rest = bk[hd, pl.ds(pl.multiple_of(s * 8, 8), 8), :]
                        return jnp.concatenate([_dot(h_scr[0:L - 8, :], w), rest], 0)
                    return _dot(h_scr[...], w)

                def wo1(n):
                    acc_scr[:, 128 * n:128 * n + 128] = _dot(
                        o_scr[:, 0:split * DH], _bf16(wo[n, 0:split * DH // 2, :]))

                tail = list(range(8))
                for i in range(H + 3):
                    if i < H:
                        qkv[i] = (proj(0, i), proj(1, i).astype(jnp.bfloat16), proj(2, i).astype(jnp.bfloat16))
                    else:
                        for _ in range(3):
                            if tail:
                                wo1(tail.pop(0))
                    if 0 <= i - 1 < H:
                        sc[i - 1] = _dot(qkv[i - 1][0], qkv[i - 1][1], NT)
                    if 0 <= i - 2 < H:
                        z = jnp.where(mask, sc.pop(i - 2) * scale, -1e9)
                        e = jnp.exp(z - jnp.max(z, axis=-1, keepdims=True))
                        pp[i - 2] = e / jnp.sum(e, axis=-1, keepdims=True)
                    if 0 <= i - 3 < H:
                        o_scr[:, (i - 3) * DH:(i - 2) * DH] = _dot(pp.pop(i - 3), qkv.pop(i - 3)[2])
                if cfg.get("xnext", False):
                    h_scr[M:L, :] = xb[jnp.minimum(s + 1, NSEG - 1)].astype(jnp.float32)
                for n in range(8):
                    r = (_dot(o_scr[:, split * DH:], _bf16(wo[n, split * DH // 2:, :]))
                         + acc_scr[:, 128 * n:128 * n + 128])
                    h_scr[0:M, 128 * n:128 * n + 128] = r[0:M]
                    outb[s, :, 128 * n:128 * n + 128] = r[M:L].astype(jnp.bfloat16)
                out_copy(s).start()
                return carry

            un = cfg.get("unroll", 2)

            def steps(t, carry):
                for u in range(un):
                    step(t * un + u, carry)
                return carry

            def group(g, carry):
                jax.lax.fori_loop(g * (FIRST // un), jnp.minimum(FIRST + g * (NSEG - FIRST), nseg) // un, steps, 0)
                pl.when(g == 0)(xb_copy(1).wait)
                return carry

            with scope("chain"):
                jax.lax.fori_loop(0, 2, group, 0)

            def drain(s, carry):
                out_copy(s).wait()
                return carry

            jax.lax.fori_loop(0, nseg, drain, 0)
            ya_copy.wait()

        branch_b()

    return kernel


class _Null:
    def __enter__(self):
        return self

    def __exit__(self, *a):
        return False


def make(cfg):
    kernel = _make_kernel(cfg)

    @functools.partial(jax.jit, static_argnames=("B_seg_len",))
    def f(A_x, A_w_r, A_w_i, B_x, B_mem0, B_Wq, B_Wk, B_Wv, B_Wo, B_seg_len):
        assert B_seg_len == SEG
        any_spec = pl.BlockSpec(memory_space=pltpu.HBM)
        out = pl.pallas_call(
            kernel,
            out_shape=jax.ShapeDtypeStruct((P, Q, 2 * D), jnp.bfloat16),
            in_specs=[any_spec] * 12,
            out_specs=any_spec,
            scratch_shapes=[
                pltpu.VMEM((3 * H, D // 2, DH), jnp.uint32),
                pltpu.VMEM((8, H * DH // 2, 128), jnp.uint32),
                [pltpu.VMEM((D // 2, PITCH, DH), jnp.uint32)] * 3,
                pltpu.VMEM((NSEG, SEG, D), jnp.bfloat16),
                pltpu.VMEM((NSEG, 8, D), jnp.bfloat16),
                pltpu.VMEM((H, NSEG * 8, DH), jnp.float32),
                pltpu.VMEM((M, D), jnp.bfloat16),
                pltpu.VMEM((P, Q, D), jnp.bfloat16),
                pltpu.VMEM((NSEG, SEG, D), jnp.bfloat16),
                pltpu.VMEM((L, D), jnp.float32),
                pltpu.VMEM((L, H * DH), jnp.float32),
                pltpu.VMEM((L, D), jnp.float32),
                pltpu.SemaphoreType.DMA((24,)),
                pltpu.SemaphoreType.DMA((8,)),
                pltpu.SemaphoreType.DMA((5,)),
                pltpu.SemaphoreType.DMA(()),
            ],
            compiler_params=pltpu.CompilerParams(
                vmem_limit_bytes=cfg.get("vmem", 120) * 1024 * 1024, flags=cfg.get("flags")),
        )(
            A_x.reshape(P, Q, D), A_w_r.T, A_w_i.T,
            B_x.reshape(NSEG, SEG, D), B_mem0.reshape(M, D),
            B_Wq.reshape(D // 2, 2 * H, DH), B_Wk.reshape(D // 2, 2 * H, DH), B_Wv.reshape(D // 2, 2 * H, DH),
            B_Wo.reshape(H * DH, D), _F_TAB, _G_TAB, _N_TAB,
        )
        return out.reshape(1, S, 2 * D)

    return f


pallas_concat_heads__spectral_gfnet__memory_aug_recurrent_mem_tr__prompt_kernel = make(dict())
```

```python
import functools

import jax
import jax.numpy as jnp
import numpy as np
from jax.experimental import pallas as pl
from jax.experimental.pallas import tpu as pltpu

S, D = 2048, 1024
H, DH, M, SEG = 32, 128, 8, 32
L = M + SEG
NSEG = S // SEG

P, Q = 16, 128
CB = 16
NCH = Q // CB
NB = 4
CLASSES = ((0, 4), (1, 7), (2, 6), (3, 5))

TAIL = 8
HB = 24
NW = 8
WP = D // 2 // NW
PITCH = 40
SPLIT = 16
FIRST = 8
UNROLL = 2

RS = float(np.sqrt(0.5))
NN = (((1,), (0,)), ((), ()))
NT = (((1,), (1,)), ((), ()))


def _dot(a, b, dims=NN):
    return jax.lax.dot_general(a, b, dims, preferred_element_type=jnp.float32)


def _bf16(words):
    return pltpu.bitcast(words, jnp.bfloat16)


def _words(x):
    return pltpu.bitcast(x.astype(jnp.bfloat16), jnp.uint32)


def _low_halves(a, b):
    return (a & jnp.uint32(0xFFFF)) | (b << 16)


def _high_halves(a, b):
    return (a >> 16) | (b & jnp.uint32(0xFFFF0000))


def _aligned(start, multiple):
    return start if isinstance(start, int) else pl.multiple_of(start, multiple)


def _in_order(n, start):
    def body(t, carry):
        start(t)
        return carry

    jax.lax.fori_loop(0, n, body, 0)


def _radix8(x):
    t0 = x[0] + x[4]; t1 = x[0] - x[4]; t2 = x[2] + x[6]; t3 = x[2] - x[6]
    t4 = x[1] + x[5]; t5 = x[1] - x[5]; t6 = x[3] + x[7]; t7 = x[3] - x[7]
    e = t0 + t2; o = t4 + t6
    u = (t5 - t7) * RS; w = (t5 + t7) * RS
    return [e + o, e - o, t1 + u, t3 + w, t0 - t2, t4 - t6, t1 - u, t3 - w]


def _radix8_transposed(p):
    e = p[0] + p[1]; o = p[0] - p[1]
    t1 = p[2] + p[6]; u = (p[2] - p[6]) * RS
    t3 = p[3] + p[7]; w = (p[3] - p[7]) * RS
    t0 = e + p[4]; t2 = e - p[4]
    t4 = o + p[5]; t6 = o - p[5]
    t5 = w + u; t7 = w - u
    return [t0 + t1, t4 + t5, t2 + t3, t6 + t7, t0 - t1, t4 - t5, t2 - t3, t6 - t7]


def _radix4(ar, ai):
    s0r = ar[0] + ar[2]; s0i = ai[0] + ai[2]; d0r = ar[0] - ar[2]; d0i = ai[0] - ai[2]
    s1r = ar[1] + ar[3]; s1i = ai[1] + ai[3]; d1r = ar[1] - ar[3]; d1i = ai[1] - ai[3]
    return ([s0r + s1r, d0r + d1i, s0r - s1r, d0r - d1i],
            [s0i + s1i, d0i - d1r, s0i - s1i, d0i + d1r])


def _twiddle(r, i, e, n):
    e %= n
    if e == 0:
        return r, i
    if 8 * e % n == 0:
        octant = 8 * e // n
        if octant == 2:
            return i, -r
        if octant == 4:
            return -r, -i
        if octant == 6:
            return -i, r
        if octant == 1:
            return (r + i) * RS, (i - r) * RS
        if octant == 3:
            return (i - r) * RS, (r + i) * (-RS)
        if octant == 5:
            return (r + i) * (-RS), (r - i) * RS
        return (r - i) * RS, (r + i) * RS
    c, s = float(np.cos(2 * np.pi * e / n)), float(-np.sin(2 * np.pi * e / n))
    return r * c - i * s, r * s + i * c


def _radix16(xr, xi):
    ur = [[None] * 4 for _ in range(4)]
    ui = [[None] * 4 for _ in range(4)]
    for n in range(4):
        pr, pi = _radix4([xr[4 * m + n] for m in range(4)], [xi[4 * m + n] for m in range(4)])
        for p in range(4):
            ur[n][p], ui[n][p] = _twiddle(pr[p], pi[p], n * p, 16)
    yr = [None] * 16
    yi = [None] * 16
    for p in range(4):
        qr, qi = _radix4([ur[n][p] for n in range(4)], [ui[n][p] for n in range(4)])
        for q in range(4):
            yr[p + 4 * q], yi[p + 4 * q] = qr[q], qi[q]
    return yr, yi


def _real_form(z):
    n = z.shape[0]
    r = np.arange(2 * n)
    order = (r >> 4) * 8 + (r & 7) + n * ((r >> 3) & 1)
    return np.block([[z.real, -z.imag], [z.imag, z.real]])[order][:, order]


def _tables():
    lane = np.arange(128)
    combos = np.exp(-2j * np.pi * np.outer(np.arange(8), np.arange(8)) / 8) @ np.linalg.inv(
        np.array(_radix8(list(np.eye(8)))))
    f = np.zeros((NB, 256, 256))
    for j in range(NB):
        cls = np.where(lane >= 64, CLASSES[j][1], CLASSES[j][0])
        phase = np.exp(-2j * np.pi * (np.outer(lane, 8 * (lane & 63) + cls) % D) / D)
        for half in range(2):
            z = combos[cls, 2 * j + half][None, :] * phase
            f[j, 128 * half:128 * half + 128, :128] = z.real
            f[j, 128 * half:128 * half + 128, 128:] = z.imag
    f[0, :128, 128] = combos[0, 0].real * (1 - 2 * (lane % 2))
    f[0, 128:, 128] = 0
    f_inv = np.transpose(f, (0, 2, 1)) * (2.0 / (S * D))
    f_inv[0, 0, :] *= 0.5
    f_inv[0, 128, :] *= 0.5
    dft128 = _real_form(np.exp(-2j * np.pi * np.outer(np.arange(Q), np.arange(Q)) / Q))
    bits = np.concatenate([f, f_inv, dft128[None], dft128.T[None]]).astype(np.float32).view(np.uint32)
    bits = (bits + 0x7FFF + ((bits >> 16) & 1)) >> 16
    f_tab = np.ascontiguousarray(bits[:, 0::2, :] | (bits[:, 1::2, :] << 16))
    z = np.exp(-2j * np.pi * np.outer(np.arange(Q // 2), np.arange(Q // 2)) / (Q // 2))
    residue = np.array([k + P * e for k in range(P) for e in range(2)])
    col = np.exp(-2j * np.pi * np.outer(residue, (lane >> 4) * 8 + (lane & 7)) / S)
    g_tab = np.concatenate([_real_form(z), _real_form(1j * z), col.real, col.imag]).astype(np.float32)
    outer = np.exp(-2j * np.pi * np.outer(np.arange(P), lane) / P) * (lane < P)
    twiddle = np.exp(-2j * np.pi * np.outer(np.arange(Q), lane) / S) * (lane < P)
    n_tab = np.concatenate([outer.real, outer.imag, twiddle.real, twiddle.imag]).astype(np.float32)
    return f_tab, g_tab, n_tab


_F_TAB, _G_TAB, _N_TAB = _tables()


def _kernel(xa_hbm, wr_hbm, wi_hbm, xb_hbm, mem0_hbm, wq_hbm, wk_hbm, wv_hbm, wo_hbm, f_hbm, g_hbm, n_hbm,
            out_hbm,
            wqkv, wo, stage, xb, xtail, bk, mem0, ya, outb, h_scr, o_scr, acc_scr,
            sem_w, sem_o, sem_x, sem_out):

    def w_copy(i, c):
        rows = pl.ds(_aligned(c * WP, WP), WP)
        return pltpu.make_async_copy(
            (wq_hbm, wk_hbm, wv_hbm)[i].bitcast(jnp.uint32).at[rows], stage[i].at[rows, pl.ds(0, H), :],
            sem_w.at[i * NW + c])

    def wo_copy(n):
        return pltpu.make_async_copy(wo_hbm.bitcast(jnp.uint32).at[:, pl.ds(128 * n, 128)], wo.at[n], sem_o.at[n])

    def xb_copy(t):
        part = pl.ds(0, FIRST) if t == 0 else pl.ds(FIRST, NSEG - FIRST)
        return pltpu.make_async_copy(xb_hbm.at[part], xb.at[part], sem_x.at[4 * t])

    mem_copy = pltpu.make_async_copy(mem0_hbm, mem0, sem_x.at[1])
    xtail_copy = pltpu.make_async_copy(xb_hbm.at[:, pl.ds(SEG - TAIL, TAIL), :], xtail, sem_x.at[2])
    ya_copy = pltpu.make_async_copy(ya, out_hbm.at[:, :, pl.ds(0, D)], sem_x.at[3])

    def relayout(i, c, part):
        flat = stage[i].reshape((D // 2 + 1) * PITCH, DH)
        src = flat.at[pl.ds(_aligned(c * (WP * PITCH), WP * PITCH), (WP + 1) * PITCH), :]
        rows = pl.ds(_aligned(c * WP, WP), WP)
        for j in (2 * part, 2 * part + 1):
            a = src[pl.ds(j, WP, stride=PITCH), :]
            b = src[pl.ds(H // 2 + j, WP, stride=PITCH), :]
            wqkv[i * H + 2 * j, rows, :] = _low_halves(a, b)
            wqkv[i * H + 2 * j + 1, rows, :] = _high_halves(a, b)

    def branch_a(xa, f_tab, g_src, g_tab, n_tab, nyq, w_st, w_last, w_perm, outer_out, spec,
                 sem_a, sem_f, sem_c):
        def xa_copy(i):
            return pltpu.make_async_copy(xa_hbm.at[:, pl.ds(_aligned(CB * i, CB), CB), :], xa.at[i], sem_a.at[i])

        def f_copy(t):
            part = pl.ds(4 * t, 4 + 2 * t)
            return pltpu.make_async_copy(f_hbm.at[part], f_tab.at[part], sem_c.at[t])

        def filter_copy(t, ub):
            src = (wr_hbm, wi_hbm)[t].at[pl.ds(0, D // 2), :].bitcast(jnp.uint32)
            return pltpu.make_async_copy(
                src.at[:, pl.ds(_aligned(128 * ub, 128), 128)], w_st.at[t, ub, pl.ds(0, D // 4), :],
                sem_f.at[t * P + ub])

        def last_copy(t):
            return pltpu.make_async_copy(
                (wr_hbm, wi_hbm)[t].at[pl.ds(D // 2, 1), :], w_last.at[t], sem_c.at[2 + t])

        n_copy = pltpu.make_async_copy(n_hbm, n_tab, sem_c.at[4])
        g_copy = pltpu.make_async_copy(g_hbm, g_src, sem_c.at[5])

        def start_filter(ub):
            filter_copy(0, ub).start()
            filter_copy(1, ub).start()

        def wait_filter(ub):
            filter_copy(0, ub).wait()
            filter_copy(1, ub).wait()

        def start_small():
            last_copy(0).start()
            last_copy(1).start()
            mem_copy.start()

        first_copies = [
            g_copy.start,
            lambda: xa_copy(0).start(),
            lambda: f_copy(0).start(),
            n_copy.start,
            lambda: _in_order(NCH - 1, lambda i: xa_copy(i + 1).start()),
            start_small,
            lambda: _in_order(P, start_filter),
        ]

        def start_first(t):
            for n, start in enumerate(first_copies):
                pl.when(t == n)(start)

        _in_order(len(first_copies), start_first)

        lane0 = jax.lax.broadcasted_iota(jnp.int32, (8, 128), 1) == 0

        def inner_matrices(t, carry):
            for u in range(4):
                n = 4 * t + u
                m = (g_src[0:Q, :] * g_src[pl.ds(2 * Q + n, 1), :]
                     + g_src[Q:2 * Q, :] * g_src[pl.ds(2 * Q + 2 * P + n, 1), :])
                g_tab[n] = _words(m)
                g_tab[2 * P + n] = _words(m.T)
            return carry

        g_copy.wait()
        jax.lax.fori_loop(0, 2 * P // 4, inner_matrices, 0)

        def forward(i, carry):
            xa_copy(i).wait()

            @pl.when(i == 0)
            def _():
                f_copy(0).wait()
                n_copy.wait()

            @pl.when(i == 4)
            def _():
                f_copy(1).start()

            @pl.when(i == 5)
            def _():
                _in_order(NW // 2, lambda c: w_copy(0, c).start())

            @pl.when(i == 6)
            def _():
                xtail_copy.start()

            @pl.when(i == 7)
            def _():
                _in_order(NW // 2, lambda c: w_copy(0, NW // 2 + c).start())

            combos = []
            for a in range(P):
                x = xa[i, a].astype(jnp.float32)
                combos.append(_radix8([x[:, 128 * c:128 * c + 128] for c in range(8)]))

            def features(j, hh):
                lhs = jnp.concatenate(
                    [jnp.concatenate([p[8 * hh:8 * hh + 8] for p in combos[a][2 * j:2 * j + 2]], 1)
                     for a in range(P)], 0)
                return _dot(lhs, _bf16(f_tab[j]))

            def outer(j, hh, x):
                xr = [x[8 * a:8 * a + 8, :128] for a in range(P)]
                xi = [x[8 * a:8 * a + 8, 128:] for a in range(P)]
                rows = pl.ds(pl.multiple_of(i * CB + 8 * hh, 8), 8)
                if j == 0:
                    re = im = None
                    for a in range(P):
                        t = jnp.broadcast_to(xi[a][:, 0:1], (8, 128))
                        pr, pi = t * n_tab[a:a + 1, :], t * n_tab[P + a:P + a + 1, :]
                        re, im = (pr, pi) if a == 0 else (re + pr, im + pi)
                    nyq[0, rows, :] = re
                    nyq[1, rows, :] = im
                    xi = [jnp.where(lane0, 0.0, v) for v in xi]
                yr, yi = _radix16(xr, xi)
                for k in range(P):
                    outer_out[k, rows, 128 * j:128 * j + 128] = _words(jnp.concatenate([yr[k], yi[k]], 0))

            parts = [(j, hh) for j in range(NB) for hh in range(CB // 8)]
            pending = {}
            for n in range(len(parts) + 1):
                if n < len(parts):
                    pending[n] = features(*parts[n])
                if n >= 1:
                    outer(*parts[n - 1], pending.pop(n - 1))
            return carry

        jax.lax.fori_loop(0, NCH, forward, 0)

        def filter_tile(ub, j):
            parts = []
            for cls in CLASSES[j]:
                a = w_st[0, ub, pl.ds(cls // 2, 64, stride=4), :]
                b = w_st[1, ub, pl.ds(cls // 2, 64, stride=4), :]
                parts.append(_high_halves(a, b) if cls % 2 else _low_halves(a, b))
            t = jnp.concatenate(parts, 0).T
            for m in range(4):
                r0 = (4 * ub + m) * PITCH
                w_perm[j, r0:r0 + 32, :] = t[32 * m:32 * m + 32]

        def halves(k, j):
            x = _bf16(outer_out[k, :, 128 * j:128 * j + 128]).astype(jnp.float32)
            even, odd = [], []
            for t in range(Q // 16):
                lr, li = x[16 * t:16 * t + 8], x[16 * t + 8:16 * t + 16]
                hr, hi = _twiddle(x[Q + 16 * t:Q + 16 * t + 8], x[Q + 16 * t + 8:Q + 16 * t + 16], k, 2 * P)
                even += [lr + hr, li + hi]
                odd += [lr - hr, li - hi]
            return [jnp.concatenate(v, 0).astype(jnp.bfloat16) for v in (even, odd)]

        last_copy(0).wait()
        last_copy(1).wait()
        for c in range(NW):
            w_copy(1, c).start()
        ready = 0
        for group, count in enumerate((4, 6)):
            tiles = []
            for ub in range(ready, ready + count):
                wait_filter(ub)
                tiles += [(ub, j) for j in range(NB)]
            ready += count
            items = [(k, j) for k in range(P // 2 * group, P // 2 * (group + 1)) for j in range(NB)]
            rhs = halves(*items[0])
            for n, (k, j) in enumerate(items):
                rhs_next = halves(*items[n + 1]) if n + 1 < len(items) else None
                for e in range(2):
                    spec[k, e, :, 128 * j:128 * j + 128] = _dot(_bf16(g_tab[2 * k + e]), rhs[e])
                rhs = rhs_next
                for t in tiles[n * len(tiles) // len(items):(n + 1) * len(tiles) // len(items)]:
                    filter_tile(*t)

        def filtered(k, j):
            res = []
            for e in range(2):
                x = spec[k, e, :, 128 * j:128 * j + 128]
                w = w_perm[j, pl.ds(k + P * e, Q // 2, stride=PITCH), :]
                wr = jax.lax.bitcast_convert_type(w << 16, jnp.float32)
                wi = jax.lax.bitcast_convert_type(w & jnp.uint32(0xFFFF0000), jnp.float32)
                out = []
                for t in range(Q // 16):
                    xr, xi = x[16 * t:16 * t + 8], x[16 * t + 8:16 * t + 16]
                    a, b = wr[8 * t:8 * t + 8], wi[8 * t:8 * t + 8]
                    out += [xr * a - xi * b, xr * b + xi * a]
                res.append(jnp.concatenate(out, 0).astype(jnp.bfloat16))
            return res

        def merge(k, j, even, odd):
            lo, hi = [], []
            for t in range(Q // 16):
                er, ei = even[16 * t:16 * t + 8], even[16 * t + 8:16 * t + 16]
                dr, di = odd[16 * t:16 * t + 8], odd[16 * t + 8:16 * t + 16]
                lo += [er + dr, ei + di]
                hi += list(_twiddle(er - dr, ei - di, -k, 2 * P))
            spec[k, 0, :, 128 * j:128 * j + 128] = jnp.concatenate(lo, 0)
            spec[k, 1, :, 128 * j:128 * j + 128] = jnp.concatenate(hi, 0)

        for ub in range(ready, P):
            wait_filter(ub)
        for c in range(NW):
            w_copy(2, c).start()
        for ub in range(ready, P):
            filter_tile(ub, 0)
        items = [(k, j) for j in range(NB) for k in range(P)]
        y = filtered(*items[0])
        prev = None
        for n, (k, j) in enumerate(items):
            if j + 1 < NB and k < P - ready:
                filter_tile(ready + k, j + 1)
            y_next = filtered(*items[n + 1]) if n + 1 < len(items) else None
            cur = [_dot(_bf16(g_tab[2 * P + 2 * k + e]), y[e]) for e in range(2)]
            if prev is not None:
                merge(*items[n - 1], *prev)
            prev, y = cur, y_next
        merge(*items[-1], *prev)

        def nyquist_column():
            row = jax.lax.broadcasted_iota(jnp.int32, (8, 128), 0)
            lane = jax.lax.broadcasted_iota(jnp.int32, (8, 128), 1)
            idx = (P * row + lane) & 127

            def twiddles(t):
                r0 = 2 * P + 8 * t
                return n_tab[r0:r0 + 8, :], n_tab[Q + r0:Q + r0 + 8, :]

            out = []
            for t in range(Q // 8):
                c, s = twiddles(t)
                re, im = nyq[0, 8 * t:8 * t + 8, :], nyq[1, 8 * t:8 * t + 8, :]
                out += [re * c - im * s, re * s + im * c]
            x = _dot(_bf16(f_tab[8]), jnp.concatenate(out, 0).astype(jnp.bfloat16))
            out = []
            for t in range(Q // 8):
                a, b = [
                    jnp.where(lane < P, jnp.take_along_axis(
                        jnp.broadcast_to(w_last[p, :, 128 * t:128 * t + 128].astype(jnp.float32), (8, 128)),
                        idx, axis=1, mode="promise_in_bounds"), 0.0)
                    for p in range(2)]
                xr, xi = x[16 * t:16 * t + 8], x[16 * t + 8:16 * t + 16]
                out += [xr * a - xi * b, xr * b + xi * a]
            z = _dot(_bf16(f_tab[9]), jnp.concatenate(out, 0).astype(jnp.bfloat16))
            for t in range(Q // 8):
                c, s = twiddles(t)
                re, im = z[16 * t:16 * t + 8], z[16 * t + 8:16 * t + 16]
                nyq[0, 8 * t:8 * t + 8, :] = re * c + im * s
                nyq[1, 8 * t:8 * t + 8, :] = im * c - re * s

        freq, combos = {}, {}

        def inverse_outer(i, j, hh):
            r0 = i * CB + 8 * hh
            half, t0 = divmod(2 * r0, Q)
            b = [spec[k, half, t0:t0 + 16, 128 * j:128 * j + 128] for k in range(P)]
            zi, zr = _radix16([x[8:16] for x in b], [x[0:8] for x in b])
            if j == 0:
                for a in range(P):
                    z = (nyq[0, r0:r0 + 8, :] * n_tab[a:a + 1, :]
                         + nyq[1, r0:r0 + 8, :] * n_tab[P + a:P + a + 1, :])
                    zi[a] = jnp.where(lane0, jnp.sum(z, axis=1, keepdims=True), zi[a])
            freq[i, j, hh] = jnp.concatenate([jnp.concatenate([zr[a], zi[a]], 1) for a in range(P)], 0)

        def inverse_features(i, j, hh):
            combos[i, j, hh] = _dot(freq[i, j, hh], _bf16(f_tab[4 + j]))

        def inverse_radix8(i, a):
            out = _radix8_transposed([
                jnp.concatenate([combos[i, c // 2, hh][8 * a:8 * a + 8, 128 * (c % 2):128 * (c % 2) + 128]
                                 for hh in range(2)], 0)
                for c in range(8)])
            for c in range(8):
                ya[a, CB * i:CB * i + CB, 128 * c:128 * c + 128] = out[c].astype(jnp.bfloat16)

        f_copy(1).wait()
        xb_copy(0).start()
        for n in range(8):
            wo_copy(n).start()
        nyquist_column()
        for t in range(NCH + 2):
            if t in (4, 6):
                w_copy(0, t - 4).wait()
                w_copy(0, t - 3).wait()
            if t == 4:
                xb_copy(1).start()
            for q in range(8):
                n = 8 * t + q - 2
                if 0 <= n < 8 * NCH:
                    inverse_features(n // 8, (n % 8 // 2 + 1) % 4, n % 2)
                if t < NCH:
                    inverse_outer(t, (q // 2 + 1) % 4, q % 2)
                n = 8 * t + q - 12
                if 0 <= n < 8 * NCH:
                    inverse_radix8(n // 8, 2 * (n % 8))
                    inverse_radix8(n // 8, 2 * (n % 8) + 1)
                if 4 <= t < 8:
                    relayout(0, t - 4, q)

    pl.run_scoped(
        branch_a,
        pltpu.VMEM((NCH, P, CB, D), jnp.bfloat16),
        pltpu.VMEM(_F_TAB.shape, jnp.uint32),
        pltpu.VMEM(_G_TAB.shape, jnp.float32),
        pltpu.VMEM((4 * P, Q // 2, Q), jnp.uint32),
        pltpu.VMEM(_N_TAB.shape, jnp.float32),
        pltpu.VMEM((2, Q, 128), jnp.float32),
        pltpu.VMEM((2, P, D // 4 + 8, 128), jnp.uint32),
        pltpu.VMEM((2, 1, S), jnp.bfloat16),
        pltpu.VMEM((NB, (S // 32 + 1) * PITCH, 128), jnp.uint32),
        pltpu.VMEM((P, Q, NB * 128), jnp.uint32),
        pltpu.VMEM((P, 2, Q, NB * 128), jnp.float32),
        pltpu.SemaphoreType.DMA((NCH,)),
        pltpu.SemaphoreType.DMA((2 * P,)),
        pltpu.SemaphoreType.DMA((6,)),
    )

    bq = stage[0].reshape((D // 2 + 1) * PITCH, DH)
    nb = NSEG * TAIL

    def tail_rows(m, parts, cols):
        n = NSEG // parts
        x = xtail[m * n:(m + 1) * n, :, cols]
        return x.reshape(n * TAIL, x.shape[-1])

    def interleave(dots, pieces):
        for n, dot in enumerate(dots):
            dot()
            for piece in pieces[n * len(pieces) // len(dots):(n + 1) * len(pieces) // len(dots)]:
                relayout(*piece)

    def q_first_half(c, carry):
        w_copy(0, NW // 2 + c).wait()

        def one(hd):
            bk[hd] = _dot(tail_rows(0, 1, slice(0, D // 2)), _bf16(wqkv[hd, :D // 4, :]))

        interleave([functools.partial(one, c * 8 + u) for u in range(8)],
                   [(0, NW // 2 + c, u) for u in range(8)])
        return carry

    def q_second_half(c, carry):
        w_copy(1, 2 * c).wait()
        w_copy(1, 2 * c + 1).wait()

        def one(hd, m):
            n = nb // 2
            r = bk[hd, m * n:(m + 1) * n, :] + _dot(tail_rows(m, 2, slice(D // 2, D)), _bf16(wqkv[hd, D // 4:, :]))
            bq[pl.ds(pl.multiple_of(hd * nb + m * n, n), n), :] = jax.lax.bitcast_convert_type(r, jnp.uint32)

        interleave([functools.partial(one, c * 8 + u, m) for u in range(8) for m in range(2)],
                   [(1, 2 * c + u // 8, u % 8) for u in range(16)])
        return carry

    def k_heads(c, carry):
        w_copy(2, 2 * c).wait()
        w_copy(2, 2 * c + 1).wait()

        def one(hd, m):
            n = nb // 4
            bk[hd, m * n:(m + 1) * n, :] = _dot(tail_rows(m, 4, slice(0, D)), _bf16(wqkv[H + hd]))

        interleave([functools.partial(one, c * (HB // 4) + u, m) for u in range(HB // 4) for m in range(4)],
                   [(2, 2 * c + u // 8, u % 8) for u in range(16)])
        return carry

    xtail_copy.wait()
    jax.lax.fori_loop(0, 4, q_first_half, 0)
    jax.lax.fori_loop(0, 4, q_second_half, 0)
    jax.lax.fori_loop(0, 4, k_heads, 0)
    for n in range(8):
        wo_copy(n).wait()
    xb_copy(0).wait()
    mem_copy.wait()
    ya_copy.start()

    scale = DH ** -0.5
    h_scr[0:M, :] = mem0[...].astype(jnp.float32)
    qi = jax.lax.broadcasted_iota(jnp.int32, (L, L), 0)
    ki = jax.lax.broadcasted_iota(jnp.int32, (L, L), 1)
    mask = (qi < M) | (qi >= ki)

    def out_copy(s):
        return pltpu.make_async_copy(
            outb.at[s], out_hbm.at[s >> 2, pl.ds(pl.multiple_of((s & 3) * SEG, SEG), SEG), pl.ds(D, D)], sem_out)

    def step(s):
        h_scr[M:L, :] = xb[s].astype(jnp.float32)

        def project(i, hd):
            w = _bf16(wqkv[i * H + hd])
            if i == 0:
                head = _dot(h_scr[0:L - TAIL, :], w)
                tail = jax.lax.bitcast_convert_type(
                    bq[pl.ds(pl.multiple_of(hd * nb + s * TAIL, TAIL), TAIL), :], jnp.float32)
            elif i == 1 and hd < HB:
                head = _dot(h_scr[0:L - TAIL, :], w)
                tail = bk[hd, pl.ds(pl.multiple_of(s * TAIL, TAIL), TAIL), :]
            else:
                return _dot(h_scr[...], w)
            return jnp.concatenate([head, tail], 0)

        def output_first_part(n):
            acc_scr[:, 128 * n:128 * n + 128] = _dot(o_scr[:, 0:SPLIT * DH], _bf16(wo[n, 0:SPLIT * DH // 2, :]))

        qkv, scores, probs = {}, {}, {}
        for i in range(H + 4):
            if i < H:
                qkv[i] = (project(0, i), project(1, i).astype(jnp.bfloat16), project(2, i).astype(jnp.bfloat16))
            else:
                for n in range(3 * (i - H), min(3 * (i - H) + 3, 8)):
                    output_first_part(n)
            if 0 <= i - 1 < H:
                scores[i - 1] = _dot(qkv[i - 1][0], qkv[i - 1][1], NT)
            if 0 <= i - 2 < H:
                z = jnp.where(mask, scores.pop(i - 2) * scale, -1e9)
                e = jnp.exp(z - jnp.max(z, axis=-1, keepdims=True))
                probs[i - 2] = e / jnp.sum(e, axis=-1, keepdims=True)
            if i - 4 >= 0:
                o_scr[:, (i - 4) * DH:(i - 3) * DH] = _dot(probs.pop(i - 4), qkv.pop(i - 4)[2])
        for n in range(8):
            r = _dot(o_scr[:, SPLIT * DH:], _bf16(wo[n, SPLIT * DH // 2:, :])) + acc_scr[:, 128 * n:128 * n + 128]
            h_scr[0:M, 128 * n:128 * n + 128] = r[0:M]
            outb[s, :, 128 * n:128 * n + 128] = r[M:L].astype(jnp.bfloat16)
        out_copy(s).start()

    def steps(t, carry):
        for u in range(UNROLL):
            step(t * UNROLL + u)
        return carry

    def phase(g, carry):
        jax.lax.fori_loop(g * (FIRST // UNROLL), (FIRST + g * (NSEG - FIRST)) // UNROLL, steps, 0)
        pl.when(g == 0)(lambda: xb_copy(1).wait())
        return carry

    jax.lax.fori_loop(0, 2, phase, 0)
    _in_order(NSEG, lambda s: out_copy(s).wait())
    ya_copy.wait()


@functools.partial(jax.jit, static_argnames=("B_seg_len",))
def pallas_concat_heads__spectral_gfnet__memory_aug_recurrent_mem_tr__prompt_kernel(
    A_x, A_w_r, A_w_i, B_x, B_mem0, B_Wq, B_Wk, B_Wv, B_Wo, B_seg_len,
):
    assert A_x.shape == B_x.shape == (1, S, D) and B_mem0.shape == (1, M, D) and B_seg_len == SEG
    assert B_Wq.shape == B_Wk.shape == B_Wv.shape == (D, H, DH) and B_Wo.shape == (H, DH, D)
    hbm = pl.BlockSpec(memory_space=pltpu.HBM)
    out = pl.pallas_call(
        _kernel,
        out_shape=jax.ShapeDtypeStruct((P, Q, 2 * D), jnp.bfloat16),
        in_specs=[hbm] * 12,
        out_specs=hbm,
        scratch_shapes=[
            pltpu.VMEM((3 * H, D // 2, DH), jnp.uint32),
            pltpu.VMEM((8, H * DH // 2, 128), jnp.uint32),
            [pltpu.VMEM((D // 2 + 1, PITCH, DH), jnp.uint32)] * 3,
            pltpu.VMEM((NSEG, SEG, D), jnp.bfloat16),
            pltpu.VMEM((NSEG, TAIL, D), jnp.bfloat16),
            pltpu.VMEM((H, NSEG * TAIL, DH), jnp.float32),
            pltpu.VMEM((M, D), jnp.bfloat16),
            pltpu.VMEM((P, Q, D), jnp.bfloat16),
            pltpu.VMEM((NSEG, SEG, D), jnp.bfloat16),
            pltpu.VMEM((L, D), jnp.float32),
            pltpu.VMEM((L, H * DH), jnp.float32),
            pltpu.VMEM((L, D), jnp.float32),
            pltpu.SemaphoreType.DMA((3 * NW,)),
            pltpu.SemaphoreType.DMA((8,)),
            pltpu.SemaphoreType.DMA((5,)),
            pltpu.SemaphoreType.DMA(()),
        ],
        compiler_params=pltpu.CompilerParams(vmem_limit_bytes=120 * 1024 * 1024),
    )(
        A_x.reshape(P, Q, D), A_w_r.T, A_w_i.T,
        B_x.reshape(NSEG, SEG, D), B_mem0.reshape(M, D),
        B_Wq.reshape(D // 2, 2 * H, DH), B_Wk.reshape(D // 2, 2 * H, DH), B_Wv.reshape(D // 2, 2 * H, DH),
        B_Wo.reshape(H * DH, D), _F_TAB, _G_TAB, _N_TAB,
    )
    return out.reshape(1, S, 2 * D)
```

```python
import functools

import jax
import jax.numpy as jnp
import numpy as np
from jax.experimental import pallas as pl
from jax.experimental.pallas import tpu as pltpu

S, D = 2048, 1024
H, DH, M, SEG = 32, 128, 8, 32
L = M + SEG
NSEG = S // SEG

P, Q = 16, 128
CB = 16
NCH = Q // CB
NB = 4
CLASSES = ((0, 4), (1, 7), (2, 6), (3, 5))

TAIL = 8
HB = 24
NW = 8
WP = D // 2 // NW
PITCH = 40
SPLIT = 16
FIRST = 8
UNROLL = 2

RS = float(np.sqrt(0.5))
NN = (((1,), (0,)), ((), ()))
NT = (((1,), (1,)), ((), ()))


def _dot(a, b, dims=NN):
    return jax.lax.dot_general(a, b, dims, preferred_element_type=jnp.float32)


def _bf16(words):
    return pltpu.bitcast(words, jnp.bfloat16)


def _words(x):
    return pltpu.bitcast(x.astype(jnp.bfloat16), jnp.uint32)


def _low_halves(a, b):
    return (a & jnp.uint32(0xFFFF)) | (b << 16)


def _high_halves(a, b):
    return (a >> 16) | (b & jnp.uint32(0xFFFF0000))


def _aligned(start, multiple):
    return start if isinstance(start, int) else pl.multiple_of(start, multiple)


def _in_order(n, start):
    def body(t, carry):
        start(t)
        return carry

    jax.lax.fori_loop(0, n, body, 0)


def _radix8(x):
    t0 = x[0] + x[4]; t1 = x[0] - x[4]; t2 = x[2] + x[6]; t3 = x[2] - x[6]
    t4 = x[1] + x[5]; t5 = x[1] - x[5]; t6 = x[3] + x[7]; t7 = x[3] - x[7]
    e = t0 + t2; o = t4 + t6
    u = (t5 - t7) * RS; w = (t5 + t7) * RS
    return [e + o, e - o, t1 + u, t3 + w, t0 - t2, t4 - t6, t1 - u, t3 - w]


def _radix8_transposed(p):
    e = p[0] + p[1]; o = p[0] - p[1]
    t1 = p[2] + p[6]; u = (p[2] - p[6]) * RS
    t3 = p[3] + p[7]; w = (p[3] - p[7]) * RS
    t0 = e + p[4]; t2 = e - p[4]
    t4 = o + p[5]; t6 = o - p[5]
    t5 = w + u; t7 = w - u
    return [t0 + t1, t4 + t5, t2 + t3, t6 + t7, t0 - t1, t4 - t5, t2 - t3, t6 - t7]


def _radix4(ar, ai):
    s0r = ar[0] + ar[2]; s0i = ai[0] + ai[2]; d0r = ar[0] - ar[2]; d0i = ai[0] - ai[2]
    s1r = ar[1] + ar[3]; s1i = ai[1] + ai[3]; d1r = ar[1] - ar[3]; d1i = ai[1] - ai[3]
    return ([s0r + s1r, d0r + d1i, s0r - s1r, d0r - d1i],
            [s0i + s1i, d0i - d1r, s0i - s1i, d0i + d1r])


def _twiddle(r, i, e, n):
    e %= n
    if e == 0:
        return r, i
    if 8 * e % n == 0:
        octant = 8 * e // n
        if octant == 2:
            return i, -r
        if octant == 4:
            return -r, -i
        if octant == 6:
            return -i, r
        if octant == 1:
            return (r + i) * RS, (i - r) * RS
        if octant == 3:
            return (i - r) * RS, (r + i) * (-RS)
        if octant == 5:
            return (r + i) * (-RS), (r - i) * RS
        return (r - i) * RS, (r + i) * RS
    c, s = float(np.cos(2 * np.pi * e / n)), float(-np.sin(2 * np.pi * e / n))
    return r * c - i * s, r * s + i * c


def _radix16(xr, xi):
    ur = [[None] * 4 for _ in range(4)]
    ui = [[None] * 4 for _ in range(4)]
    for n in range(4):
        pr, pi = _radix4([xr[4 * m + n] for m in range(4)], [xi[4 * m + n] for m in range(4)])
        for p in range(4):
            ur[n][p], ui[n][p] = _twiddle(pr[p], pi[p], n * p, 16)
    yr = [None] * 16
    yi = [None] * 16
    for p in range(4):
        qr, qi = _radix4([ur[n][p] for n in range(4)], [ui[n][p] for n in range(4)])
        for q in range(4):
            yr[p + 4 * q], yi[p + 4 * q] = qr[q], qi[q]
    return yr, yi


def _real_form(z):
    n = z.shape[0]
    r = np.arange(2 * n)
    order = (r >> 4) * 8 + (r & 7) + n * ((r >> 3) & 1)
    return np.block([[z.real, -z.imag], [z.imag, z.real]])[order][:, order]


def _tables():
    lane = np.arange(128)
    combos = np.exp(-2j * np.pi * np.outer(np.arange(8), np.arange(8)) / 8) @ np.linalg.inv(
        np.array(_radix8(list(np.eye(8)))))
    f = np.zeros((NB, 256, 256))
    for j in range(NB):
        cls = np.where(lane >= 64, CLASSES[j][1], CLASSES[j][0])
        phase = np.exp(-2j * np.pi * (np.outer(lane, 8 * (lane & 63) + cls) % D) / D)
        for half in range(2):
            z = combos[cls, 2 * j + half][None, :] * phase
            f[j, 128 * half:128 * half + 128, :128] = z.real
            f[j, 128 * half:128 * half + 128, 128:] = z.imag
    f[0, :128, 128] = combos[0, 0].real * (1 - 2 * (lane % 2))
    f[0, 128:, 128] = 0
    f_inv = np.transpose(f, (0, 2, 1)) * (2.0 / (S * D))
    f_inv[0, 0, :] *= 0.5
    f_inv[0, 128, :] *= 0.5
    dft128 = _real_form(np.exp(-2j * np.pi * np.outer(np.arange(Q), np.arange(Q)) / Q))
    bits = np.concatenate([f, f_inv, dft128[None], dft128.T[None]]).astype(np.float32).view(np.uint32)
    bits = (bits + 0x7FFF + ((bits >> 16) & 1)) >> 16
    f_tab = np.ascontiguousarray(bits[:, 0::2, :] | (bits[:, 1::2, :] << 16))
    z = np.exp(-2j * np.pi * np.outer(np.arange(Q // 2), np.arange(Q // 2)) / (Q // 2))
    residue = np.array([k + P * e for k in range(P) for e in range(2)])
    col = np.exp(-2j * np.pi * np.outer(residue, (lane >> 4) * 8 + (lane & 7)) / S)
    g_tab = np.concatenate([_real_form(z), _real_form(1j * z), col.real, col.imag]).astype(np.float32)
    outer = np.exp(-2j * np.pi * np.outer(np.arange(P), lane) / P) * (lane < P)
    twiddle = np.exp(-2j * np.pi * np.outer(np.arange(Q), lane) / S) * (lane < P)
    n_tab = np.concatenate([outer.real, outer.imag, twiddle.real, twiddle.imag]).astype(np.float32)
    return f_tab, g_tab, n_tab


_F_TAB, _G_TAB, _N_TAB = _tables()


def _kernel(xa_hbm, wr_hbm, wi_hbm, xb_hbm, mem0_hbm, wq_hbm, wk_hbm, wv_hbm, wo_hbm, f_hbm, g_hbm, n_hbm,
            out_hbm,
            wqkv, wo, stage, xb, xtail, bk, mem0, ya, outb, h_scr, o_scr, acc_scr,
            sem_w, sem_o, sem_x, sem_out):

    def w_copy(i, c):
        rows = pl.ds(_aligned(c * WP, WP), WP)
        return pltpu.make_async_copy(
            (wq_hbm, wk_hbm, wv_hbm)[i].bitcast(jnp.uint32).at[rows], stage[i].at[rows, pl.ds(0, H), :],
            sem_w.at[i * NW + c])

    def wo_copy(n):
        return pltpu.make_async_copy(wo_hbm.bitcast(jnp.uint32).at[:, pl.ds(128 * n, 128)], wo.at[n], sem_o.at[n])

    def xb_copy(t):
        part = pl.ds(0, FIRST) if t == 0 else pl.ds(FIRST, NSEG - FIRST)
        return pltpu.make_async_copy(xb_hbm.at[part], xb.at[part], sem_x.at[4 * t])

    mem_copy = pltpu.make_async_copy(mem0_hbm, mem0, sem_x.at[1])
    xtail_copy = pltpu.make_async_copy(xb_hbm.at[:, pl.ds(SEG - TAIL, TAIL), :], xtail, sem_x.at[2])
    ya_copy = pltpu.make_async_copy(ya, out_hbm.at[:, :, pl.ds(0, D)], sem_x.at[3])

    def relayout(i, c, part):
        flat = stage[i].reshape((D // 2 + 4) * PITCH, DH)
        src = flat.at[pl.ds(_aligned(c * (WP * PITCH), WP * PITCH), (WP + 1) * PITCH), :]
        rows = pl.ds(_aligned(c * WP, WP), WP)
        for j in (2 * part, 2 * part + 1):
            a = src[pl.ds(j, WP, stride=PITCH), :]
            b = src[pl.ds(H // 2 + j, WP, stride=PITCH), :]
            wqkv[i * H + 2 * j, rows, :] = _low_halves(a, b)
            wqkv[i * H + 2 * j + 1, rows, :] = _high_halves(a, b)

    def branch_a(xa, f_tab, g_src, g_tab, n_tab, nyq, w_st, w_last, w_perm, outer_out, spec,
                 sem_a, sem_f, sem_c):
        def xa_copy(i):
            return pltpu.make_async_copy(xa_hbm.at[:, pl.ds(_aligned(CB * i, CB), CB), :], xa.at[i], sem_a.at[i])

        def f_copy(t):
            part = pl.ds(4 * t, 4 + 2 * t)
            return pltpu.make_async_copy(f_hbm.at[part], f_tab.at[part], sem_c.at[t])

        def filter_copy(t, ub):
            src = (wr_hbm, wi_hbm)[t].at[pl.ds(0, D // 2), :].bitcast(jnp.uint32)
            return pltpu.make_async_copy(
                src.at[:, pl.ds(_aligned(128 * ub, 128), 128)], w_st.at[t, ub, pl.ds(0, D // 4), :],
                sem_f.at[t * P + ub])

        def last_copy(t):
            return pltpu.make_async_copy(
                (wr_hbm, wi_hbm)[t].at[pl.ds(D // 2, 1), :], w_last.at[t], sem_c.at[2 + t])

        n_copy = pltpu.make_async_copy(n_hbm, n_tab, sem_c.at[4])
        g_copy = pltpu.make_async_copy(g_hbm, g_src, sem_c.at[5])

        def start_filter(ub):
            filter_copy(0, ub).start()
            filter_copy(1, ub).start()

        def wait_filter(ub):
            filter_copy(0, ub).wait()
            filter_copy(1, ub).wait()

        def start_small():
            last_copy(0).start()
            last_copy(1).start()
            mem_copy.start()

        first_copies = [
            g_copy.start,
            lambda: xa_copy(0).start(),
            lambda: f_copy(0).start(),
            n_copy.start,
            lambda: _in_order(NCH - 1, lambda i: xa_copy(i + 1).start()),
            start_small,
            lambda: _in_order(P, start_filter),
        ]

        def start_first(t):
            for n, start in enumerate(first_copies):
                pl.when(t == n)(start)

        _in_order(len(first_copies), start_first)

        lane0 = jax.lax.broadcasted_iota(jnp.int32, (8, 128), 1) == 0

        def inner_matrices(t, carry):
            for u in range(4):
                n = 4 * t + u
                m = (g_src[0:Q, :] * g_src[pl.ds(2 * Q + n, 1), :]
                     + g_src[Q:2 * Q, :] * g_src[pl.ds(2 * Q + 2 * P + n, 1), :])
                g_tab[n] = _words(m)
                g_tab[2 * P + n] = _words(m.T)
            return carry

        g_copy.wait()
        jax.lax.fori_loop(0, 2 * P // 4, inner_matrices, 0)

        def forward(i, carry):
            xa_copy(i).wait()

            @pl.when(i == 0)
            def _():
                f_copy(0).wait()
                n_copy.wait()

            @pl.when(i == 4)
            def _():
                f_copy(1).start()

            @pl.when(i == 5)
            def _():
                _in_order(NW // 2, lambda c: w_copy(0, c).start())

            @pl.when(i == 6)
            def _():
                xtail_copy.start()

            @pl.when(i == 7)
            def _():
                _in_order(NW // 2, lambda c: w_copy(0, NW // 2 + c).start())

            combos = []
            for a in range(P):
                x = xa[i, a].astype(jnp.float32)
                combos.append(_radix8([x[:, 128 * c:128 * c + 128] for c in range(8)]))

            def features(j, hh):
                lhs = jnp.concatenate(
                    [jnp.concatenate([p[8 * hh:8 * hh + 8] for p in combos[a][2 * j:2 * j + 2]], 1)
                     for a in range(P)], 0)
                return _dot(lhs, _bf16(f_tab[j]))

            def outer(j, hh, x):
                xr = [x[8 * a:8 * a + 8, :128] for a in range(P)]
                xi = [x[8 * a:8 * a + 8, 128:] for a in range(P)]
                rows = pl.ds(pl.multiple_of(i * CB + 8 * hh, 8), 8)
                if j == 0:
                    re = im = None
                    for a in range(P):
                        t = jnp.broadcast_to(xi[a][:, 0:1], (8, 128))
                        pr, pi = t * n_tab[a:a + 1, :], t * n_tab[P + a:P + a + 1, :]
                        re, im = (pr, pi) if a == 0 else (re + pr, im + pi)
                    nyq[0, rows, :] = re
                    nyq[1, rows, :] = im
                    xi = [jnp.where(lane0, 0.0, v) for v in xi]
                yr, yi = _radix16(xr, xi)
                for k in range(P):
                    outer_out[k, rows, 128 * j:128 * j + 128] = _words(jnp.concatenate([yr[k], yi[k]], 0))

            parts = [(j, hh) for j in range(NB) for hh in range(CB // 8)]
            pending = {}
            for n in range(len(parts) + 1):
                if n < len(parts):
                    pending[n] = features(*parts[n])
                if n >= 1:
                    outer(*parts[n - 1], pending.pop(n - 1))
            return carry

        jax.lax.fori_loop(0, NCH, forward, 0)

        def filter_tile(ub, j):
            parts = []
            for cls in CLASSES[j]:
                a = w_st[0, ub, pl.ds(cls // 2, 64, stride=4), :]
                b = w_st[1, ub, pl.ds(cls // 2, 64, stride=4), :]
                parts.append(_high_halves(a, b) if cls % 2 else _low_halves(a, b))
            t = jnp.concatenate(parts, 0).T
            for m in range(4):
                r0 = (4 * ub + m) * PITCH
                w_perm[j, r0:r0 + 32, :] = t[32 * m:32 * m + 32]

        def halves(k, j):
            x = _bf16(outer_out[k, :, 128 * j:128 * j + 128]).astype(jnp.float32)
            even, odd = [], []
            for t in range(Q // 16):
                lr, li = x[16 * t:16 * t + 8], x[16 * t + 8:16 * t + 16]
                hr, hi = _twiddle(x[Q + 16 * t:Q + 16 * t + 8], x[Q + 16 * t + 8:Q + 16 * t + 16], k, 2 * P)
                even += [lr + hr, li + hi]
                odd += [lr - hr, li - hi]
            return [jnp.concatenate(v, 0).astype(jnp.bfloat16) for v in (even, odd)]

        last_copy(0).wait()
        last_copy(1).wait()
        for c in range(NW):
            w_copy(1, c).start()
        ready = 0
        for group, count in enumerate((4, 6)):
            tiles = []
            for ub in range(ready, ready + count):
                wait_filter(ub)
                tiles += [(ub, j) for j in range(NB)]
            ready += count
            items = [(k, j) for k in range(P // 2 * group, P // 2 * (group + 1)) for j in range(NB)]
            rhs = halves(*items[0])
            for n, (k, j) in enumerate(items):
                rhs_next = halves(*items[n + 1]) if n + 1 < len(items) else None
                for e in range(2):
                    spec[k, e, :, 128 * j:128 * j + 128] = _dot(_bf16(g_tab[2 * k + e]), rhs[e])
                rhs = rhs_next
                for t in tiles[n * len(tiles) // len(items):(n + 1) * len(tiles) // len(items)]:
                    filter_tile(*t)

        def filtered(k, j):
            res = []
            for e in range(2):
                x = spec[k, e, :, 128 * j:128 * j + 128]
                w = w_perm[j, pl.ds(k + P * e, Q // 2, stride=PITCH), :]
                wr = jax.lax.bitcast_convert_type(w << 16, jnp.float32)
                wi = jax.lax.bitcast_convert_type(w & jnp.uint32(0xFFFF0000), jnp.float32)
                out = []
                for t in range(Q // 16):
                    xr, xi = x[16 * t:16 * t + 8], x[16 * t + 8:16 * t + 16]
                    a, b = wr[8 * t:8 * t + 8], wi[8 * t:8 * t + 8]
                    out += [xr * a - xi * b, xr * b + xi * a]
                res.append(jnp.concatenate(out, 0).astype(jnp.bfloat16))
            return res

        def merge(k, j, even, odd):
            lo, hi = [], []
            for t in range(Q // 16):
                er, ei = even[16 * t:16 * t + 8], even[16 * t + 8:16 * t + 16]
                dr, di = odd[16 * t:16 * t + 8], odd[16 * t + 8:16 * t + 16]
                lo += [er + dr, ei + di]
                hi += list(_twiddle(er - dr, ei - di, -k, 2 * P))
            spec[k, 0, :, 128 * j:128 * j + 128] = jnp.concatenate(lo, 0)
            spec[k, 1, :, 128 * j:128 * j + 128] = jnp.concatenate(hi, 0)

        for ub in range(ready, P):
            wait_filter(ub)
        for c in range(NW):
            w_copy(2, c).start()
        for ub in range(ready, P):
            filter_tile(ub, 0)
        items = [(k, j) for j in range(NB) for k in range(P)]
        y = filtered(*items[0])
        prev = None
        for n, (k, j) in enumerate(items):
            if j + 1 < NB and k < P - ready:
                filter_tile(ready + k, j + 1)
            y_next = filtered(*items[n + 1]) if n + 1 < len(items) else None
            cur = [_dot(_bf16(g_tab[2 * P + 2 * k + e]), y[e]) for e in range(2)]
            if prev is not None:
                merge(*items[n - 1], *prev)
            prev, y = cur, y_next
        merge(*items[-1], *prev)

        def nyquist_column():
            row = jax.lax.broadcasted_iota(jnp.int32, (8, 128), 0)
            lane = jax.lax.broadcasted_iota(jnp.int32, (8, 128), 1)
            idx = (P * row + lane) & 127

            def twiddles(t):
                r0 = 2 * P + 8 * t
                return n_tab[r0:r0 + 8, :], n_tab[Q + r0:Q + r0 + 8, :]

            out = []
            for t in range(Q // 8):
                c, s = twiddles(t)
                re, im = nyq[0, 8 * t:8 * t + 8, :], nyq[1, 8 * t:8 * t + 8, :]
                out += [re * c - im * s, re * s + im * c]
            x = _dot(_bf16(f_tab[8]), jnp.concatenate(out, 0).astype(jnp.bfloat16))
            out = []
            for t in range(Q // 8):
                a, b = [
                    jnp.where(lane < P, jnp.take_along_axis(
                        jnp.broadcast_to(w_last[p, :, 128 * t:128 * t + 128].astype(jnp.float32), (8, 128)),
                        idx, axis=1, mode="promise_in_bounds"), 0.0)
                    for p in range(2)]
                xr, xi = x[16 * t:16 * t + 8], x[16 * t + 8:16 * t + 16]
                out += [xr * a - xi * b, xr * b + xi * a]
            z = _dot(_bf16(f_tab[9]), jnp.concatenate(out, 0).astype(jnp.bfloat16))
            for t in range(Q // 8):
                c, s = twiddles(t)
                re, im = z[16 * t:16 * t + 8], z[16 * t + 8:16 * t + 16]
                nyq[0, 8 * t:8 * t + 8, :] = re * c + im * s
                nyq[1, 8 * t:8 * t + 8, :] = im * c - re * s

        freq, combos = {}, {}

        def inverse_outer(i, j, hh):
            r0 = i * CB + 8 * hh
            half, t0 = divmod(2 * r0, Q)
            b = [spec[k, half, t0:t0 + 16, 128 * j:128 * j + 128] for k in range(P)]
            zi, zr = _radix16([x[8:16] for x in b], [x[0:8] for x in b])
            if j == 0:
                for a in range(P):
                    z = (nyq[0, r0:r0 + 8, :] * n_tab[a:a + 1, :]
                         + nyq[1, r0:r0 + 8, :] * n_tab[P + a:P + a + 1, :])
                    zi[a] = jnp.where(lane0, jnp.sum(z, axis=1, keepdims=True), zi[a])
            freq[i, j, hh] = jnp.concatenate([jnp.concatenate([zr[a], zi[a]], 1) for a in range(P)], 0)

        def inverse_features(i, j, hh):
            combos[i, j, hh] = _dot(freq[i, j, hh], _bf16(f_tab[4 + j]))

        def inverse_radix8(i, a):
            out = _radix8_transposed([
                jnp.concatenate([combos[i, c // 2, hh][8 * a:8 * a + 8, 128 * (c % 2):128 * (c % 2) + 128]
                                 for hh in range(2)], 0)
                for c in range(8)])
            for c in range(8):
                ya[a, CB * i:CB * i + CB, 128 * c:128 * c + 128] = out[c].astype(jnp.bfloat16)

        f_copy(1).wait()
        xb_copy(0).start()
        for n in range(8):
            wo_copy(n).start()
        nyquist_column()
        for t in range(NCH + 2):
            if t in (4, 6):
                w_copy(0, t - 4).wait()
                w_copy(0, t - 3).wait()
            if t == 4:
                xb_copy(1).start()
            for q in range(8):
                n = 8 * t + q - 2
                if 0 <= n < 8 * NCH:
                    inverse_features(n // 8, (n % 8 // 2 + 1) % 4, n % 2)
                if t < NCH:
                    inverse_outer(t, (q // 2 + 1) % 4, q % 2)
                n = 8 * t + q - 12
                if 0 <= n < 8 * NCH:
                    inverse_radix8(n // 8, 2 * (n % 8))
                    inverse_radix8(n // 8, 2 * (n % 8) + 1)
                if 4 <= t < 8:
                    relayout(0, t - 4, q)

    pl.run_scoped(
        branch_a,
        pltpu.VMEM((NCH, P, CB, D), jnp.bfloat16),
        pltpu.VMEM(_F_TAB.shape, jnp.uint32),
        pltpu.VMEM(_G_TAB.shape, jnp.float32),
        pltpu.VMEM((4 * P, Q // 2, Q), jnp.uint32),
        pltpu.VMEM(_N_TAB.shape, jnp.float32),
        pltpu.VMEM((2, Q, 128), jnp.float32),
        pltpu.VMEM((2, P, D // 4 + 32, 128), jnp.uint32),
        pltpu.VMEM((2, 1, S), jnp.bfloat16),
        pltpu.VMEM((NB, (S // 32 + 1) * PITCH, 128), jnp.uint32),
        pltpu.VMEM((P, Q, NB * 128), jnp.uint32),
        pltpu.VMEM((P, 2, Q, NB * 128), jnp.float32),
        pltpu.SemaphoreType.DMA((NCH,)),
        pltpu.SemaphoreType.DMA((2 * P,)),
        pltpu.SemaphoreType.DMA((6,)),
    )

    bq = stage[0].reshape((D // 2 + 4) * PITCH, DH)
    nb = NSEG * TAIL

    def tail_rows(m, parts, cols):
        n = NSEG // parts
        x = xtail[m * n:(m + 1) * n, :, cols]
        return x.reshape(n * TAIL, x.shape[-1])

    def interleave(dots, pieces):
        for n, dot in enumerate(dots):
            dot()
            for piece in pieces[n * len(pieces) // len(dots):(n + 1) * len(pieces) // len(dots)]:
                relayout(*piece)

    def q_first_half(c, carry):
        w_copy(0, NW // 2 + c).wait()

        def one(hd):
            bk[hd] = _dot(tail_rows(0, 1, slice(0, D // 2)), _bf16(wqkv[hd, :D // 4, :]))

        interleave([functools.partial(one, c * 8 + u) for u in range(8)],
                   [(0, NW // 2 + c, u) for u in range(8)])
        return carry

    def q_second_half(c, carry):
        w_copy(1, 2 * c).wait()
        w_copy(1, 2 * c + 1).wait()

        def one(hd, m):
            n = nb // 2
            r = bk[hd, m * n:(m + 1) * n, :] + _dot(tail_rows(m, 2, slice(D // 2, D)), _bf16(wqkv[hd, D // 4:, :]))
            bq[pl.ds(pl.multiple_of(hd * nb + m * n, n), n), :] = jax.lax.bitcast_convert_type(r, jnp.uint32)

        interleave([functools.partial(one, c * 8 + u, m) for u in range(8) for m in range(2)],
                   [(1, 2 * c + u // 8, u % 8) for u in range(16)])
        return carry

    def k_heads(c, carry):
        w_copy(2, 2 * c).wait()
        w_copy(2, 2 * c + 1).wait()

        def one(hd, m):
            n = nb // 4
            bk[hd, m * n:(m + 1) * n, :] = _dot(tail_rows(m, 4, slice(0, D)), _bf16(wqkv[H + hd]))

        interleave([functools.partial(one, c * (HB // 4) + u, m) for u in range(HB // 4) for m in range(4)],
                   [(2, 2 * c + u // 8, u % 8) for u in range(16)])
        return carry

    xtail_copy.wait()
    jax.lax.fori_loop(0, 4, q_first_half, 0)
    jax.lax.fori_loop(0, 4, q_second_half, 0)
    jax.lax.fori_loop(0, 4, k_heads, 0)
    for n in range(8):
        wo_copy(n).wait()
    xb_copy(0).wait()
    mem_copy.wait()
    ya_copy.start()

    scale = DH ** -0.5
    h_scr[0:M, :] = mem0[...].astype(jnp.float32)
    qi = jax.lax.broadcasted_iota(jnp.int32, (L, L), 0)
    ki = jax.lax.broadcasted_iota(jnp.int32, (L, L), 1)
    mask = (qi < M) | (qi >= ki)

    def out_copy(s):
        return pltpu.make_async_copy(
            outb.at[s], out_hbm.at[s >> 2, pl.ds(pl.multiple_of((s & 3) * SEG, SEG), SEG), pl.ds(D, D)], sem_out)

    def step(s):
        h_scr[M:L, :] = xb[s].astype(jnp.float32)

        def project(i, hd):
            w = _bf16(wqkv[i * H + hd])
            if i == 0:
                head = _dot(h_scr[0:L - TAIL, :], w)
                tail = jax.lax.bitcast_convert_type(
                    bq[pl.ds(pl.multiple_of(hd * nb + s * TAIL, TAIL), TAIL), :], jnp.float32)
            elif i == 1 and hd < HB:
                head = _dot(h_scr[0:L - TAIL, :], w)
                tail = bk[hd, pl.ds(pl.multiple_of(s * TAIL, TAIL), TAIL), :]
            else:
                return _dot(h_scr[...], w)
            return jnp.concatenate([head, tail], 0)

        def output_first_part(n):
            acc_scr[:, 128 * n:128 * n + 128] = _dot(o_scr[:, 0:SPLIT * DH], _bf16(wo[n, 0:SPLIT * DH // 2, :]))

        qkv, scores, probs = {}, {}, {}
        for i in range(H + 4):
            if i < H:
                qkv[i] = (project(0, i), project(1, i).astype(jnp.bfloat16), project(2, i).astype(jnp.bfloat16))
            else:
                for n in range(3 * (i - H), min(3 * (i - H) + 3, 8)):
                    output_first_part(n)
            if 0 <= i - 1 < H:
                scores[i - 1] = _dot(qkv[i - 1][0], qkv[i - 1][1], NT)
            if 0 <= i - 2 < H:
                z = jnp.where(mask, scores.pop(i - 2) * scale, -1e9)
                e = jnp.exp(z - jnp.max(z, axis=-1, keepdims=True))
                probs[i - 2] = e / jnp.sum(e, axis=-1, keepdims=True)
            if i - 4 >= 0:
                o_scr[:, (i - 4) * DH:(i - 3) * DH] = _dot(probs.pop(i - 4), qkv.pop(i - 4)[2])
        for n in range(8):
            r = _dot(o_scr[:, SPLIT * DH:], _bf16(wo[n, SPLIT * DH // 2:, :])) + acc_scr[:, 128 * n:128 * n + 128]
            h_scr[0:M, 128 * n:128 * n + 128] = r[0:M]
            outb[s, :, 128 * n:128 * n + 128] = r[M:L].astype(jnp.bfloat16)
        out_copy(s).start()

    def steps(t, carry):
        for u in range(UNROLL):
            step(t * UNROLL + u)
        return carry

    def phase(g, carry):
        jax.lax.fori_loop(g * (FIRST // UNROLL), (FIRST + g * (NSEG - FIRST)) // UNROLL, steps, 0)
        pl.when(g == 0)(lambda: xb_copy(1).wait())
        return carry

    jax.lax.fori_loop(0, 2, phase, 0)
    _in_order(NSEG, lambda s: out_copy(s).wait())
    ya_copy.wait()


@functools.partial(jax.jit, static_argnames=("B_seg_len",))
def pallas_concat_heads__spectral_gfnet__memory_aug_recurrent_mem_tr__prompt_kernel(
    A_x, A_w_r, A_w_i, B_x, B_mem0, B_Wq, B_Wk, B_Wv, B_Wo, B_seg_len,
):
    assert A_x.shape == B_x.shape == (1, S, D) and B_mem0.shape == (1, M, D) and B_seg_len == SEG
    assert B_Wq.shape == B_Wk.shape == B_Wv.shape == (D, H, DH) and B_Wo.shape == (H, DH, D)
    hbm = pl.BlockSpec(memory_space=pltpu.HBM)
    out = pl.pallas_call(
        _kernel,
        out_shape=jax.ShapeDtypeStruct((P, Q, 2 * D), jnp.bfloat16),
        in_specs=[hbm] * 12,
        out_specs=hbm,
        scratch_shapes=[
            pltpu.VMEM((3 * H, D // 2, DH), jnp.uint32),
            pltpu.VMEM((8, H * DH // 2, 128), jnp.uint32),
            [pltpu.VMEM((D // 2 + 4, PITCH, DH), jnp.uint32)] * 3,
            pltpu.VMEM((NSEG, SEG, D), jnp.bfloat16),
            pltpu.VMEM((NSEG, TAIL, D), jnp.bfloat16),
            pltpu.VMEM((H, NSEG * TAIL, DH), jnp.float32),
            pltpu.VMEM((M, D), jnp.bfloat16),
            pltpu.VMEM((P, Q, D), jnp.bfloat16),
            pltpu.VMEM((NSEG, SEG, D), jnp.bfloat16),
            pltpu.VMEM((L, D), jnp.float32),
            pltpu.VMEM((L, H * DH), jnp.float32),
            pltpu.VMEM((L, D), jnp.float32),
            pltpu.SemaphoreType.DMA((3 * NW,)),
            pltpu.SemaphoreType.DMA((8,)),
            pltpu.SemaphoreType.DMA((5,)),
            pltpu.SemaphoreType.DMA(()),
        ],
        compiler_params=pltpu.CompilerParams(vmem_limit_bytes=120 * 1024 * 1024),
    )(
        A_x.reshape(P, Q, D), A_w_r.T, A_w_i.T,
        B_x.reshape(NSEG, SEG, D), B_mem0.reshape(M, D),
        B_Wq.reshape(D // 2, 2 * H, DH), B_Wk.reshape(D // 2, 2 * H, DH), B_Wv.reshape(D // 2, 2 * H, DH),
        B_Wo.reshape(H * DH, D), _F_TAB, _G_TAB, _N_TAB,
    )
    return out.reshape(1, S, 2 * D)
```

```python
import functools

import jax
import jax.numpy as jnp
import numpy as np
from jax.experimental import pallas as pl
from jax.experimental.pallas import tpu as pltpu

S, D = 2048, 1024
H, DH, M, SEG = 32, 128, 8, 32
L = M + SEG
NSEG = S // SEG

P, Q = 16, 128
CB = 16
NCH = Q // CB
NB = 4
CLASSES = ((0, 4), (1, 7), (2, 6), (3, 5))

TAIL = 8
HB = 24
NW = 8
WP = D // 2 // NW
PITCH = 40
SPLIT = 16
FIRST = 8
UNROLL = 2

RS = float(np.sqrt(0.5))
NN = (((1,), (0,)), ((), ()))
NT = (((1,), (1,)), ((), ()))


def _dot(a, b, dims=NN):
    return jax.lax.dot_general(a, b, dims, preferred_element_type=jnp.float32)


def _bf16(words):
    return pltpu.bitcast(words, jnp.bfloat16)


def _words(x):
    return pltpu.bitcast(x.astype(jnp.bfloat16), jnp.uint32)


def _low_halves(a, b):
    return (a & jnp.uint32(0xFFFF)) | (b << 16)


def _high_halves(a, b):
    return (a >> 16) | (b & jnp.uint32(0xFFFF0000))


def _aligned(start, multiple):
    return start if isinstance(start, int) else pl.multiple_of(start, multiple)


def _in_order(n, start):
    def body(t, carry):
        start(t)
        return carry

    jax.lax.fori_loop(0, n, body, 0)


def _radix8(x):
    t0 = x[0] + x[4]; t1 = x[0] - x[4]; t2 = x[2] + x[6]; t3 = x[2] - x[6]
    t4 = x[1] + x[5]; t5 = x[1] - x[5]; t6 = x[3] + x[7]; t7 = x[3] - x[7]
    e = t0 + t2; o = t4 + t6
    u = (t5 - t7) * RS; w = (t5 + t7) * RS
    return [e + o, e - o, t1 + u, t3 + w, t0 - t2, t4 - t6, t1 - u, t3 - w]


def _radix8_transposed(p):
    e = p[0] + p[1]; o = p[0] - p[1]
    t1 = p[2] + p[6]; u = (p[2] - p[6]) * RS
    t3 = p[3] + p[7]; w = (p[3] - p[7]) * RS
    t0 = e + p[4]; t2 = e - p[4]
    t4 = o + p[5]; t6 = o - p[5]
    t5 = w + u; t7 = w - u
    return [t0 + t1, t4 + t5, t2 + t3, t6 + t7, t0 - t1, t4 - t5, t2 - t3, t6 - t7]


def _radix4(ar, ai):
    s0r = ar[0] + ar[2]; s0i = ai[0] + ai[2]; d0r = ar[0] - ar[2]; d0i = ai[0] - ai[2]
    s1r = ar[1] + ar[3]; s1i = ai[1] + ai[3]; d1r = ar[1] - ar[3]; d1i = ai[1] - ai[3]
    return ([s0r + s1r, d0r + d1i, s0r - s1r, d0r - d1i],
            [s0i + s1i, d0i - d1r, s0i - s1i, d0i + d1r])


def _twiddle(r, i, e, n):
    e %= n
    if e == 0:
        return r, i
    if 8 * e % n == 0:
        octant = 8 * e // n
        if octant == 2:
            return i, -r
        if octant == 4:
            return -r, -i
        if octant == 6:
            return -i, r
        if octant == 1:
            return (r + i) * RS, (i - r) * RS
        if octant == 3:
            return (i - r) * RS, (r + i) * (-RS)
        if octant == 5:
            return (r + i) * (-RS), (r - i) * RS
        return (r - i) * RS, (r + i) * RS
    c, s = float(np.cos(2 * np.pi * e / n)), float(-np.sin(2 * np.pi * e / n))
    return r * c - i * s, r * s + i * c


def _radix16(xr, xi):
    ur = [[None] * 4 for _ in range(4)]
    ui = [[None] * 4 for _ in range(4)]
    for n in range(4):
        pr, pi = _radix4([xr[4 * m + n] for m in range(4)], [xi[4 * m + n] for m in range(4)])
        for p in range(4):
            ur[n][p], ui[n][p] = _twiddle(pr[p], pi[p], n * p, 16)
    yr = [None] * 16
    yi = [None] * 16
    for p in range(4):
        qr, qi = _radix4([ur[n][p] for n in range(4)], [ui[n][p] for n in range(4)])
        for q in range(4):
            yr[p + 4 * q], yi[p + 4 * q] = qr[q], qi[q]
    return yr, yi


def _real_form(z):
    n = z.shape[0]
    r = np.arange(2 * n)
    order = (r >> 4) * 8 + (r & 7) + n * ((r >> 3) & 1)
    return np.block([[z.real, -z.imag], [z.imag, z.real]])[order][:, order]


def _tables():
    lane = np.arange(128)
    combos = np.exp(-2j * np.pi * np.outer(np.arange(8), np.arange(8)) / 8) @ np.linalg.inv(
        np.array(_radix8(list(np.eye(8)))))
    f = np.zeros((NB, 256, 256))
    for j in range(NB):
        cls = np.where(lane >= 64, CLASSES[j][1], CLASSES[j][0])
        phase = np.exp(-2j * np.pi * (np.outer(lane, 8 * (lane & 63) + cls) % D) / D)
        for half in range(2):
            z = combos[cls, 2 * j + half][None, :] * phase
            f[j, 128 * half:128 * half + 128, :128] = z.real
            f[j, 128 * half:128 * half + 128, 128:] = z.imag
    f[0, :128, 128] = combos[0, 0].real * (1 - 2 * (lane % 2))
    f[0, 128:, 128] = 0
    f_inv = np.transpose(f, (0, 2, 1)) * (2.0 / (S * D))
    f_inv[0, 0, :] *= 0.5
    f_inv[0, 128, :] *= 0.5
    dft128 = _real_form(np.exp(-2j * np.pi * np.outer(np.arange(Q), np.arange(Q)) / Q))
    bits = np.concatenate([f, f_inv, dft128[None], dft128.T[None]]).astype(np.float32).view(np.uint32)
    bits = (bits + 0x7FFF + ((bits >> 16) & 1)) >> 16
    f_tab = np.ascontiguousarray(bits[:, 0::2, :] | (bits[:, 1::2, :] << 16))
    z = np.exp(-2j * np.pi * np.outer(np.arange(Q // 2), np.arange(Q // 2)) / (Q // 2))
    residue = np.array([k + P * e for k in range(P) for e in range(2)])
    col = np.exp(-2j * np.pi * np.outer(residue, (lane >> 4) * 8 + (lane & 7)) / S)
    g_tab = np.concatenate([_real_form(z), _real_form(1j * z), col.real, col.imag]).astype(np.float32)
    outer = np.exp(-2j * np.pi * np.outer(np.arange(P), lane) / P) * (lane < P)
    twiddle = np.exp(-2j * np.pi * np.outer(np.arange(Q), lane) / S) * (lane < P)
    n_tab = np.concatenate([outer.real, outer.imag, twiddle.real, twiddle.imag]).astype(np.float32)
    return f_tab, g_tab, n_tab


_F_TAB, _G_TAB, _N_TAB = _tables()


def _kernel(xa_hbm, wr_hbm, wi_hbm, xb_hbm, mem0_hbm, wq_hbm, wk_hbm, wv_hbm, wo_hbm, f_hbm, g_hbm, n_hbm,
            out_hbm,
            wqkv, wo, stage, xb, xtail, bk, mem0, ya, outb, h_scr, o_scr, acc_scr,
            sem_w, sem_o, sem_x, sem_out):

    def w_copy(i, c):
        rows = pl.ds(_aligned(c * WP, WP), WP)
        return pltpu.make_async_copy(
            (wq_hbm, wk_hbm, wv_hbm)[i].bitcast(jnp.uint32).at[rows], stage[i].at[rows, pl.ds(0, H), :],
            sem_w.at[i * NW + c])

    def wo_copy(n):
        return pltpu.make_async_copy(wo_hbm.bitcast(jnp.uint32).at[:, pl.ds(128 * n, 128)], wo.at[n], sem_o.at[n])

    def xb_copy(t):
        part = pl.ds(0, FIRST) if t == 0 else pl.ds(FIRST, NSEG - FIRST)
        return pltpu.make_async_copy(xb_hbm.at[part], xb.at[part], sem_x.at[4 * t])

    mem_copy = pltpu.make_async_copy(mem0_hbm, mem0, sem_x.at[1])
    xtail_copy = pltpu.make_async_copy(xb_hbm.at[:, pl.ds(SEG - TAIL, TAIL), :], xtail, sem_x.at[2])
    ya_copy = pltpu.make_async_copy(ya, out_hbm.at[:, :, pl.ds(0, D)], sem_x.at[3])

    def relayout(i, c, part):
        flat = stage[i].reshape((D // 2 + 4) * PITCH, DH)
        src = flat.at[pl.ds(_aligned(c * (WP * PITCH), WP * PITCH), (WP + 1) * PITCH), :]
        rows = pl.ds(_aligned(c * WP, WP), WP)
        for j in (2 * part, 2 * part + 1):
            a = src[pl.ds(j, WP, stride=PITCH), :]
            b = src[pl.ds(H // 2 + j, WP, stride=PITCH), :]
            wqkv[i * H + 2 * j, rows, :] = _low_halves(a, b)
            wqkv[i * H + 2 * j + 1, rows, :] = _high_halves(a, b)

    def branch_a(xa, f_tab, g_src, g_tab, n_tab, nyq, w_st, w_last, w_perm, outer_out, spec,
                 sem_a, sem_f, sem_c):
        def xa_copy(i):
            return pltpu.make_async_copy(xa_hbm.at[:, pl.ds(_aligned(CB * i, CB), CB), :], xa.at[i], sem_a.at[i])

        def f_copy(t):
            part = pl.ds(4 * t, 4 + 2 * t)
            return pltpu.make_async_copy(f_hbm.at[part], f_tab.at[part], sem_c.at[t])

        def filter_copy(t, ub):
            src = (wr_hbm, wi_hbm)[t].at[pl.ds(0, D // 2), :].bitcast(jnp.uint32)
            return pltpu.make_async_copy(
                src.at[:, pl.ds(_aligned(128 * ub, 128), 128)], w_st.at[t, ub, pl.ds(0, D // 4), :],
                sem_f.at[t * P + ub])

        def last_copy(t):
            return pltpu.make_async_copy(
                (wr_hbm, wi_hbm)[t].at[pl.ds(D // 2, 1), :], w_last.at[t], sem_c.at[2 + t])

        n_copy = pltpu.make_async_copy(n_hbm, n_tab, sem_c.at[4])
        g_copy = pltpu.make_async_copy(g_hbm, g_src, sem_c.at[5])

        def start_filter(ub):
            filter_copy(0, ub).start()
            filter_copy(1, ub).start()

        def wait_filter(ub):
            filter_copy(0, ub).wait()
            filter_copy(1, ub).wait()

        def start_small():
            last_copy(0).start()
            last_copy(1).start()
            mem_copy.start()

        first_copies = [
            g_copy.start,
            lambda: xa_copy(0).start(),
            lambda: f_copy(0).start(),
            n_copy.start,
            lambda: _in_order(NCH - 1, lambda i: xa_copy(i + 1).start()),
            start_small,
            lambda: _in_order(P, start_filter),
        ]

        def start_first(t):
            for n, start in enumerate(first_copies):
                pl.when(t == n)(start)

        _in_order(len(first_copies), start_first)

        lane0 = jax.lax.broadcasted_iota(jnp.int32, (8, 128), 1) == 0

        def inner_matrices(t, carry):
            for u in range(4):
                n = 4 * t + u
                m = (g_src[0:Q, :] * g_src[pl.ds(2 * Q + n, 1), :]
                     + g_src[Q:2 * Q, :] * g_src[pl.ds(2 * Q + 2 * P + n, 1), :])
                g_tab[n] = _words(m)
                g_tab[2 * P + n] = _words(m.T)
            return carry

        g_copy.wait()
        jax.lax.fori_loop(0, 2 * P // 4, inner_matrices, 0)

        def forward(i, carry):
            xa_copy(i).wait()

            @pl.when(i == 0)
            def _():
                f_copy(0).wait()
                n_copy.wait()

            @pl.when(i == 4)
            def _():
                f_copy(1).start()

            @pl.when(i == 5)
            def _():
                _in_order(NW // 2, lambda c: w_copy(0, c).start())

            @pl.when(i == 6)
            def _():
                xtail_copy.start()

            @pl.when(i == 7)
            def _():
                _in_order(NW // 2, lambda c: w_copy(0, NW // 2 + c).start())

            combos = []
            for a in range(P):
                x = xa[i, a].astype(jnp.float32)
                combos.append(_radix8([x[:, 128 * c:128 * c + 128] for c in range(8)]))

            def features(j, hh):
                lhs = jnp.concatenate(
                    [jnp.concatenate([p[8 * hh:8 * hh + 8] for p in combos[a][2 * j:2 * j + 2]], 1)
                     for a in range(P)], 0)
                return _dot(lhs, _bf16(f_tab[j]))

            def outer(j, hh, x):
                xr = [x[8 * a:8 * a + 8, :128] for a in range(P)]
                xi = [x[8 * a:8 * a + 8, 128:] for a in range(P)]
                rows = pl.ds(pl.multiple_of(i * CB + 8 * hh, 8), 8)
                if j == 0:
                    re = im = None
                    for a in range(P):
                        t = jnp.broadcast_to(xi[a][:, 0:1], (8, 128))
                        pr, pi = t * n_tab[a:a + 1, :], t * n_tab[P + a:P + a + 1, :]
                        re, im = (pr, pi) if a == 0 else (re + pr, im + pi)
                    nyq[0, rows, :] = re
                    nyq[1, rows, :] = im
                    xi = [jnp.where(lane0, 0.0, v) for v in xi]
                yr, yi = _radix16(xr, xi)
                for k in range(P):
                    outer_out[k, rows, 128 * j:128 * j + 128] = _words(jnp.concatenate([yr[k], yi[k]], 0))

            parts = [(j, hh) for j in range(NB) for hh in range(CB // 8)]
            pending = {}
            for n in range(len(parts) + 1):
                if n < len(parts):
                    pending[n] = features(*parts[n])
                if n >= 1:
                    outer(*parts[n - 1], pending.pop(n - 1))
            return carry

        jax.lax.fori_loop(0, NCH, forward, 0)

        def filter_tile(ub, j):
            parts = []
            for cls in CLASSES[j]:
                a = w_st[0, ub, pl.ds(cls // 2, 64, stride=4), :]
                b = w_st[1, ub, pl.ds(cls // 2, 64, stride=4), :]
                parts.append(_high_halves(a, b) if cls % 2 else _low_halves(a, b))
            t = jnp.concatenate(parts, 0).T
            for m in range(4):
                r0 = (4 * ub + m) * PITCH
                w_perm[j, r0:r0 + 32, :] = t[32 * m:32 * m + 32]

        def halves(k, j):
            x = _bf16(outer_out[k, :, 128 * j:128 * j + 128]).astype(jnp.float32)
            even, odd = [], []
            for t in range(Q // 16):
                lr, li = x[16 * t:16 * t + 8], x[16 * t + 8:16 * t + 16]
                hr, hi = _twiddle(x[Q + 16 * t:Q + 16 * t + 8], x[Q + 16 * t + 8:Q + 16 * t + 16], k, 2 * P)
                even += [lr + hr, li + hi]
                odd += [lr - hr, li - hi]
            return [jnp.concatenate(v, 0).astype(jnp.bfloat16) for v in (even, odd)]

        last_copy(0).wait()
        last_copy(1).wait()
        for c in range(NW):
            w_copy(1, c).start()
        ready = 0
        for group, count in enumerate((4, 6)):
            tiles = []
            for ub in range(ready, ready + count):
                wait_filter(ub)
                tiles += [(ub, j) for j in range(NB)]
            ready += count
            items = [(k, j) for k in range(P // 2 * group, P // 2 * (group + 1)) for j in range(NB)]
            rhs = halves(*items[0])
            for n, (k, j) in enumerate(items):
                rhs_next = halves(*items[n + 1]) if n + 1 < len(items) else None
                for e in range(2):
                    spec[k, e, :, 128 * j:128 * j + 128] = _dot(_bf16(g_tab[2 * k + e]), rhs[e])
                rhs = rhs_next
                for t in tiles[n * len(tiles) // len(items):(n + 1) * len(tiles) // len(items)]:
                    filter_tile(*t)

        def filtered(k, j):
            res = []
            for e in range(2):
                x = spec[k, e, :, 128 * j:128 * j + 128]
                w = w_perm[j, pl.ds(k + P * e, Q // 2, stride=PITCH), :]
                wr = jax.lax.bitcast_convert_type(w << 16, jnp.float32)
                wi = jax.lax.bitcast_convert_type(w & jnp.uint32(0xFFFF0000), jnp.float32)
                out = []
                for t in range(Q // 16):
                    xr, xi = x[16 * t:16 * t + 8], x[16 * t + 8:16 * t + 16]
                    a, b = wr[8 * t:8 * t + 8], wi[8 * t:8 * t + 8]
                    out += [xr * a - xi * b, xr * b + xi * a]
                res.append(jnp.concatenate(out, 0).astype(jnp.bfloat16))
            return res

        def merge(k, j, even, odd):
            lo, hi = [], []
            for t in range(Q // 16):
                er, ei = even[16 * t:16 * t + 8], even[16 * t + 8:16 * t + 16]
                dr, di = odd[16 * t:16 * t + 8], odd[16 * t + 8:16 * t + 16]
                lo += [er + dr, ei + di]
                hi += list(_twiddle(er - dr, ei - di, -k, 2 * P))
            spec[k, 0, :, 128 * j:128 * j + 128] = jnp.concatenate(lo, 0)
            spec[k, 1, :, 128 * j:128 * j + 128] = jnp.concatenate(hi, 0)

        for ub in range(ready, P):
            wait_filter(ub)
        for c in range(NW):
            w_copy(2, c).start()
        for ub in range(ready, P):
            filter_tile(ub, 0)
        items = [(k, j) for j in range(NB) for k in range(P)]
        y = filtered(*items[0])
        prev = None
        for n, (k, j) in enumerate(items):
            if j + 1 < NB and k < P - ready:
                filter_tile(ready + k, j + 1)
            y_next = filtered(*items[n + 1]) if n + 1 < len(items) else None
            cur = [_dot(_bf16(g_tab[2 * P + 2 * k + e]), y[e]) for e in range(2)]
            if prev is not None:
                merge(*items[n - 1], *prev)
            prev, y = cur, y_next
        merge(*items[-1], *prev)

        def nyquist_column():
            row = jax.lax.broadcasted_iota(jnp.int32, (8, 128), 0)
            lane = jax.lax.broadcasted_iota(jnp.int32, (8, 128), 1)
            idx = (P * row + lane) & 127

            def twiddles(t):
                r0 = 2 * P + 8 * t
                return n_tab[r0:r0 + 8, :], n_tab[Q + r0:Q + r0 + 8, :]

            out = []
            for t in range(Q // 8):
                c, s = twiddles(t)
                re, im = nyq[0, 8 * t:8 * t + 8, :], nyq[1, 8 * t:8 * t + 8, :]
                out += [re * c - im * s, re * s + im * c]
            x = _dot(_bf16(f_tab[8]), jnp.concatenate(out, 0).astype(jnp.bfloat16))
            out = []
            for t in range(Q // 8):
                a, b = [
                    jnp.where(lane < P, jnp.take_along_axis(
                        jnp.broadcast_to(w_last[p, :, 128 * t:128 * t + 128].astype(jnp.float32), (8, 128)),
                        idx, axis=1, mode="promise_in_bounds"), 0.0)
                    for p in range(2)]
                xr, xi = x[16 * t:16 * t + 8], x[16 * t + 8:16 * t + 16]
                out += [xr * a - xi * b, xr * b + xi * a]
            z = _dot(_bf16(f_tab[9]), jnp.concatenate(out, 0).astype(jnp.bfloat16))
            for t in range(Q // 8):
                c, s = twiddles(t)
                re, im = z[16 * t:16 * t + 8], z[16 * t + 8:16 * t + 16]
                nyq[0, 8 * t:8 * t + 8, :] = re * c + im * s
                nyq[1, 8 * t:8 * t + 8, :] = im * c - re * s

        freq, combos = {}, {}

        def inverse_outer(i, j, hh):
            r0 = i * CB + 8 * hh
            half, t0 = divmod(2 * r0, Q)
            b = [spec[k, half, t0:t0 + 16, 128 * j:128 * j + 128] for k in range(P)]
            zi, zr = _radix16([x[8:16] for x in b], [x[0:8] for x in b])
            if j == 0:
                for a in range(P):
                    z = (nyq[0, r0:r0 + 8, :] * n_tab[a:a + 1, :]
                         + nyq[1, r0:r0 + 8, :] * n_tab[P + a:P + a + 1, :])
                    zi[a] = jnp.where(lane0, jnp.sum(z, axis=1, keepdims=True), zi[a])
            freq[i, j, hh] = jnp.concatenate([jnp.concatenate([zr[a], zi[a]], 1) for a in range(P)], 0)

        def inverse_features(i, j, hh):
            combos[i, j, hh] = _dot(freq[i, j, hh], _bf16(f_tab[4 + j]))

        def inverse_radix8(i, a):
            out = _radix8_transposed([
                jnp.concatenate([combos[i, c // 2, hh][8 * a:8 * a + 8, 128 * (c % 2):128 * (c % 2) + 128]
                                 for hh in range(2)], 0)
                for c in range(8)])
            for c in range(8):
                ya[a, CB * i:CB * i + CB, 128 * c:128 * c + 128] = out[c].astype(jnp.bfloat16)

        f_copy(1).wait()
        xb_copy(0).start()
        for n in range(8):
            wo_copy(n).start()
        nyquist_column()
        for t in range(NCH + 2):
            if t in (4, 6):
                w_copy(0, t - 4).wait()
                w_copy(0, t - 3).wait()
            if t == 4:
                xb_copy(1).start()
            for q in range(8):
                n = 8 * t + q - 2
                if 0 <= n < 8 * NCH:
                    inverse_features(n // 8, (n % 8 // 2 + 1) % 4, n % 2)
                if t < NCH:
                    inverse_outer(t, (q // 2 + 1) % 4, q % 2)
                n = 8 * t + q - 12
                if 0 <= n < 8 * NCH:
                    inverse_radix8(n // 8, 2 * (n % 8))
                    inverse_radix8(n // 8, 2 * (n % 8) + 1)
                if 4 <= t < 8:
                    relayout(0, t - 4, q)

    pl.run_scoped(
        branch_a,
        pltpu.VMEM((NCH, P, CB, D), jnp.bfloat16),
        pltpu.VMEM(_F_TAB.shape, jnp.uint32),
        pltpu.VMEM(_G_TAB.shape, jnp.float32),
        pltpu.VMEM((4 * P, Q // 2, Q), jnp.uint32),
        pltpu.VMEM(_N_TAB.shape, jnp.float32),
        pltpu.VMEM((2, Q, 128), jnp.float32),
        pltpu.VMEM((2, P, D // 4 + 32, 128), jnp.uint32),
        pltpu.VMEM((2, 1, S), jnp.bfloat16),
        pltpu.VMEM((NB, (S // 32 + 1) * PITCH, 128), jnp.uint32),
        pltpu.VMEM((P, Q, NB * 128), jnp.uint32),
        pltpu.VMEM((P, 2, Q, NB * 128), jnp.float32),
        pltpu.SemaphoreType.DMA((NCH,)),
        pltpu.SemaphoreType.DMA((2 * P,)),
        pltpu.SemaphoreType.DMA((6,)),
    )

    bq = stage[0].reshape((D // 2 + 4) * PITCH, DH)
    nb = NSEG * TAIL

    def tail_rows(m, parts, cols):
        n = NSEG // parts
        x = xtail[m * n:(m + 1) * n, :, cols]
        return x.reshape(n * TAIL, x.shape[-1])

    def interleave(dots, pieces):
        for n, dot in enumerate(dots):
            dot()
            for piece in pieces[n * len(pieces) // len(dots):(n + 1) * len(pieces) // len(dots)]:
                relayout(*piece)

    def q_first_half(c, carry):
        for t in range(2):
            w_copy(0, NW // 2 + 2 * c + t).wait()

        def one(hd):
            bk[hd] = _dot(tail_rows(0, 1, slice(0, D // 2)), _bf16(wqkv[hd, :D // 4, :]))

        interleave([functools.partial(one, c * 16 + u) for u in range(16)],
                   [(0, NW // 2 + 2 * c + u // 8, u % 8) for u in range(16)])
        return carry

    def q_second_half(c, carry):
        for t in range(4):
            w_copy(1, 4 * c + t).wait()

        def one(hd, m):
            n = nb // 2
            r = bk[hd, m * n:(m + 1) * n, :] + _dot(tail_rows(m, 2, slice(D // 2, D)), _bf16(wqkv[hd, D // 4:, :]))
            bq[pl.ds(pl.multiple_of(hd * nb + m * n, n), n), :] = jax.lax.bitcast_convert_type(r, jnp.uint32)

        interleave([functools.partial(one, c * 16 + u, m) for u in range(16) for m in range(2)],
                   [(1, 4 * c + u // 8, u % 8) for u in range(32)])
        return carry

    def k_heads(c, carry):
        for t in range(2):
            w_copy(2, 2 * c + t).wait()

        def one(hd, m):
            n = nb // 4
            bk[hd, m * n:(m + 1) * n, :] = _dot(tail_rows(m, 4, slice(0, D)), _bf16(wqkv[H + hd]))

        interleave([functools.partial(one, c * (HB // 4) + u, m) for u in range(HB // 4) for m in range(4)],
                   [(2, 2 * c + u // 8, u % 8) for u in range(16)])
        return carry

    xtail_copy.wait()
    jax.lax.fori_loop(0, 2, q_first_half, 0)
    jax.lax.fori_loop(0, 2, q_second_half, 0)
    jax.lax.fori_loop(0, 4, k_heads, 0)
    for n in range(8):
        wo_copy(n).wait()
    xb_copy(0).wait()
    mem_copy.wait()
    ya_copy.start()

    scale = DH ** -0.5
    h_scr[0:M, :] = mem0[...].astype(jnp.float32)
    qi = jax.lax.broadcasted_iota(jnp.int32, (L, L), 0)
    ki = jax.lax.broadcasted_iota(jnp.int32, (L, L), 1)
    mask = (qi < M) | (qi >= ki)

    def out_copy(s):
        return pltpu.make_async_copy(
            outb.at[s], out_hbm.at[s >> 2, pl.ds(pl.multiple_of((s & 3) * SEG, SEG), SEG), pl.ds(D, D)], sem_out)

    def step(s):
        h_scr[M:L, :] = xb[s].astype(jnp.float32)

        def project(i, hd):
            w = _bf16(wqkv[i * H + hd])
            if i == 0:
                head = _dot(h_scr[0:L - TAIL, :], w)
                tail = jax.lax.bitcast_convert_type(
                    bq[pl.ds(pl.multiple_of(hd * nb + s * TAIL, TAIL), TAIL), :], jnp.float32)
            elif i == 1 and hd < HB:
                head = _dot(h_scr[0:L - TAIL, :], w)
                tail = bk[hd, pl.ds(pl.multiple_of(s * TAIL, TAIL), TAIL), :]
            else:
                return _dot(h_scr[...], w)
            return jnp.concatenate([head, tail], 0)

        def output_first_part(n):
            acc_scr[:, 128 * n:128 * n + 128] = _dot(o_scr[:, 0:SPLIT * DH], _bf16(wo[n, 0:SPLIT * DH // 2, :]))

        qkv, scores, probs = {}, {}, {}
        for i in range(H + 4):
            if i < H:
                qkv[i] = (project(0, i), project(1, i).astype(jnp.bfloat16), project(2, i).astype(jnp.bfloat16))
            else:
                for n in range(3 * (i - H), min(3 * (i - H) + 3, 8)):
                    output_first_part(n)
            if 0 <= i - 1 < H:
                scores[i - 1] = _dot(qkv[i - 1][0], qkv[i - 1][1], NT)
            if 0 <= i - 2 < H:
                z = jnp.where(mask, scores.pop(i - 2) * scale, -1e9)
                e = jnp.exp(z - jnp.max(z, axis=-1, keepdims=True))
                probs[i - 2] = e / jnp.sum(e, axis=-1, keepdims=True)
            if i - 4 >= 0:
                o_scr[:, (i - 4) * DH:(i - 3) * DH] = _dot(probs.pop(i - 4), qkv.pop(i - 4)[2])
        for n in range(8):
            r = _dot(o_scr[:, SPLIT * DH:], _bf16(wo[n, SPLIT * DH // 2:, :])) + acc_scr[:, 128 * n:128 * n + 128]
            h_scr[0:M, 128 * n:128 * n + 128] = r[0:M]
            outb[s, :, 128 * n:128 * n + 128] = r[M:L].astype(jnp.bfloat16)
        out_copy(s).start()

    def steps(t, carry):
        for u in range(UNROLL):
            step(t * UNROLL + u)
        return carry

    def phase(g, carry):
        jax.lax.fori_loop(g * (FIRST // UNROLL), (FIRST + g * (NSEG - FIRST)) // UNROLL, steps, 0)
        pl.when(g == 0)(lambda: xb_copy(1).wait())
        return carry

    jax.lax.fori_loop(0, 2, phase, 0)
    _in_order(NSEG, lambda s: out_copy(s).wait())
    ya_copy.wait()


@functools.partial(jax.jit, static_argnames=("B_seg_len",))
def pallas_concat_heads__spectral_gfnet__memory_aug_recurrent_mem_tr__prompt_kernel(
    A_x, A_w_r, A_w_i, B_x, B_mem0, B_Wq, B_Wk, B_Wv, B_Wo, B_seg_len,
):
    assert A_x.shape == B_x.shape == (1, S, D) and B_mem0.shape == (1, M, D) and B_seg_len == SEG
    assert B_Wq.shape == B_Wk.shape == B_Wv.shape == (D, H, DH) and B_Wo.shape == (H, DH, D)
    hbm = pl.BlockSpec(memory_space=pltpu.HBM)
    out = pl.pallas_call(
        _kernel,
        out_shape=jax.ShapeDtypeStruct((P, Q, 2 * D), jnp.bfloat16),
        in_specs=[hbm] * 12,
        out_specs=hbm,
        scratch_shapes=[
            pltpu.VMEM((3 * H, D // 2, DH), jnp.uint32),
            pltpu.VMEM((8, H * DH // 2, 128), jnp.uint32),
            [pltpu.VMEM((D // 2 + 4, PITCH, DH), jnp.uint32)] * 3,
            pltpu.VMEM((NSEG, SEG, D), jnp.bfloat16),
            pltpu.VMEM((NSEG, TAIL, D), jnp.bfloat16),
            pltpu.VMEM((H, NSEG * TAIL, DH), jnp.float32),
            pltpu.VMEM((M, D), jnp.bfloat16),
            pltpu.VMEM((P, Q, D), jnp.bfloat16),
            pltpu.VMEM((NSEG, SEG, D), jnp.bfloat16),
            pltpu.VMEM((L, D), jnp.float32),
            pltpu.VMEM((L, H * DH), jnp.float32),
            pltpu.VMEM((L, D), jnp.float32),
            pltpu.SemaphoreType.DMA((3 * NW,)),
            pltpu.SemaphoreType.DMA((8,)),
            pltpu.SemaphoreType.DMA((5,)),
            pltpu.SemaphoreType.DMA(()),
        ],
        compiler_params=pltpu.CompilerParams(vmem_limit_bytes=120 * 1024 * 1024),
    )(
        A_x.reshape(P, Q, D), A_w_r.T, A_w_i.T,
        B_x.reshape(NSEG, SEG, D), B_mem0.reshape(M, D),
        B_Wq.reshape(D // 2, 2 * H, DH), B_Wk.reshape(D // 2, 2 * H, DH), B_Wv.reshape(D // 2, 2 * H, DH),
        B_Wo.reshape(H * DH, D), _F_TAB, _G_TAB, _N_TAB,
    )
    return out.reshape(1, S, 2 * D)
```

```python
import functools

import jax
import jax.numpy as jnp
import numpy as np
from jax.experimental import pallas as pl
from jax.experimental.pallas import tpu as pltpu

S, D = 2048, 1024
H, DH, M, SEG = 32, 128, 8, 32
L = M + SEG
NSEG = S // SEG

P, Q = 16, 128
CB = 16
NCH = Q // CB
NB = 4
CLASSES = ((0, 4), (1, 7), (2, 6), (3, 5))

TAIL = 8
HB = 24
NW = 8
WP = D // 2 // NW
PITCH = 40
SPLIT = 16
FIRST = 8
UNROLL = 2

RS = float(np.sqrt(0.5))
NN = (((1,), (0,)), ((), ()))
NT = (((1,), (1,)), ((), ()))


def _dot(a, b, dims=NN):
    return jax.lax.dot_general(a, b, dims, preferred_element_type=jnp.float32)


def _bf16(words):
    return pltpu.bitcast(words, jnp.bfloat16)


def _words(x):
    return pltpu.bitcast(x.astype(jnp.bfloat16), jnp.uint32)


def _low_halves(a, b):
    return (a & jnp.uint32(0xFFFF)) | (b << 16)


def _high_halves(a, b):
    return (a >> 16) | (b & jnp.uint32(0xFFFF0000))


def _aligned(start, multiple):
    return start if isinstance(start, int) else pl.multiple_of(start, multiple)


def _in_order(n, start):
    def body(t, carry):
        start(t)
        return carry

    jax.lax.fori_loop(0, n, body, 0)


def _radix8(x):
    t0 = x[0] + x[4]; t1 = x[0] - x[4]; t2 = x[2] + x[6]; t3 = x[2] - x[6]
    t4 = x[1] + x[5]; t5 = x[1] - x[5]; t6 = x[3] + x[7]; t7 = x[3] - x[7]
    e = t0 + t2; o = t4 + t6
    u = (t5 - t7) * RS; w = (t5 + t7) * RS
    return [e + o, e - o, t1 + u, t3 + w, t0 - t2, t4 - t6, t1 - u, t3 - w]


def _radix8_transposed(p):
    e = p[0] + p[1]; o = p[0] - p[1]
    t1 = p[2] + p[6]; u = (p[2] - p[6]) * RS
    t3 = p[3] + p[7]; w = (p[3] - p[7]) * RS
    t0 = e + p[4]; t2 = e - p[4]
    t4 = o + p[5]; t6 = o - p[5]
    t5 = w + u; t7 = w - u
    return [t0 + t1, t4 + t5, t2 + t3, t6 + t7, t0 - t1, t4 - t5, t2 - t3, t6 - t7]


def _radix4(ar, ai):
    s0r = ar[0] + ar[2]; s0i = ai[0] + ai[2]; d0r = ar[0] - ar[2]; d0i = ai[0] - ai[2]
    s1r = ar[1] + ar[3]; s1i = ai[1] + ai[3]; d1r = ar[1] - ar[3]; d1i = ai[1] - ai[3]
    return ([s0r + s1r, d0r + d1i, s0r - s1r, d0r - d1i],
            [s0i + s1i, d0i - d1r, s0i - s1i, d0i + d1r])


def _twiddle(r, i, e, n):
    e %= n
    if e == 0:
        return r, i
    if 8 * e % n == 0:
        octant = 8 * e // n
        if octant == 2:
            return i, -r
        if octant == 4:
            return -r, -i
        if octant == 6:
            return -i, r
        if octant == 1:
            return (r + i) * RS, (i - r) * RS
        if octant == 3:
            return (i - r) * RS, (r + i) * (-RS)
        if octant == 5:
            return (r + i) * (-RS), (r - i) * RS
        return (r - i) * RS, (r + i) * RS
    c, s = float(np.cos(2 * np.pi * e / n)), float(-np.sin(2 * np.pi * e / n))
    return r * c - i * s, r * s + i * c


def _radix16(xr, xi):
    ur = [[None] * 4 for _ in range(4)]
    ui = [[None] * 4 for _ in range(4)]
    for n in range(4):
        pr, pi = _radix4([xr[4 * m + n] for m in range(4)], [xi[4 * m + n] for m in range(4)])
        for p in range(4):
            ur[n][p], ui[n][p] = _twiddle(pr[p], pi[p], n * p, 16)
    yr = [None] * 16
    yi = [None] * 16
    for p in range(4):
        qr, qi = _radix4([ur[n][p] for n in range(4)], [ui[n][p] for n in range(4)])
        for q in range(4):
            yr[p + 4 * q], yi[p + 4 * q] = qr[q], qi[q]
    return yr, yi


def _real_form(z):
    n = z.shape[0]
    r = np.arange(2 * n)
    order = (r >> 4) * 8 + (r & 7) + n * ((r >> 3) & 1)
    return np.block([[z.real, -z.imag], [z.imag, z.real]])[order][:, order]


def _tables():
    lane = np.arange(128)
    combos = np.exp(-2j * np.pi * np.outer(np.arange(8), np.arange(8)) / 8) @ np.linalg.inv(
        np.array(_radix8(list(np.eye(8)))))
    f = np.zeros((NB, 256, 256))
    for j in range(NB):
        cls = np.where(lane >= 64, CLASSES[j][1], CLASSES[j][0])
        phase = np.exp(-2j * np.pi * (np.outer(lane, 8 * (lane & 63) + cls) % D) / D)
        for half in range(2):
            z = combos[cls, 2 * j + half][None, :] * phase
            f[j, 128 * half:128 * half + 128, :128] = z.real
            f[j, 128 * half:128 * half + 128, 128:] = z.imag
    f[0, :128, 128] = combos[0, 0].real * (1 - 2 * (lane % 2))
    f[0, 128:, 128] = 0
    f_inv = np.transpose(f, (0, 2, 1)) * (2.0 / (S * D))
    f_inv[0, 0, :] *= 0.5
    f_inv[0, 128, :] *= 0.5
    dft128 = _real_form(np.exp(-2j * np.pi * np.outer(np.arange(Q), np.arange(Q)) / Q))
    bits = np.concatenate([f, f_inv, dft128[None], dft128.T[None]]).astype(np.float32).view(np.uint32)
    bits = (bits + 0x7FFF + ((bits >> 16) & 1)) >> 16
    f_tab = np.ascontiguousarray(bits[:, 0::2, :] | (bits[:, 1::2, :] << 16))
    z = np.exp(-2j * np.pi * np.outer(np.arange(Q // 2), np.arange(Q // 2)) / (Q // 2))
    residue = np.array([k + P * e for k in range(P) for e in range(2)])
    col = np.exp(-2j * np.pi * np.outer(residue, (lane >> 4) * 8 + (lane & 7)) / S)
    g_tab = np.concatenate([_real_form(z), _real_form(1j * z), col.real, col.imag]).astype(np.float32)
    outer = np.exp(-2j * np.pi * np.outer(np.arange(P), lane) / P) * (lane < P)
    twiddle = np.exp(-2j * np.pi * np.outer(np.arange(Q), lane) / S) * (lane < P)
    n_tab = np.concatenate([outer.real, outer.imag, twiddle.real, twiddle.imag]).astype(np.float32)
    return f_tab, g_tab, n_tab


_F_TAB, _G_TAB, _N_TAB = _tables()


def _kernel(xa_hbm, wr_hbm, wi_hbm, xb_hbm, mem0_hbm, wq_hbm, wk_hbm, wv_hbm, wo_hbm, f_hbm, g_hbm, n_hbm,
            out_hbm,
            wqkv, wo, stage, xb, xtail, bk, mem0, ya, outb, h_scr, o_scr, acc_scr,
            sem_w, sem_o, sem_x, sem_out):

    def w_copy(i, c):
        return pltpu.make_async_copy(
            (wq_hbm, wk_hbm, wv_hbm)[i].bitcast(jnp.uint32).at[pl.ds(c * WP, WP)],
            stage[i].at[pl.ds(c * (WP + 1), WP), pl.ds(0, H), :], sem_w.at[i * NW + c])

    def wo_copy(n):
        return pltpu.make_async_copy(wo_hbm.bitcast(jnp.uint32).at[:, pl.ds(128 * n, 128)], wo.at[n], sem_o.at[n])

    def xb_copy(t):
        part = pl.ds(0, FIRST) if t == 0 else pl.ds(FIRST, NSEG - FIRST)
        return pltpu.make_async_copy(xb_hbm.at[part], xb.at[part], sem_x.at[4 * t])

    mem_copy = pltpu.make_async_copy(mem0_hbm, mem0, sem_x.at[1])
    xtail_copy = pltpu.make_async_copy(xb_hbm.at[:, pl.ds(SEG - TAIL, TAIL), :], xtail, sem_x.at[2])
    ya_copy = pltpu.make_async_copy(ya, out_hbm.at[:, :, pl.ds(0, D)], sem_x.at[3])

    def relayout(i, c, part):
        span = (WP + 1) * PITCH
        src = stage[i].reshape(NW * span, DH).at[pl.ds(_aligned(c * span, PITCH), span), :]
        rows = pl.ds(_aligned(c * WP, WP), WP)
        for j in (2 * part, 2 * part + 1):
            a = src[pl.ds(j, WP, stride=PITCH), :]
            b = src[pl.ds(H // 2 + j, WP, stride=PITCH), :]
            wqkv[i * H + 2 * j, rows, :] = _low_halves(a, b)
            wqkv[i * H + 2 * j + 1, rows, :] = _high_halves(a, b)

    def branch_a(xa, f_tab, g_src, g_tab, n_tab, nyq, w_st, w_last, w_perm, outer_out, spec,
                 sem_a, sem_f, sem_c):
        def xa_copy(i):
            return pltpu.make_async_copy(xa_hbm.at[:, pl.ds(_aligned(CB * i, CB), CB), :], xa.at[i], sem_a.at[i])

        def f_copy(t):
            part = pl.ds(4 * t, 4 + 2 * t)
            return pltpu.make_async_copy(f_hbm.at[part], f_tab.at[part], sem_c.at[t])

        def filter_copy(t, ub):
            src = (wr_hbm, wi_hbm)[t].at[pl.ds(0, D // 2), :].bitcast(jnp.uint32)
            return pltpu.make_async_copy(
                src.at[:, pl.ds(_aligned(128 * ub, 128), 128)], w_st.at[t, ub, pl.ds(0, D // 4), :],
                sem_f.at[t * P + ub])

        def last_copy(t):
            return pltpu.make_async_copy(
                (wr_hbm, wi_hbm)[t].at[pl.ds(D // 2, 1), :], w_last.at[t], sem_c.at[2 + t])

        n_copy = pltpu.make_async_copy(n_hbm, n_tab, sem_c.at[4])
        g_copy = pltpu.make_async_copy(g_hbm, g_src, sem_c.at[5])

        def start_filter(ub):
            filter_copy(0, ub).start()
            filter_copy(1, ub).start()

        def wait_filter(ub):
            filter_copy(0, ub).wait()
            filter_copy(1, ub).wait()

        def start_small():
            last_copy(0).start()
            last_copy(1).start()
            mem_copy.start()

        first_copies = [
            g_copy.start,
            lambda: xa_copy(0).start(),
            lambda: f_copy(0).start(),
            n_copy.start,
            lambda: _in_order(NCH - 1, lambda i: xa_copy(i + 1).start()),
            start_small,
            lambda: _in_order(P, start_filter),
        ]

        def start_first(t):
            for n, start in enumerate(first_copies):
                pl.when(t == n)(start)

        _in_order(len(first_copies), start_first)

        lane0 = jax.lax.broadcasted_iota(jnp.int32, (8, 128), 1) == 0

        def inner_matrices(t, carry):
            for u in range(4):
                n = 4 * t + u
                m = (g_src[0:Q, :] * g_src[pl.ds(2 * Q + n, 1), :]
                     + g_src[Q:2 * Q, :] * g_src[pl.ds(2 * Q + 2 * P + n, 1), :])
                g_tab[n] = _words(m)
                g_tab[2 * P + n] = _words(m.T)
            return carry

        g_copy.wait()
        jax.lax.fori_loop(0, 2 * P // 4, inner_matrices, 0)

        def forward(i, carry):
            xa_copy(i).wait()

            @pl.when(i == 0)
            def _():
                f_copy(0).wait()
                n_copy.wait()

            @pl.when(i == 4)
            def _():
                f_copy(1).start()

            @pl.when(i == 5)
            def _():
                _in_order(NW // 2, lambda c: w_copy(0, c).start())

            @pl.when(i == 6)
            def _():
                xtail_copy.start()

            @pl.when(i == 7)
            def _():
                _in_order(NW // 2, lambda c: w_copy(0, NW // 2 + c).start())

            combos = []
            for a in range(P):
                x = xa[i, a].astype(jnp.float32)
                combos.append(_radix8([x[:, 128 * c:128 * c + 128] for c in range(8)]))

            def features(j, hh):
                lhs = jnp.concatenate(
                    [jnp.concatenate([p[8 * hh:8 * hh + 8] for p in combos[a][2 * j:2 * j + 2]], 1)
                     for a in range(P)], 0)
                return _dot(lhs, _bf16(f_tab[j]))

            def outer(j, hh, x):
                xr = [x[8 * a:8 * a + 8, :128] for a in range(P)]
                xi = [x[8 * a:8 * a + 8, 128:] for a in range(P)]
                rows = pl.ds(pl.multiple_of(i * CB + 8 * hh, 8), 8)
                if j == 0:
                    re = im = None
                    for a in range(P):
                        t = jnp.broadcast_to(xi[a][:, 0:1], (8, 128))
                        pr, pi = t * n_tab[a:a + 1, :], t * n_tab[P + a:P + a + 1, :]
                        re, im = (pr, pi) if a == 0 else (re + pr, im + pi)
                    nyq[0, rows, :] = re
                    nyq[1, rows, :] = im
                    xi = [jnp.where(lane0, 0.0, v) for v in xi]
                yr, yi = _radix16(xr, xi)
                for k in range(P):
                    outer_out[k, rows, 128 * j:128 * j + 128] = _words(jnp.concatenate([yr[k], yi[k]], 0))

            parts = [(j, hh) for j in range(NB) for hh in range(CB // 8)]
            pending = {}
            for n in range(len(parts) + 1):
                if n < len(parts):
                    pending[n] = features(*parts[n])
                if n >= 1:
                    outer(*parts[n - 1], pending.pop(n - 1))
            return carry

        jax.lax.fori_loop(0, NCH, forward, 0)

        def filter_tile(ub, j):
            parts = []
            for cls in CLASSES[j]:
                a = w_st[0, ub, pl.ds(cls // 2, 64, stride=4), :]
                b = w_st[1, ub, pl.ds(cls // 2, 64, stride=4), :]
                parts.append(_high_halves(a, b) if cls % 2 else _low_halves(a, b))
            t = jnp.concatenate(parts, 0).T
            for m in range(4):
                r0 = (4 * ub + m) * PITCH
                w_perm[j, r0:r0 + 32, :] = t[32 * m:32 * m + 32]

        def halves(k, j):
            x = _bf16(outer_out[k, :, 128 * j:128 * j + 128]).astype(jnp.float32)
            even, odd = [], []
            for t in range(Q // 16):
                lr, li = x[16 * t:16 * t + 8], x[16 * t + 8:16 * t + 16]
                hr, hi = _twiddle(x[Q + 16 * t:Q + 16 * t + 8], x[Q + 16 * t + 8:Q + 16 * t + 16], k, 2 * P)
                even += [lr + hr, li + hi]
                odd += [lr - hr, li - hi]
            return [jnp.concatenate(v, 0).astype(jnp.bfloat16) for v in (even, odd)]

        last_copy(0).wait()
        last_copy(1).wait()
        for c in range(NW):
            w_copy(1, c).start()
        ready = 0
        for group, count in enumerate((4, 6)):
            tiles = []
            for ub in range(ready, ready + count):
                wait_filter(ub)
                tiles += [(ub, j) for j in range(NB)]
            ready += count
            items = [(k, j) for k in range(P // 2 * group, P // 2 * (group + 1)) for j in range(NB)]
            rhs = halves(*items[0])
            for n, (k, j) in enumerate(items):
                rhs_next = halves(*items[n + 1]) if n + 1 < len(items) else None
                for e in range(2):
                    spec[k, e, :, 128 * j:128 * j + 128] = _dot(_bf16(g_tab[2 * k + e]), rhs[e])
                rhs = rhs_next
                for t in tiles[n * len(tiles) // len(items):(n + 1) * len(tiles) // len(items)]:
                    filter_tile(*t)

        def filtered(k, j):
            res = []
            for e in range(2):
                x = spec[k, e, :, 128 * j:128 * j + 128]
                w = w_perm[j, pl.ds(k + P * e, Q // 2, stride=PITCH), :]
                wr = jax.lax.bitcast_convert_type(w << 16, jnp.float32)
                wi = jax.lax.bitcast_convert_type(w & jnp.uint32(0xFFFF0000), jnp.float32)
                out = []
                for t in range(Q // 16):
                    xr, xi = x[16 * t:16 * t + 8], x[16 * t + 8:16 * t + 16]
                    a, b = wr[8 * t:8 * t + 8], wi[8 * t:8 * t + 8]
                    out += [xr * a - xi * b, xr * b + xi * a]
                res.append(jnp.concatenate(out, 0).astype(jnp.bfloat16))
            return res

        def merge(k, j, even, odd):
            lo, hi = [], []
            for t in range(Q // 16):
                er, ei = even[16 * t:16 * t + 8], even[16 * t + 8:16 * t + 16]
                dr, di = odd[16 * t:16 * t + 8], odd[16 * t + 8:16 * t + 16]
                lo += [er + dr, ei + di]
                hi += list(_twiddle(er - dr, ei - di, -k, 2 * P))
            spec[k, 0, :, 128 * j:128 * j + 128] = jnp.concatenate(lo, 0)
            spec[k, 1, :, 128 * j:128 * j + 128] = jnp.concatenate(hi, 0)

        for ub in range(ready, P):
            wait_filter(ub)
        for c in range(NW):
            w_copy(2, c).start()
        for ub in range(ready, P):
            filter_tile(ub, 0)
        items = [(k, j) for j in range(NB) for k in range(P)]
        y = filtered(*items[0])
        prev = None
        for n, (k, j) in enumerate(items):
            if j + 1 < NB and k < P - ready:
                filter_tile(ready + k, j + 1)
            y_next = filtered(*items[n + 1]) if n + 1 < len(items) else None
            cur = [_dot(_bf16(g_tab[2 * P + 2 * k + e]), y[e]) for e in range(2)]
            if prev is not None:
                merge(*items[n - 1], *prev)
            prev, y = cur, y_next
        merge(*items[-1], *prev)

        def nyquist_column():
            row = jax.lax.broadcasted_iota(jnp.int32, (8, 128), 0)
            lane = jax.lax.broadcasted_iota(jnp.int32, (8, 128), 1)
            idx = (P * row + lane) & 127

            def twiddles(t):
                r0 = 2 * P + 8 * t
                return n_tab[r0:r0 + 8, :], n_tab[Q + r0:Q + r0 + 8, :]

            out = []
            for t in range(Q // 8):
                c, s = twiddles(t)
                re, im = nyq[0, 8 * t:8 * t + 8, :], nyq[1, 8 * t:8 * t + 8, :]
                out += [re * c - im * s, re * s + im * c]
            x = _dot(_bf16(f_tab[8]), jnp.concatenate(out, 0).astype(jnp.bfloat16))
            out = []
            for t in range(Q // 8):
                a, b = [
                    jnp.where(lane < P, jnp.take_along_axis(
                        jnp.broadcast_to(w_last[p, :, 128 * t:128 * t + 128].astype(jnp.float32), (8, 128)),
                        idx, axis=1, mode="promise_in_bounds"), 0.0)
                    for p in range(2)]
                xr, xi = x[16 * t:16 * t + 8], x[16 * t + 8:16 * t + 16]
                out += [xr * a - xi * b, xr * b + xi * a]
            z = _dot(_bf16(f_tab[9]), jnp.concatenate(out, 0).astype(jnp.bfloat16))
            for t in range(Q // 8):
                c, s = twiddles(t)
                re, im = z[16 * t:16 * t + 8], z[16 * t + 8:16 * t + 16]
                nyq[0, 8 * t:8 * t + 8, :] = re * c + im * s
                nyq[1, 8 * t:8 * t + 8, :] = im * c - re * s

        freq, combos = {}, {}

        def inverse_outer(i, j, hh):
            r0 = i * CB + 8 * hh
            half, t0 = divmod(2 * r0, Q)
            b = [spec[k, half, t0:t0 + 16, 128 * j:128 * j + 128] for k in range(P)]
            zi, zr = _radix16([x[8:16] for x in b], [x[0:8] for x in b])
            if j == 0:
                for a in range(P):
                    z = (nyq[0, r0:r0 + 8, :] * n_tab[a:a + 1, :]
                         + nyq[1, r0:r0 + 8, :] * n_tab[P + a:P + a + 1, :])
                    zi[a] = jnp.where(lane0, jnp.sum(z, axis=1, keepdims=True), zi[a])
            freq[i, j, hh] = jnp.concatenate([jnp.concatenate([zr[a], zi[a]], 1) for a in range(P)], 0)

        def inverse_features(i, j, hh):
            combos[i, j, hh] = _dot(freq[i, j, hh], _bf16(f_tab[4 + j]))

        def inverse_radix8(i, a):
            out = _radix8_transposed([
                jnp.concatenate([combos[i, c // 2, hh][8 * a:8 * a + 8, 128 * (c % 2):128 * (c % 2) + 128]
                                 for hh in range(2)], 0)
                for c in range(8)])
            for c in range(8):
                ya[a, CB * i:CB * i + CB, 128 * c:128 * c + 128] = out[c].astype(jnp.bfloat16)

        f_copy(1).wait()
        xb_copy(0).start()
        for n in range(8):
            wo_copy(n).start()
        nyquist_column()
        for t in range(NCH + 2):
            if t in (4, 6):
                w_copy(0, t - 4).wait()
                w_copy(0, t - 3).wait()
            if t == 4:
                xb_copy(1).start()
            for q in range(8):
                n = 8 * t + q - 2
                if 0 <= n < 8 * NCH:
                    inverse_features(n // 8, (n % 8 // 2 + 1) % 4, n % 2)
                if t < NCH:
                    inverse_outer(t, (q // 2 + 1) % 4, q % 2)
                n = 8 * t + q - 12
                if 0 <= n < 8 * NCH:
                    inverse_radix8(n // 8, 2 * (n % 8))
                    inverse_radix8(n // 8, 2 * (n % 8) + 1)
                if 4 <= t < 8:
                    relayout(0, t - 4, q)

    pl.run_scoped(
        branch_a,
        pltpu.VMEM((NCH, P, CB, D), jnp.bfloat16),
        pltpu.VMEM(_F_TAB.shape, jnp.uint32),
        pltpu.VMEM(_G_TAB.shape, jnp.float32),
        pltpu.VMEM((4 * P, Q // 2, Q), jnp.uint32),
        pltpu.VMEM(_N_TAB.shape, jnp.float32),
        pltpu.VMEM((2, Q, 128), jnp.float32),
        pltpu.VMEM((2, P, D // 4 + 32, 128), jnp.uint32),
        pltpu.VMEM((2, 1, S), jnp.bfloat16),
        pltpu.VMEM((NB, (S // 32 + 1) * PITCH, 128), jnp.uint32),
        pltpu.VMEM((P, Q, NB * 128), jnp.uint32),
        pltpu.VMEM((P, 2, Q, NB * 128), jnp.float32),
        pltpu.SemaphoreType.DMA((NCH,)),
        pltpu.SemaphoreType.DMA((2 * P,)),
        pltpu.SemaphoreType.DMA((6,)),
    )

    bq = stage[0].reshape(NW * (WP + 1) * PITCH, DH)
    nb = NSEG * TAIL

    def tail_rows(m, parts, cols):
        n = NSEG // parts
        x = xtail[m * n:(m + 1) * n, :, cols]
        return x.reshape(n * TAIL, x.shape[-1])

    def interleave(dots, pieces):
        for n, dot in enumerate(dots):
            dot()
            for piece in pieces[n * len(pieces) // len(dots):(n + 1) * len(pieces) // len(dots)]:
                relayout(*piece)

    def q_first_half(c, carry):
        for t in range(2):
            w_copy(0, NW // 2 + 2 * c + t).wait()

        def one(hd):
            bk[hd] = _dot(tail_rows(0, 1, slice(0, D // 2)), _bf16(wqkv[hd, :D // 4, :]))

        interleave([functools.partial(one, c * 16 + u) for u in range(16)],
                   [(0, NW // 2 + 2 * c + u // 8, u % 8) for u in range(16)])
        return carry

    def q_second_half(c, carry):
        for t in range(4):
            w_copy(1, 4 * c + t).wait()

        def one(hd, m):
            n = nb // 2
            r = bk[hd, m * n:(m + 1) * n, :] + _dot(tail_rows(m, 2, slice(D // 2, D)), _bf16(wqkv[hd, D // 4:, :]))
            bq[pl.ds(pl.multiple_of(hd * nb + m * n, n), n), :] = jax.lax.bitcast_convert_type(r, jnp.uint32)

        interleave([functools.partial(one, c * 16 + u, m) for u in range(16) for m in range(2)],
                   [(1, 4 * c + u // 8, u % 8) for u in range(32)])
        return carry

    def k_heads(c, carry):
        for t in range(2):
            w_copy(2, 2 * c + t).wait()

        def one(hd, m):
            n = nb // 4
            bk[hd, m * n:(m + 1) * n, :] = _dot(tail_rows(m, 4, slice(0, D)), _bf16(wqkv[H + hd]))

        interleave([functools.partial(one, c * (HB // 4) + u, m) for u in range(HB // 4) for m in range(4)],
                   [(2, 2 * c + u // 8, u % 8) for u in range(16)])
        return carry

    xtail_copy.wait()
    jax.lax.fori_loop(0, 2, q_first_half, 0)
    jax.lax.fori_loop(0, 2, q_second_half, 0)
    jax.lax.fori_loop(0, 4, k_heads, 0)
    for n in range(8):
        wo_copy(n).wait()
    xb_copy(0).wait()
    mem_copy.wait()
    ya_copy.start()

    scale = DH ** -0.5
    h_scr[0:M, :] = mem0[...].astype(jnp.float32)
    qi = jax.lax.broadcasted_iota(jnp.int32, (L, L), 0)
    ki = jax.lax.broadcasted_iota(jnp.int32, (L, L), 1)
    mask = (qi < M) | (qi >= ki)

    def out_copy(s):
        return pltpu.make_async_copy(
            outb.at[s], out_hbm.at[s >> 2, pl.ds(pl.multiple_of((s & 3) * SEG, SEG), SEG), pl.ds(D, D)], sem_out)

    def step(s):
        h_scr[M:L, :] = xb[s].astype(jnp.float32)

        def project(i, hd):
            w = _bf16(wqkv[i * H + hd])
            if i == 0:
                head = _dot(h_scr[0:L - TAIL, :], w)
                tail = jax.lax.bitcast_convert_type(
                    bq[pl.ds(pl.multiple_of(hd * nb + s * TAIL, TAIL), TAIL), :], jnp.float32)
            elif i == 1 and hd < HB:
                head = _dot(h_scr[0:L - TAIL, :], w)
                tail = bk[hd, pl.ds(pl.multiple_of(s * TAIL, TAIL), TAIL), :]
            else:
                return _dot(h_scr[...], w)
            return jnp.concatenate([head, tail], 0)

        def output_first_part(n):
            acc_scr[:, 128 * n:128 * n + 128] = _dot(o_scr[:, 0:SPLIT * DH], _bf16(wo[n, 0:SPLIT * DH // 2, :]))

        qkv, scores, probs = {}, {}, {}
        for i in range(H + 4):
            if i < H:
                qkv[i] = (project(0, i), project(1, i).astype(jnp.bfloat16), project(2, i).astype(jnp.bfloat16))
            else:
                for n in range(3 * (i - H), min(3 * (i - H) + 3, 8)):
                    output_first_part(n)
            if 0 <= i - 1 < H:
                scores[i - 1] = _dot(qkv[i - 1][0], qkv[i - 1][1], NT)
            if 0 <= i - 2 < H:
                z = jnp.where(mask, scores.pop(i - 2) * scale, -1e9)
                e = jnp.exp(z - jnp.max(z, axis=-1, keepdims=True))
                probs[i - 2] = e / jnp.sum(e, axis=-1, keepdims=True)
            if i - 4 >= 0:
                o_scr[:, (i - 4) * DH:(i - 3) * DH] = _dot(probs.pop(i - 4), qkv.pop(i - 4)[2])
        for n in range(8):
            r = _dot(o_scr[:, SPLIT * DH:], _bf16(wo[n, SPLIT * DH // 2:, :])) + acc_scr[:, 128 * n:128 * n + 128]
            h_scr[0:M, 128 * n:128 * n + 128] = r[0:M]
            outb[s, :, 128 * n:128 * n + 128] = r[M:L].astype(jnp.bfloat16)
        out_copy(s).start()

    def steps(t, carry):
        for u in range(UNROLL):
            step(t * UNROLL + u)
        return carry

    def phase(g, carry):
        jax.lax.fori_loop(g * (FIRST // UNROLL), (FIRST + g * (NSEG - FIRST)) // UNROLL, steps, 0)
        pl.when(g == 0)(lambda: xb_copy(1).wait())
        return carry

    jax.lax.fori_loop(0, 2, phase, 0)
    _in_order(NSEG, lambda s: out_copy(s).wait())
    ya_copy.wait()


@functools.partial(jax.jit, static_argnames=("B_seg_len",))
def pallas_concat_heads__spectral_gfnet__memory_aug_recurrent_mem_tr__prompt_kernel(
    A_x, A_w_r, A_w_i, B_x, B_mem0, B_Wq, B_Wk, B_Wv, B_Wo, B_seg_len,
):
    assert A_x.shape == B_x.shape == (1, S, D) and B_mem0.shape == (1, M, D) and B_seg_len == SEG
    assert B_Wq.shape == B_Wk.shape == B_Wv.shape == (D, H, DH) and B_Wo.shape == (H, DH, D)
    hbm = pl.BlockSpec(memory_space=pltpu.HBM)
    out = pl.pallas_call(
        _kernel,
        out_shape=jax.ShapeDtypeStruct((P, Q, 2 * D), jnp.bfloat16),
        in_specs=[hbm] * 12,
        out_specs=hbm,
        scratch_shapes=[
            pltpu.VMEM((3 * H, D // 2, DH), jnp.uint32),
            pltpu.VMEM((8, H * DH // 2, 128), jnp.uint32),
            [pltpu.VMEM((NW * (WP + 1), PITCH, DH), jnp.uint32)] * 3,
            pltpu.VMEM((NSEG, SEG, D), jnp.bfloat16),
            pltpu.VMEM((NSEG, TAIL, D), jnp.bfloat16),
            pltpu.VMEM((H, NSEG * TAIL, DH), jnp.float32),
            pltpu.VMEM((M, D), jnp.bfloat16),
            pltpu.VMEM((P, Q, D), jnp.bfloat16),
            pltpu.VMEM((NSEG, SEG, D), jnp.bfloat16),
            pltpu.VMEM((L, D), jnp.float32),
            pltpu.VMEM((L, H * DH), jnp.float32),
            pltpu.VMEM((L, D), jnp.float32),
            pltpu.SemaphoreType.DMA((3 * NW,)),
            pltpu.SemaphoreType.DMA((8,)),
            pltpu.SemaphoreType.DMA((5,)),
            pltpu.SemaphoreType.DMA(()),
        ],
        compiler_params=pltpu.CompilerParams(vmem_limit_bytes=120 * 1024 * 1024),
    )(
        A_x.reshape(P, Q, D), A_w_r.T, A_w_i.T,
        B_x.reshape(NSEG, SEG, D), B_mem0.reshape(M, D),
        B_Wq.reshape(D // 2, 2 * H, DH), B_Wk.reshape(D // 2, 2 * H, DH), B_Wv.reshape(D // 2, 2 * H, DH),
        B_Wo.reshape(H * DH, D), _F_TAB, _G_TAB, _N_TAB,
    )
    return out.reshape(1, S, 2 * D)
```
